```python
import jax
import jax.numpy as jnp

def _softmax(x, axis=-1):
    return jax.nn.softmax(x, axis=axis)

def _gelu(x):
    return jax.nn.gelu(x, approximate=True)

def _silu(x):
    return jax.nn.silu(x)

def _sigmoid(x):
    return jax.nn.sigmoid(x)

def _layernorm(x, axis=-1, eps=1e-05):
    m = jnp.mean(x, axis=axis, keepdims=True)
    v = jnp.var(x, axis=axis, keepdims=True)
    return (x - m) / jnp.sqrt(v + eps)

def _scatter_add(tgt, idx, src, axis=0):
    return tgt.at[idx].add(src)

def _segment_sum(src, seg, n):
    return jax.ops.segment_sum(src, seg, n)

class _Rng:

    def __init__(self, key):
        self._k = key

    def _next(self):
        self._k, sub = jax.random.split(self._k)
        return sub

    def normal(self, shape):
        return jax.random.normal(self._next(), shape, dtype=jnp.bfloat16)

    def randint(self, lo, hi, shape):
        return jax.random.randint(self._next(), shape, lo, hi, dtype=jnp.int32)

    def uniform(self, shape, lo=0.0, hi=1.0):
        return jax.random.uniform(self._next(), shape, jnp.bfloat16, lo, hi)

    def permutation(self, n):
        return jax.random.permutation(self._next(), n)
kernel_name = 'sequential_preLN__memory_aug_infini_attn__moe_arch_mod__prompt'

def setup_inputs():
    _rng = _Rng(jax.random.key(int.from_bytes(__import__("os").urandom(4), "little")))
    _w = lambda a: (lambda t: t.astype(jnp.bfloat16) if jnp.issubdtype(t.dtype, jnp.floating) else t)(jnp.asarray(a))

    def _A_setup():
        B, S, D, H = (1, 2048, 576, 32)
        N = 4
        L = max(1, S // N)
        sc = D ** (-0.5)
        return {'x': _w((lambda *s: _rng.normal(s) * 0.05)(B, N * L, D)), 'wq': _w((lambda *s: _rng.normal(s) * 0.05)(D, D) * sc), 'wk': _w((lambda *s: _rng.normal(s) * 0.05)(D, D) * sc), 'wv': _w((lambda *s: _rng.normal(s) * 0.05)(D, D) * sc), 'wo': _w((lambda *s: _rng.normal(s) * 0.05)(D, D) * sc), 'beta': _w((lambda *s: _rng.normal(s) * 0.05)(H))}
    _A_in = _A_setup()

    def _B_setup():
        B, S, D, F, C = (1, 2048, 576, 4608, 1)
        return {'x': _w((lambda *s: _rng.normal(s) * 0.05)(B, S, D)), 'w_r': _w((lambda *s: _rng.normal(s) * 0.05)(D)), 'w_gate': _w((lambda *s: _rng.normal(s) * 0.05)(D, F)), 'w_up': _w((lambda *s: _rng.normal(s) * 0.05)(D, F)), 'w_down': _w((lambda *s: _rng.normal(s) * 0.05)(F, D))}
    _B_in = _B_setup()
    return {'A_x': _A_in['x'], 'A_wq': _A_in['wq'], 'A_wk': _A_in['wk'], 'A_wv': _A_in['wv'], 'A_wo': _A_in['wo'], 'A_beta': _A_in['beta'], 'B_x': _B_in['x'], 'B_w_r': _B_in['w_r'], 'B_w_gate': _B_in['w_gate'], 'B_w_up': _B_in['w_up'], 'B_w_down': _B_in['w_down']}

def reference(A_x, A_wq, A_wk, A_wv, A_wo, A_beta, B_x, B_w_r, B_w_gate, B_w_up, B_w_down):

    def _A_ref(x, wq, wk, wv, wo, beta):
        B, S, D = x.shape
        H = 32
        Dh = D // H
        N = 4
        L = S // N
        q = (lambda x, *d: x.transpose(*d))((x @ wq).reshape(B, S, H, Dh), 0, 2, 1, 3).reshape(B, H, N, L, Dh)
        k = (lambda x, *d: x.transpose(*d))((x @ wk).reshape(B, S, H, Dh), 0, 2, 1, 3).reshape(B, H, N, L, Dh)
        v = (lambda x, *d: x.transpose(*d))((x @ wv).reshape(B, S, H, Dh), 0, 2, 1, 3).reshape(B, H, N, L, Dh)
        phi = lambda t: jnp.where(t > 0, t + 1.0, jnp.exp(t))
        scale = Dh ** (-0.5)
        ar = jnp.arange(L)
        mask = (lambda x, dt: x.astype(dt))(ar[:, None] < ar[None, :], x.dtype) * -1000000000.0
        g = _sigmoid(beta).reshape(1, H, 1, 1)
        M = jnp.einsum('bhd,bhe->bhde', q[:, :, 0, 0, :] * 0.0, q[:, :, 0, 0, :] * 0.0)
        z = q[:, :, 0, 0, :] * 0.0
        outs = []
        for s in range(N):
            qs, ks, vs = (q[:, :, s].copy(), k[:, :, s].copy(), v[:, :, s].copy())
            logits = jnp.einsum('bhqd,bhkd->bhqk', qs, ks) * scale + mask
            p = _softmax(logits, axis=-1)
            a_dot = jnp.einsum('bhqk,bhkd->bhqd', p, vs)
            pq = phi(qs)
            num = jnp.einsum('bhld,bhde->bhle', pq, M)
            den = jnp.einsum('bhld,bhd->bhl', pq, z)[..., None] + 1e-06
            a_mem = num / den
            o = g * a_mem + (1.0 - g) * a_dot
            outs.append(o)
            pk = phi(ks)
            M = M + jnp.einsum('bhld,bhle->bhde', pk, vs)
            z = z + jnp.einsum('bhld->bhd', pk)
        o = (lambda x, *d: x.transpose(*d))(jnp.stack(outs, 2).reshape(B, H, S, Dh), 0, 2, 1, 3).reshape(B, S, D)
        return o @ wo

    def _B_ref(x, w_r, w_gate, w_up, w_down):
        B, S, D = x.shape
        C = 1
        r = x @ w_r
        idx = jnp.argsort(-r, axis=-1)[:, :C]
        idx_e = jnp.repeat(idx.reshape(B, C, 1), D, axis=2)
        x_sel = jnp.take_along_axis(x, idx_e, axis=1)
        g = _silu(x_sel @ w_gate)
        u = x_sel @ w_up
        y = g * u @ w_down
        r_sel = _sigmoid(jnp.take_along_axis(r, idx, axis=1))
        y = y * r_sel.reshape(B, C, 1)
        b_off = (jnp.arange(B) * S).reshape(B, 1)
        flat_idx = (idx + b_off).reshape(B * C)
        zero = (x * 0.0).reshape(B * S, D)
        upd = _scatter_add(zero, flat_idx, y.reshape(B * C, D), axis=0)
        return x + upd.reshape(B, S, D)
    x = A_x
    h = x + _A_ref(_layernorm(x, axis=-1), A_wq, A_wk, A_wv, A_wo, A_beta)
    h2 = h + _B_ref(_layernorm(h, axis=-1), B_w_r, B_w_gate, B_w_up, B_w_down)
    return h2
```

```python
import jax
import jax.numpy as jnp
from jax import lax
from jax.experimental import pallas as pl
from jax.experimental.pallas import tpu as pltpu

S, D, H, DH = 2048, 576, 32, 18
NSEG, L, F = 4, 512, 4608
NQ = 8
QW = 4 * DH
bf, u32, f32, i32 = jnp.bfloat16, jnp.uint32, jnp.float32, jnp.int32
LOG2E = 1.4426950408889634
QSCALE = DH ** -0.5 * LOG2E
MASKB = -1000000000.0 * LOG2E
EPS = 1e-5
NT = (((1,), (1,)), ((), ()))
ONES2 = 0x3F803F80


def _tobf(x):
    return pltpu.bitcast(x, bf)


def _tou(x):
    return pltpu.bitcast(x, u32)


def _pack(x):
    return pltpu.bitcast(x.astype(bf), u32)


def _dot(a, b):
    return jnp.dot(a, b, preferred_element_type=f32)


def _dot_nt(a, b):
    return lax.dot_general(a, b, NT, preferred_element_type=f32)


def _phi(t):
    return jnp.where(t > 0, t + 1.0, jnp.exp(t))


def _ln_t(x):
    m = jnp.mean(x, axis=0, keepdims=True)
    c = x - m
    v = jnp.mean(c * c, axis=0, keepdims=True)
    return c * lax.rsqrt(v + EPS)


def _iota(shape, dim):
    return lax.broadcasted_iota(i32, shape, dim)


def _kernel(x_hbm, wq_hbm, wk_hbm, wv_hbm, wo_hbm, beta_ref, wr_ref,
            wg_hbm, wu_hbm, wd_hbm, out_hbm,
            x_s, wq_s, wk_s, wv_s, wo_s, wg_s, wu_s, wd_s,
            w4_u, wvt_u, wot_u, xn_u, xnt_u, qx, kx, pqx, pkx, vt_u,
            s0, s1, mx0, mx1, ot_s, m_f, m_u, g_s, wr_s, out_s, ln_s, best_s, fin_s, sems):
    cp = pltpu.make_async_copy

    def x_copy(s):
        return cp(x_hbm.at[:, pl.ds(s * L, L)], x_s.at[s], sems.at[s])

    def out_copy(s):
        r = pl.multiple_of(s * L, L)
        return cp(out_s.at[s], out_hbm.at[:, pl.ds(r, L)], sems.at[11 + s])

    def ln1(s):
        xt = _ln_t(x_s[s].astype(f32)).astype(bf)
        xnt_u[...] = _tou(xt)
        xn_u[...] = _tou(xt.T)

    w_copies = [cp(wq_hbm, wq_s, sems.at[4]), cp(wk_hbm, wk_s, sems.at[5]),
                cp(wv_hbm, wv_s, sems.at[6]), cp(wo_hbm, wo_s, sems.at[7])]
    e_copies = [cp(wg_hbm, wg_s, sems.at[8]), cp(wu_hbm, wu_s, sems.at[9]),
                cp(wd_hbm, wd_s, sems.at[10])]

    x_copy(0).start()
    for c in w_copies[:3]:
        c.start()
    for s in range(1, NSEG):
        x_copy(s).start()
    w_copies[3].start()
    for c in e_copies:
        c.start()

    g32 = jax.nn.sigmoid(beta_ref[...].astype(f32)).reshape(1, H)
    sel = _iota((D, H), 1) == (_iota((D, H), 0) // DH)
    gcol = jnp.sum(jnp.where(sel, g32, 0.0), axis=1, keepdims=True)
    g_s[...] = jnp.broadcast_to(gcol, (D, 128))
    wr_s[...] = jnp.broadcast_to(wr_ref[...].astype(f32).reshape(1, D), (128, D)).T
    m_f[...] = jnp.zeros_like(m_f)
    m_u[...] = jnp.zeros_like(m_u)
    best_s[...] = jnp.concatenate(
        [jnp.full((1, 128), -jnp.inf, f32), jnp.zeros((7, 128), f32)], axis=0)

    x_copy(0).wait()
    ln1(0)

    w_copies[0].wait()
    w_copies[1].wait()
    w4_u[...] = _tou(jnp.concatenate([wq_s[:, 512:D], wk_s[:, 512:D]], axis=1))
    w_copies[2].wait()
    wvt_u[...] = _tou(wv_s[...].T)
    w_copies[3].wait()
    wot_u[...] = _tou(wo_s[...].T)
    for s in range(1, NSEG):
        x_copy(s).wait()

    lane1 = _iota((1, 128), 1)
    bias = jnp.where(_iota((128, 128), 0) <= _iota((128, 128), 1), 0.0, MASKB).astype(f32)

    def proj():
        xn = _tobf(xn_u[...])
        q = _dot(xn, wq_s[:, 0:512])
        k = _dot(xn, wk_s[:, 0:512])
        r4 = _dot(xn, _tobf(w4_u[...]))
        k4 = pltpu.roll(r4, 64, 1)
        for src, last, raw_ref, phi_ref, sc in ((q, r4, qx, pqx, QSCALE), (k, k4, kx, pkx, None)):
            tiles = [src[:, 128 * t:128 * (t + 1)] for t in range(4)] + [last]
            raw = [_pack(t * sc if sc is not None else t) for t in tiles]
            ph = [_pack(_phi(t)) for t in tiles]
            for c in range(NQ):
                t = c // 2
                if c % 2 == 0:
                    raw_ref[c] = raw[t]
                    phi_ref[c] = ph[t]
                else:
                    keep = lane1 >= (QW * c) % 128
                    raw_ref[c] = jnp.where(keep, raw[t], raw[t + 1])
                    phi_ref[c] = jnp.where(keep, ph[t], ph[t + 1])
        vt_u[...] = _pack(_dot(_tobf(wvt_u[...]), _tobf(xnt_u[...])))

    def head_mask(c, i):
        st = (QW * c + DH * i) % 128
        return ((lane1 - st) & 127) < DH

    def stage_a(c, s_ref, mx_ref):
        lms = [jnp.where(head_mask(c, i), jnp.uint32(0xFFFFFFFF), jnp.uint32(0)) for i in range(4)]
        for j in range(4):
            q = qx[c, pl.ds(64 * j, 64), :]
            qm = _tobf(jnp.concatenate([q & lms[i] for i in range(4)], axis=0))
            k = _tobf(kx[c, pl.ds(0, 64 * (j + 1)), :])
            s = _dot_nt(k, qm)
            sd = s[128 * j:] + jnp.concatenate([bias] * 4, axis=1)
            mx = jnp.max(sd, axis=0, keepdims=True)
            off = 128 * (j * (j + 1) // 2)
            if j > 0:
                mx = jnp.maximum(mx, jnp.max(s[:128 * j], axis=0, keepdims=True))
                s_ref[pl.ds(off, 128 * j), :] = s[:128 * j]
            s_ref[pl.ds(off + 128 * j, 128), :] = sd
            mx_ref[j] = mx

    def stage_b(c, s_ref, mx_ref):
        base = QW * c
        mwin = base - base % 16
        moff = base - mwin
        zrow = 72 if moff == 0 else 0
        srow = _iota((8, 128), 0)
        grow = [g_s[pl.ds(base + DH * i, 1), :] for i in range(4)]
        mq = _tobf(m_u[c])
        for j in range(4):
            off = 128 * (j * (j + 1) // 2)
            mem = _dot_nt(mq, _tobf(pqx[c, pl.ds(64 * j, 64), :]))
            accs, rds, rms = [], [], []
            for i in range(4):
                r0 = base + DH * i
                w = r0 - r0 % 16
                o = r0 - w
                vt = vt_u[pl.ds(w // 2, 16), pl.ds(0, 128 * (j + 1))]
                orow = 15 if o < 14 else 0
                vt = jnp.where(_iota(vt.shape, 0) == orow, jnp.uint32(ONES2), vt)
                sc = s_ref[pl.ds(off, 128 * (j + 1)), pl.ds(128 * i, 128)]
                p = jnp.exp2(sc - mx_ref[j, :, pl.ds(128 * i, 128)]).astype(bf)
                acc = _dot(_tobf(vt), p)
                den = acc[2 * orow:2 * orow + 1]
                rds.append((1.0 - grow[i]) / den)
                rms.append(grow[i] / (mem[zrow + i:zrow + i + 1] + 1e-6))
                a0 = o - o % 8
                accs.append(acc[a0:a0 + 24])
            for v in range(9):
                lo_h, hi_h = (8 * v) // DH, (8 * v + 7) // DH

                def piece(h):
                    a = accs[h][8 * (v - (DH * h) // 8):8 * (v - (DH * h) // 8) + 8]
                    return a * rds[h] + mem[moff + 8 * v:moff + 8 * v + 8] * rms[h]
                val = piece(lo_h)
                if hi_h != lo_h:
                    val = jnp.where(srow < DH * hi_h - 8 * v, val, piece(hi_h))
                ot_s[pl.ds(base + 8 * v, 8), pl.ds(128 * j, 128)] = val
        vw = vt_u[pl.ds(mwin // 2, 40), :]
        rr = _iota(vw.shape, 0)
        isz = (rr >= 36) if moff == 0 else (rr < 4)
        vw = jnp.where(isz, jnp.uint32(ONES2), vw)
        upd = _dot(_tobf(vw), _tobf(pkx[c]))
        r80 = _iota((80, 128), 0)
        l80 = (_iota((80, 128), 1) - base) & 127
        hrow = jnp.where((r80 >= zrow) & (r80 < zrow + 8), r80 - zrow, (r80 - moff) // DH)
        keep = (l80 < QW) & (l80 // DH == hrow)
        mnew = m_f[c] + jnp.where(keep, upd, 0.0)
        m_f[c] = mnew
        m_u[c] = _pack(mnew)

    def out_proj():
        return _dot(_tobf(wot_u[...]), ot_s[...].astype(bf))

    def post(s, out_t):
        h = x_s[s].astype(f32) + out_t
        ln = _ln_t(h)
        out_s[s] = (h + ln).astype(bf)
        lnb = ln.astype(bf)
        for t in range(4):
            ln_s[4 * s + t] = _tou(lnb[:, 128 * t:128 * (t + 1)])
        wr = wr_s[...]
        sc = jnp.sum(ln * jnp.concatenate([wr] * 4, axis=1), axis=0, keepdims=True)
        smax = jnp.max(sc, axis=1, keepdims=True)
        pos = (_iota((1, L), 1) + s * L).astype(f32)
        sidx = jnp.min(jnp.where(sc == smax, pos, 1e9), axis=1, keepdims=True)
        old = best_s[...]
        better = smax > old[0:1, 0:1]
        new = jnp.concatenate([jnp.broadcast_to(smax, (1, 128)), jnp.broadcast_to(sidx, (1, 128)),
                               jnp.zeros((6, 128), f32)], axis=0)
        best_s[...] = jnp.where(better, new, old)

    def seg_body(s, carry):
        proj()
        bufs = ((s0, mx0), (s1, mx1))
        stage_a(0, *bufs[0])
        for c in range(1, NQ):
            stage_a(c, *bufs[c % 2])
            stage_b(c - 1, *bufs[(c - 1) % 2])
        stage_b(NQ - 1, *bufs[(NQ - 1) % 2])
        out_t = out_proj()
        ln1(jnp.minimum(s + 1, NSEG - 1))
        post(s, out_t)
        out_copy(s).start()
        return carry

    lax.fori_loop(0, NSEG, seg_body, 0)

    for c in e_copies:
        c.wait()
    best = best_s[...]
    idx = jnp.clip(best[1, 0].astype(i32), 0, S - 1)
    blk = idx // 128
    col = idx - blk * 128
    onehot = ((_iota((16, 128), 1) == col) & (_iota((16, 128), 0) == 0)).astype(bf)
    xs = _dot_nt(onehot, _tobf(ln_s[blk])).astype(bf)
    gate = _dot(xs, wg_s[...])
    up = _dot(xs, wu_s[...])
    act = (gate * jax.nn.sigmoid(gate) * up).astype(bf)
    y = _dot_nt(act, wd_s[...]) * jax.nn.sigmoid(best[0:1, 0:1])
    yt = jnp.broadcast_to(y[0:1], (128, D)).T
    for s in range(NSEG):
        out_copy(s).wait()
    seg = blk // 4
    c0 = pl.multiple_of((blk - seg * 4) * 128, 128)
    cur = out_s[seg, :, pl.ds(c0, 128)].astype(f32)
    hit = _iota((D, 128), 1) == col
    fin_s[...] = (cur + jnp.where(hit, yt, 0.0)).astype(bf)
    fin = cp(fin_s, out_hbm.at[:, pl.ds(pl.multiple_of(blk * 128, 128), 128)], sems.at[15])
    fin.start()
    fin.wait()


@jax.jit
def pallas_sequential_preLN__memory_aug_infini_attn__moe_arch_mod__prompt_kernel(
    A_x, A_wq, A_wk, A_wv, A_wo, A_beta, B_x, B_w_r, B_w_gate, B_w_up, B_w_down,
):
    hbm = pl.BlockSpec(memory_space=pltpu.HBM)
    vm = pltpu.VMEM
    x_t = A_x.reshape(S, D).T
    out_t = pl.pallas_call(
        _kernel,
        out_shape=jax.ShapeDtypeStruct((D, S), bf),
        in_specs=[hbm] * 5 + [pl.BlockSpec(memory_space=pltpu.VMEM)] * 2 + [hbm] * 3,
        out_specs=hbm,
        scratch_shapes=[
            vm((NSEG, D, L), bf), vm((D, D), bf), vm((D, D), bf), vm((D, D), bf), vm((D, D), bf),
            vm((D, F), bf), vm((D, F), bf), vm((D, F), bf),
            vm((D // 2, 128), u32), vm((D // 2, D), u32), vm((D // 2, D), u32),
            vm((L // 2, D), u32), vm((D // 2, L), u32),
            vm((NQ, L // 2, 128), u32), vm((NQ, L // 2, 128), u32),
            vm((NQ, L // 2, 128), u32), vm((NQ, L // 2, 128), u32),
            vm((D // 2, L), u32),
            vm((1280, 512), f32), vm((1280, 512), f32),
            vm((4, 1, 512), f32), vm((4, 1, 512), f32),
            vm((D, L), f32), vm((NQ, 80, 128), f32), vm((NQ, 40, 128), u32),
            vm((D, 128), f32), vm((D, 128), f32), vm((NSEG, D, L), bf), vm((16, D // 2, 128), u32),
            vm((8, 128), f32), vm((D, 128), bf),
            pltpu.SemaphoreType.DMA((16,)),
        ],
        compiler_params=pltpu.CompilerParams(vmem_limit_bytes=100 * 1024 * 1024),
        name="infini_moe",
    )(x_t, A_wq, A_wk, A_wv, A_wo, A_beta, B_w_r, B_w_gate, B_w_up, B_w_down.T)
    return out_t.T.reshape(1, S, D)
```

```python
import jax
import jax.numpy as jnp
from jax import lax
from jax.experimental import pallas as pl
from jax.experimental.pallas import tpu as pltpu

S, D, H, DH = 2048, 576, 32, 18
NSEG, L, F = 4, 512, 4608
NQ = 8
QW = 4 * DH
bf, u32, f32, i32 = jnp.bfloat16, jnp.uint32, jnp.float32, jnp.int32
LOG2E = 1.4426950408889634
QSCALE = DH ** -0.5 * LOG2E
MASKB = -1000000000.0 * LOG2E
EPS = 1e-5
NT = (((1,), (1,)), ((), ()))
ONES2 = 0x3F803F80
DEN_LO, DEN_HI, WV_MAX = 2.0 ** -60, 2.0 ** 60, 2.0 ** 40


def _tobf(x):
    return pltpu.bitcast(x, bf)


def _tou(x):
    return pltpu.bitcast(x, u32)


def _pack(x):
    return pltpu.bitcast(x.astype(bf), u32)


def _dot(a, b):
    return jnp.dot(a, b, preferred_element_type=f32)


def _dot_nt(a, b):
    return lax.dot_general(a, b, NT, preferred_element_type=f32)


def _phi(t):
    return jnp.where(t > 0, t + 1.0, jnp.exp(t))


def _ln_t(x):
    m = jnp.mean(x, axis=0, keepdims=True)
    c = x - m
    v = jnp.mean(c * c, axis=0, keepdims=True)
    return c * lax.rsqrt(v + EPS)


def _iota(shape, dim):
    return lax.broadcasted_iota(i32, shape, dim)


def _al(x, n):
    return x if isinstance(x, int) else pl.multiple_of(x, n)


def _kernel(x_hbm, wq_hbm, wk_hbm, wv_hbm, wo_hbm, beta_ref, wr_ref,
            wg_hbm, wu_hbm, wd_hbm, out_hbm,
            x_s, wq_s, wk_s, wv_s, wo_s, wg_s, wu_s, wd_s,
            w4_u, wvt_u, wot_u, xn_u, xnt_u, qx, kx, pqx, pkx, vt_u,
            p0, p1, outt_s, ot_s, m_f, m_u, g_s, wr_s, out_s, ln_s, best_s, den_s, fin_s,
            sems):
    cp = pltpu.make_async_copy

    def x_copy(s):
        return cp(x_hbm.at[:, pl.ds(_al(s * L, L), L)], x_s.at[s], sems.at[s])

    def out_copy(s):
        return cp(out_s.at[s], out_hbm.at[:, pl.ds(_al(s * L, L), L)], sems.at[11 + s])

    def ln1(s, t):
        c = _al(128 * t, 128)
        xt = _ln_t(x_s[s, :, pl.ds(c, 128)].astype(f32)).astype(bf)
        xnt_u[t] = _tou(xt)
        xn_u[pl.ds(_al(64 * t, 64), 64), :] = _tou(xt.T)

    w_copies = [cp(wq_hbm, wq_s, sems.at[4]), cp(wk_hbm, wk_s, sems.at[5]),
                cp(wv_hbm, wv_s, sems.at[6]), cp(wo_hbm, wo_s, sems.at[7])]
    e_copies = [cp(wg_hbm, wg_s, sems.at[8]), cp(wu_hbm, wu_s, sems.at[9]),
                cp(wd_hbm, wd_s, sems.at[10])]

    w_copies[2].start()
    x_copy(0).start()
    w_copies[0].start()
    w_copies[1].start()

    g32 = jax.nn.sigmoid(beta_ref[...].astype(f32)).reshape(1, H)
    sel = _iota((H, H), 1) == _iota((H, H), 0)
    gcol = jnp.sum(jnp.where(sel, g32, 0.0), axis=1, keepdims=True)
    for h in range(H):
        g_s[h] = jnp.broadcast_to(gcol[h:h + 1], (1, 128))
    wr_s[...] = jnp.broadcast_to(wr_ref[...].astype(f32).reshape(1, D), (128, D)).T
    m_f[...] = jnp.zeros_like(m_f)
    m_u[...] = jnp.zeros_like(m_u)
    outt_s[...] = jnp.zeros_like(outt_s)
    best_s[...] = jnp.concatenate(
        [jnp.full((1, 128), -jnp.inf, f32), jnp.zeros((7, 128), f32)], axis=0)

    w_copies[2].wait()
    wv = wv_s[...]
    wvt_u[...] = _tou(wv.T)
    wv_ok = jnp.max(jnp.abs(wv.astype(f32))) < WV_MAX
    x_copy(0).wait()
    for t in range(4):
        ln1(0, t)
    w_copies[0].wait()
    w_copies[1].wait()
    w_copies[3].start()
    for s in range(1, NSEG):
        x_copy(s).start()
    for c in e_copies:
        c.start()
    w4_u[...] = _tou(jnp.concatenate([wq_s[:, 512:D], wk_s[:, 512:D]], axis=1))

    lane1 = _iota((1, 128), 1)
    causal = _iota((128, 128), 0) <= _iota((128, 128), 1)

    def proj():
        xn = _tobf(xn_u[...])
        q = _dot(xn, wq_s[:, 0:512])
        k = _dot(xn, wk_s[:, 0:512])
        r4 = _dot(xn, _tobf(w4_u[...]))
        k4 = pltpu.roll(r4, 64, 1)
        for src, last, raw_ref, phi_ref, sc in ((q, r4, qx, pqx, QSCALE), (k, k4, kx, pkx, None)):
            tiles = [src[:, 128 * t:128 * (t + 1)] for t in range(4)] + [last]
            raw = [_pack(t * sc if sc is not None else t) for t in tiles]
            ph = [_pack(_phi(t)) for t in tiles]
            for c in range(NQ):
                t = c // 2
                if c % 2 == 0:
                    raw_ref[c] = raw[t]
                    phi_ref[c] = ph[t]
                else:
                    keep = lane1 >= (QW * c) % 128
                    raw_ref[c] = jnp.where(keep, raw[t], raw[t + 1])
                    phi_ref[c] = jnp.where(keep, ph[t], ph[t + 1])
        wvt = _tobf(wvt_u[...])
        for t in range(4):
            vt_u[:, pl.ds(128 * t, 128)] = _pack(_dot(wvt, _tobf(xnt_u[t])))

    def scores(k, par, j):
        c = 2 * k + par
        lms = []
        for i in range(4):
            st = (2 * QW * k + QW * par + DH * i) % 128
            lms.append(jnp.where(((lane1 - st) & 127) < DH, jnp.uint32(0xFFFFFFFF), jnp.uint32(0)))
        q = qx[c, pl.ds(64 * j, 64), :]
        qm = _tobf(jnp.concatenate([q & lms[i] for i in range(4)], axis=0))
        kk = _tobf(kx[c, pl.ds(0, 64 * (j + 1)), :])
        return _dot_nt(kk, qm)

    def stage_a(k, par, j, p_ref):
        p = jnp.exp2(scores(k, par, j))
        pd = jnp.concatenate([jnp.where(causal, p[128 * j:, 128 * i:128 * (i + 1)], 0.0)
                              for i in range(4)], axis=1)
        off = 64 * (j * (j + 1) // 2)
        if j > 0:
            p_ref[pl.ds(off, 64 * j), :] = _pack(p[:128 * j])
        p_ref[pl.ds(off + 64 * j, 64), :] = _pack(pd)

    def stage_a_safe(k, par, j, p_ref):
        s = scores(k, par, j)
        bias = jnp.where(causal, 0.0, MASKB).astype(f32)
        sd = s[128 * j:] + jnp.concatenate([bias] * 4, axis=1)
        s = sd if j == 0 else jnp.concatenate([s[:128 * j], sd], axis=0)
        p = jnp.exp2(s - jnp.max(s, axis=0, keepdims=True))
        p_ref[pl.ds(64 * (j * (j + 1) // 2), 64 * (j + 1)), :] = _pack(p)

    def stage_b(mslot, k, par, j, p_ref):
        c = 2 * k + par
        base = QW * par
        mwin = base - base % 16
        moff = base - mwin
        zrow = 72 if moff == 0 else 0
        srow = _iota((8, 128), 0)
        grow = [g_s[4 * c + i] for i in range(4)]
        off = 64 * (j * (j + 1) // 2)
        mem = _dot_nt(_tobf(m_u[mslot, c]), _tobf(pqx[c, pl.ds(64 * j, 64), :]))
        accs, rds, rms = [], [], []
        dlo, dhi = den_s[0:1], den_s[1:2]
        for i in range(4):
            r0 = base + DH * i
            w = r0 - r0 % 16
            o = r0 - w
            vt = vt_u[pl.ds(_al(QW * k + w // 2, 8), 16), pl.ds(0, 128 * (j + 1))]
            orow = 15 if o < 14 else 0
            vt = jnp.where(_iota(vt.shape, 0) == orow, jnp.uint32(ONES2), vt)
            p = _tobf(p_ref[pl.ds(off, 64 * (j + 1)), pl.ds(128 * i, 128)])
            acc = _dot(_tobf(vt), p)
            den = acc[2 * orow:2 * orow + 1]
            dlo, dhi = jnp.minimum(dlo, den), jnp.maximum(dhi, den)
            rds.append((1.0 - grow[i]) / den)
            rms.append(grow[i] / (mem[zrow + i:zrow + i + 1] + 1e-6))
            a0 = o - o % 8
            accs.append(acc[a0:a0 + 24])
        den_s[0:1] = dlo
        den_s[1:2] = dhi
        for v in range(9):
            lo_h, hi_h = (8 * v) // DH, (8 * v + 7) // DH

            def piece(h):
                a = accs[h][8 * (v - (DH * h) // 8):8 * (v - (DH * h) // 8) + 8]
                return a * rds[h] + mem[moff + 8 * v:moff + 8 * v + 8] * rms[h]
            val = piece(lo_h)
            if hi_h != lo_h:
                val = jnp.where(srow < DH * hi_h - 8 * v, val, piece(hi_h))
            ot_s[pl.ds(_al(2 * QW * k + base + 8 * v, 8), 8), pl.ds(128 * j, 128)] = val

    def mem_update(mslot, k, par):
        c = 2 * k + par
        base = QW * par
        mwin = base - base % 16
        moff = base - mwin
        zrow = 72 if moff == 0 else 0
        vw = vt_u[pl.ds(_al(QW * k + mwin // 2, 8), 40), :]
        rr = _iota(vw.shape, 0)
        isz = (rr >= 36) if moff == 0 else (rr < 4)
        vw = jnp.where(isz, jnp.uint32(ONES2), vw)
        upd = _dot(_tobf(vw), _tobf(pkx[c]))
        r80 = _iota((80, 128), 0)
        l80 = (_iota((80, 128), 1) - (2 * QW * k + base)) & 127
        hrow = jnp.where((r80 >= zrow) & (r80 < zrow + 8), r80 - zrow, (r80 - moff) // DH)
        keep = (l80 >= DH * hrow) & (l80 < DH * hrow + DH) & (hrow < 4) & (hrow >= 0)
        mnew = m_f[c] + jnp.where(keep, upd, 0.0)
        m_f[c] = mnew
        m_u[1 - mslot, c] = _pack(mnew)

    pb = (p0, p1)

    def step(mslot, a, b):
        for j in range(4):
            if a is not None:
                stage_a(a[0], a[1], j, pb[a[1]])
            if b is not None:
                stage_b(mslot, b[0], b[1], j, pb[b[1]])
        if b is not None:
            mem_update(mslot, b[0], b[1])

    def out_proj(t):
        o = ot_s[:, pl.ds(128 * t, 128)].astype(bf)
        outt_s[:, pl.ds(128 * t, 128)] = _dot(_tobf(wot_u[...]), o)

    def post(s, t, live):
        c = 128 * t
        h = x_s[s, :, pl.ds(c, 128)].astype(f32) + outt_s[:, pl.ds(c, 128)]
        ln = _ln_t(h)
        out_s[s, :, pl.ds(c, 128)] = (h + ln).astype(bf)
        ln_s[4 * s + t] = _pack(ln)
        sc = jnp.sum(ln * wr_s[...], axis=0, keepdims=True)
        smax = jnp.max(sc, axis=1, keepdims=True)
        pos = (lane1 + (s * L + c)).astype(f32)
        sidx = jnp.min(jnp.where(sc == smax, pos, 1e9), axis=1, keepdims=True)
        old = best_s[...]
        better = jnp.logical_and(smax > old[0:1, 0:1], live)
        new = jnp.concatenate([jnp.broadcast_to(smax, (1, 128)), jnp.broadcast_to(sidx, (1, 128)),
                               jnp.zeros((6, 128), f32)], axis=0)
        best_s[...] = jnp.where(better, new, old)

    def seg_body(s, carry):
        mslot = s % 2
        nxt = jnp.minimum(s + 1, NSEG - 1)
        den_s[...] = jnp.ones_like(den_s)
        post(jnp.maximum(s - 1, 0), 3, s > 0)
        proj()
        step(mslot, (0, 0), None)

        @pl.when(s == 0)
        def _():
            w_copies[3].wait()
            wot_u[...] = _tou(wo_s[...].T)

        @pl.when(s < NSEG - 1)
        def _():
            x_copy(nxt).wait()

        def pair(k, carry):
            step(mslot, (k, 1), (k, 0))
            step(mslot, (k + 1, 0), (k, 1))
            ln1(nxt, k)
            return carry
        lax.fori_loop(0, NQ // 2 - 1, pair, 0)

        @pl.when(s > 0)
        def _():
            out_copy(s - 1).start()

        step(mslot, (3, 1), (3, 0))
        step(mslot, None, (3, 1))
        ln1(nxt, 3)

        dl = den_s[...]
        safe = jnp.logical_and(jnp.min(dl[0:1]) >= DEN_LO, jnp.max(dl[1:2]) <= DEN_HI)
        safe = jnp.logical_and(safe, wv_ok)

        @pl.when(jnp.logical_not(safe))
        def _():
            def redo(k, carry):
                for par in range(2):
                    for j in range(4):
                        stage_a_safe(k, par, j, p0)
                        stage_b(mslot, k, par, j, p0)
                return carry
            lax.fori_loop(0, NQ // 2, redo, 0)

        for t in range(4):
            out_proj(t)
            if t < 3:
                post(s, t, True)
        return carry

    lax.fori_loop(0, NSEG, seg_body, 0)
    post(NSEG - 1, 3, True)
    out_copy(NSEG - 1).start()

    for c in e_copies:
        c.wait()
    best = best_s[...]
    idx = jnp.clip(best[1, 0].astype(i32), 0, S - 1)
    blk = idx // 128
    col = idx - blk * 128
    onehot = ((_iota((16, 128), 1) == col) & (_iota((16, 128), 0) == 0)).astype(bf)
    xs = _dot_nt(onehot, _tobf(ln_s[blk])).astype(bf)
    gate = _dot(xs, wg_s[...])
    up = _dot(xs, wu_s[...])
    act = (gate * jax.nn.sigmoid(gate) * up).astype(bf)
    y = _dot_nt(act, wd_s[...]) * jax.nn.sigmoid(best[0:1, 0:1])
    yt = jnp.broadcast_to(y[0:1], (128, D)).T
    for s in range(NSEG):
        out_copy(s).wait()
    seg = blk // 4
    c0 = pl.multiple_of((blk - seg * 4) * 128, 128)
    cur = out_s[seg, :, pl.ds(c0, 128)].astype(f32)
    hit = _iota((D, 128), 1) == col
    fin_s[...] = (cur + jnp.where(hit, yt, 0.0)).astype(bf)
    fin = cp(fin_s, out_hbm.at[:, pl.ds(pl.multiple_of(blk * 128, 128), 128)], sems.at[15])
    fin.start()
    fin.wait()


@jax.jit
def pallas_sequential_preLN__memory_aug_infini_attn__moe_arch_mod__prompt_kernel(
    A_x, A_wq, A_wk, A_wv, A_wo, A_beta, B_x, B_w_r, B_w_gate, B_w_up, B_w_down,
):
    hbm = pl.BlockSpec(memory_space=pltpu.HBM)
    vm = pltpu.VMEM
    x_t = A_x.reshape(S, D).T
    out_t = pl.pallas_call(
        _kernel,
        out_shape=jax.ShapeDtypeStruct((D, S), bf),
        in_specs=[hbm] * 5 + [pl.BlockSpec(memory_space=pltpu.VMEM)] * 2 + [hbm] * 3,
        out_specs=hbm,
        scratch_shapes=[
            vm((NSEG, D, L), bf), vm((D, D), bf), vm((D, D), bf), vm((D, D), bf), vm((D, D), bf),
            vm((D, F), bf), vm((D, F), bf), vm((D, F), bf),
            vm((D // 2, 128), u32), vm((D // 2, D), u32), vm((D // 2, D), u32),
            vm((L // 2, D), u32), vm((4, D // 2, 128), u32),
            vm((NQ, L // 2, 128), u32), vm((NQ, L // 2, 128), u32),
            vm((NQ, L // 2, 128), u32), vm((NQ, L // 2, 128), u32),
            vm((D // 2, L), u32),
            vm((640, 512), u32), vm((640, 512), u32), vm((D, L), f32),
            vm((D, L), f32), vm((NQ, 80, 128), f32), vm((2, NQ, 40, 128), u32),
            vm((H, 1, 128), f32), vm((D, 128), f32), vm((NSEG, D, L), bf),
            vm((16, D // 2, 128), u32),
            vm((8, 128), f32), vm((8, 128), f32), vm((D, 128), bf),
            pltpu.SemaphoreType.DMA((16,)),
        ],
        compiler_params=pltpu.CompilerParams(vmem_limit_bytes=100 * 1024 * 1024),
        name="infini_moe",
    )(x_t, A_wq, A_wk, A_wv, A_wo, A_beta, B_w_r, B_w_gate, B_w_up, B_w_down.T)
    return out_t.T.reshape(1, S, D)
```

```python
import jax
import jax.numpy as jnp
from jax import lax
from jax.experimental import pallas as pl
from jax.experimental.pallas import tpu as pltpu

S, D, H, DH = 2048, 576, 32, 18
NSEG, L, F = 4, 512, 4608
DP = 640
NQ = 8
QW = 4 * DH
bf, u32, f32, i32 = jnp.bfloat16, jnp.uint32, jnp.float32, jnp.int32
LOG2E = 1.4426950408889634
QSCALE = DH ** -0.5 * LOG2E
MASKB = -1000000000.0 * LOG2E
EPS = 1e-5
NT = (((1,), (1,)), ((), ()))
ONES2 = 0x3F803F80
DEN_LO, DEN_HI, WV_MAX = 2.0 ** -60, 2.0 ** 60, 2.0 ** 40


def _tobf(x):
    return pltpu.bitcast(x, bf)


def _tou(x):
    return pltpu.bitcast(x, u32)


def _pack(x):
    return pltpu.bitcast(x.astype(bf), u32)


def _dot(a, b):
    return jnp.dot(a, b, preferred_element_type=f32)


def _dot_nt(a, b):
    return lax.dot_general(a, b, NT, preferred_element_type=f32)


def _phi(t):
    return jnp.where(t > 0, t + 1.0, jnp.exp(t))


def _rowsum(parts):
    acc = [jnp.sum(p.reshape(p.shape[0] // 8, 8, 128), axis=0) for p in parts]
    while len(acc) > 1:
        acc = [acc[i] + acc[i + 1] for i in range(0, len(acc), 2)]
    return jnp.sum(acc[0], axis=0, keepdims=True)


def _ln_stats(rows, x0, w=None):
    d = [rows(144 * g, 144 * (g + 1)) - x0 for g in range(4)]
    m1 = _rowsum(d) * (1.0 / D)
    m2 = _rowsum([v * v for v in d]) * (1.0 / D)
    var = jnp.maximum(m2 - m1 * m1, 0.0)
    rstd = lax.rsqrt(var + EPS)
    if w is None:
        return x0 + m1, rstd
    dw = _rowsum([d[g] * w[0][144 * g:144 * (g + 1)] for g in range(4)])
    return x0 + m1, rstd, (dw - m1 * w[1]) * rstd


def _hi_lo(v):
    hi = v.astype(bf).astype(f32)
    return hi, (v - hi).astype(bf).astype(f32)


def _iota(shape, dim):
    return lax.broadcasted_iota(i32, shape, dim)


def _al(x, n):
    return x if isinstance(x, int) else pl.multiple_of(x, n)


def _kernel(x_hbm, wq_hbm, wk_hbm, wv_hbm, wo_hbm, beta_ref, wr_ref,
            wg_hbm, wu_hbm, wd_hbm, out_hbm,
            x_s, wq_s, wk_s, wv_s, wo_s, wg_s, wu_s, wd_s,
            w4_u, wvt_u, wot_u, xn_u, rs_s, rc_s, qx, kx, pqx, pkx, vt_u,
            p0, p1, h_s, ot_s, m_f, m_u, g_s, wr_s, wrs_s, out_s, st_s, best_s, den_s, fin_s,
            sems):
    cp = pltpu.make_async_copy

    def x_copy(s):
        return cp(x_hbm.at[:, pl.ds(_al(s * L, L), L)], x_s.at[s, pl.ds(0, D), :], sems.at[s])

    def out_copy(s):
        return cp(out_s.at[s], out_hbm.at[:, pl.ds(_al(s * L, L), L)], sems.at[11 + s])

    def prep(s, t):
        c = 128 * t
        mean, rstd = _ln_stats(lambda a, b: x_s[s, a:b, pl.ds(c, 128)].astype(f32),
                               x_s[s, 0:16, pl.ds(c, 128)].astype(f32)[0:1])
        mh, ml = _hi_lo(mean)
        r16 = _iota((16, 128), 0)
        x_s[s, D:D + 16, pl.ds(c, 128)] = jnp.where(
            r16 < 2, mh, jnp.where(r16 == 2, ml, 0.0)).astype(bf)
        rs_s[t, 0:1] = rstd
        rc_s[t] = jnp.broadcast_to(rstd, (128, 128)).T
        xn_u[pl.ds(64 * t, 64), :] = _tou(x_s[s, :, pl.ds(c, 128)].T)

    def augment(w_ref):
        ones = jnp.ones((16, D), bf)
        hi, lo = _hi_lo(_dot(ones, w_ref[0:D, :])[0:1])
        r16 = _iota((16, D), 0)
        w_ref[D:D + 16, :] = jnp.where((r16 == 0) | (r16 == 2), -hi,
                                       jnp.where(r16 == 1, -lo, 0.0)).astype(bf)

    top = pl.ds(0, D)
    w_copies = [cp(wq_hbm, wq_s.at[top, :], sems.at[4]), cp(wk_hbm, wk_s.at[top, :], sems.at[5]),
                cp(wv_hbm, wv_s.at[top, :], sems.at[6]), cp(wo_hbm, wo_s, sems.at[7])]
    e_copies = [cp(wg_hbm, wg_s, sems.at[8]), cp(wu_hbm, wu_s, sems.at[9]),
                cp(wd_hbm, wd_s, sems.at[10])]

    w_copies[2].start()
    x_copy(0).start()
    w_copies[3].start()
    w_copies[0].start()
    w_copies[1].start()
    x_copy(1).start()

    g32 = jax.nn.sigmoid(beta_ref[...].astype(f32)).reshape(1, H)
    sel = _iota((H, H), 1) == _iota((H, H), 0)
    gcol = jnp.sum(jnp.where(sel, g32, 0.0), axis=1, keepdims=True)
    for h in range(H):
        g_s[h] = jnp.broadcast_to(gcol[h:h + 1], (1, 128))
    wr_s[...] = jnp.broadcast_to(wr_ref[...].astype(f32).reshape(1, D), (128, D)).T
    m_f[...] = jnp.zeros_like(m_f)
    m_u[...] = jnp.zeros_like(m_u)
    wrs_s[...] = jnp.broadcast_to(jnp.sum(wr_s[...], axis=0, keepdims=True), (8, 128))
    h_s[3] = jnp.zeros((D, 128), f32)
    st_s[3] = jnp.zeros((8, 128), f32)

    for w_ref in (wq_s, wk_s, wv_s):
        w_ref[D + 16:DP, :] = jnp.zeros((DP - D - 16, D), bf)
    for s in range(NSEG):
        x_s[s, D + 16:DP, :] = jnp.zeros((DP - D - 16, L), bf)

    w_copies[2].wait()
    augment(wv_s)
    wvt_u[...] = _tou(wv_s[...].T)
    wv_ok = jnp.max(jnp.abs(wv_s[0:D, :].astype(f32))) < WV_MAX
    w_copies[3].wait()
    wot_u[...] = _tou(wo_s[...].T)
    w_copies[0].wait()
    augment(wq_s)
    w_copies[1].wait()
    augment(wk_s)
    x_copy(0).wait()
    for s in range(2, NSEG):
        x_copy(s).start()
    for c in e_copies:
        c.start()
    w4_u[...] = _tou(jnp.concatenate([wq_s[:, 512:D], wk_s[:, 512:D]], axis=1))

    lane1 = _iota((1, 128), 1)
    causal = _iota((128, 128), 0) <= _iota((128, 128), 1)

    def proj(s, t):
        rows = pl.ds(64 * t, 64)
        xn = _tobf(xn_u[rows, :])
        rc = rc_s[t]
        rc4 = jnp.concatenate([rc] * 4, axis=1)
        q = _dot(xn, wq_s[:, 0:512]) * rc4
        k = _dot(xn, wk_s[:, 0:512]) * rc4
        r4 = _dot(xn, _tobf(w4_u[...])) * rc
        k4 = pltpu.roll(r4, 64, 1)
        for src, last, raw_ref, phi_ref, sc in ((q, r4, qx, pqx, QSCALE), (k, k4, kx, pkx, None)):
            tiles = [src[:, 128 * i:128 * (i + 1)] for i in range(4)] + [last]
            raw = [_pack(v * sc if sc is not None else v) for v in tiles]
            ph = [_pack(_phi(v)) for v in tiles]
            for c in range(NQ):
                i = c // 2
                if c % 2 == 0:
                    raw_ref[c, rows, :] = raw[i]
                    phi_ref[c, rows, :] = ph[i]
                else:
                    keep = lane1 >= (QW * c) % 128
                    raw_ref[c, rows, :] = jnp.where(keep, raw[i], raw[i + 1])
                    phi_ref[c, rows, :] = jnp.where(keep, ph[i], ph[i + 1])

    def proj_v(s, t):
        vt = _dot(_tobf(wvt_u[...]), x_s[s, :, pl.ds(128 * t, 128)]) * rs_s[t, 0:1]
        vt_u[:, pl.ds(128 * t, 128)] = _pack(vt)

    def scores(k, par, j):
        c = 2 * k + par
        lms = []
        for i in range(4):
            st = (2 * QW * k + QW * par + DH * i) % 128
            lms.append(jnp.where(((lane1 - st) & 127) < DH, jnp.uint32(0xFFFFFFFF), jnp.uint32(0)))
        q = qx[c, pl.ds(64 * j, 64), :]
        qm = _tobf(jnp.concatenate([q & lms[i] for i in range(4)], axis=0))
        kk = _tobf(kx[c, pl.ds(0, 64 * (j + 1)), :])
        return _dot_nt(kk, qm)

    def stage_a(k, par, j, p_ref):
        p = jnp.exp2(scores(k, par, j))
        pd = jnp.concatenate([jnp.where(causal, p[128 * j:, 128 * i:128 * (i + 1)], 0.0)
                              for i in range(4)], axis=1)
        off = 64 * (j * (j + 1) // 2)
        if j > 0:
            p_ref[pl.ds(off, 64 * j), :] = _pack(p[:128 * j])
        p_ref[pl.ds(off + 64 * j, 64), :] = _pack(pd)

    def stage_a_safe(k, par, j, p_ref):
        s = scores(k, par, j)
        bias = jnp.where(causal, 0.0, MASKB).astype(f32)
        sd = s[128 * j:] + jnp.concatenate([bias] * 4, axis=1)
        s = sd if j == 0 else jnp.concatenate([s[:128 * j], sd], axis=0)
        p = jnp.exp2(s - jnp.max(s, axis=0, keepdims=True))
        p_ref[pl.ds(64 * (j * (j + 1) // 2), 64 * (j + 1)), :] = _pack(p)

    def stage_b(mslot, k, par, j, p_ref):
        c = 2 * k + par
        base = QW * par
        mwin = base - base % 16
        moff = base - mwin
        zrow = 72 if moff == 0 else 0
        srow = _iota((8, 128), 0)
        grow = [g_s[4 * c + i] for i in range(4)]
        off = 64 * (j * (j + 1) // 2)
        mem = _dot_nt(_tobf(m_u[mslot, c]), _tobf(pqx[c, pl.ds(64 * j, 64), :]))
        accs, rds, rms = [], [], []
        dlo, dhi = den_s[0:1], den_s[1:2]
        for i in range(4):
            r0 = base + DH * i
            w = r0 - r0 % 16
            o = r0 - w
            vt = vt_u[pl.ds(_al(QW * k + w // 2, 8), 16), pl.ds(0, 128 * (j + 1))]
            orow = 15 if o < 14 else 0
            vt = jnp.where(_iota(vt.shape, 0) == orow, jnp.uint32(ONES2), vt)
            p = _tobf(p_ref[pl.ds(off, 64 * (j + 1)), pl.ds(128 * i, 128)])
            acc = _dot(_tobf(vt), p)
            den = acc[2 * orow:2 * orow + 1]
            dlo, dhi = jnp.minimum(dlo, den), jnp.maximum(dhi, den)
            rds.append((1.0 - grow[i]) / den)
            rms.append(grow[i] / (mem[zrow + i:zrow + i + 1] + 1e-6))
            a0 = o - o % 8
            accs.append(acc[a0:a0 + 24])
        den_s[0:1] = dlo
        den_s[1:2] = dhi
        for v in range(9):
            lo_h, hi_h = (8 * v) // DH, (8 * v + 7) // DH

            def piece(h):
                a = accs[h][8 * (v - (DH * h) // 8):8 * (v - (DH * h) // 8) + 8]
                return a * rds[h] + mem[moff + 8 * v:moff + 8 * v + 8] * rms[h]
            val = piece(lo_h)
            if hi_h != lo_h:
                val = jnp.where(srow < DH * hi_h - 8 * v, val, piece(hi_h))
            ot_s[pl.ds(_al(2 * QW * k + base + 8 * v, 8), 8), pl.ds(128 * j, 128)] = val

    def mem_update(mslot, k, par):
        c = 2 * k + par
        base = QW * par
        mwin = base - base % 16
        moff = base - mwin
        zrow = 72 if moff == 0 else 0
        vw = vt_u[pl.ds(_al(QW * k + mwin // 2, 8), 40), :]
        rr = _iota(vw.shape, 0)
        isz = (rr >= 36) if moff == 0 else (rr < 4)
        vw = jnp.where(isz, jnp.uint32(ONES2), vw)
        upd = _dot(_tobf(vw), _tobf(pkx[c]))
        r80 = _iota((80, 128), 0)
        l80 = (_iota((80, 128), 1) - (2 * QW * k + base)) & 127
        hrow = jnp.where((r80 >= zrow) & (r80 < zrow + 8), r80 - zrow, (r80 - moff) // DH)
        keep = (l80 >= DH * hrow) & (l80 < DH * hrow + DH) & (hrow < 4) & (hrow >= 0)
        mnew = m_f[c] + jnp.where(keep, upd, 0.0)
        m_f[c] = mnew
        m_u[1 - mslot, c] = _pack(mnew)

    pb = (p0, p1)

    def step(mslot, a, b):
        for j in range(4):
            if b is not None:
                stage_b(mslot, b[0], b[1], j, pb[b[1]])
                if j == 3:
                    mem_update(mslot, b[0], b[1])
            if a is not None:
                stage_a(a[0], a[1], j, pb[a[1]])

    def out_proj(s, t):
        c = 128 * t
        o = ot_s[:, pl.ds(c, 128)].astype(bf)
        h = x_s[s, 0:D, pl.ds(c, 128)].astype(f32) + _dot(_tobf(wot_u[...]), o)
        h_s[4 * s + t] = h
        mean, rstd, sc = _ln_stats(lambda a, b: h[a:b], h[0:1], (wr_s[...], wrs_s[0:1]))
        st_s[4 * s + t, 0:1] = mean
        st_s[4 * s + t, 1:2] = rstd
        smax = jnp.max(sc, axis=1, keepdims=True)
        pos = (lane1 + (s * L + c)).astype(f32)
        sidx = jnp.min(jnp.where(sc == smax, pos, 1e9), axis=1, keepdims=True)
        new = jnp.concatenate([jnp.broadcast_to(smax, (1, 128)), jnp.broadcast_to(sidx, (1, 128)),
                               jnp.zeros((6, 128), f32)], axis=0)
        if t == 0:
            best_s[s] = new
        else:
            old = best_s[s]
            best_s[s] = jnp.where(smax > old[0:1, 0:1], new, old)

    def post(s, t):
        rstd = st_s[4 * s + t, 1:2]
        a = 1.0 + rstd
        b = st_s[4 * s + t, 0:1] * rstd
        out_s[s, :, pl.ds(128 * t, 128)] = (h_s[4 * s + t] * a - b).astype(bf)

    def seg_body(s, carry):
        mslot = s % 2

        @pl.when(s > 0)
        def _():
            x_copy(s).wait()

        @pl.when(s > 1)
        def _():
            out_copy(s - 2).start()

        def finish():
            for t in range(4):
                out_proj(s, t)
                if t < 3:
                    post(s, t)

        den_s[...] = jnp.ones_like(den_s)
        post(jnp.maximum(s - 1, 0), 3)
        for t in range(4):
            prep(s, t)
        for t in range(4):
            proj_v(s, t)
        for t in range(4):
            proj(s, t)
        step(mslot, (0, 0), None)
        for k in range(NQ // 2):
            step(mslot, (k, 1), (k, 0))
            step(mslot, (k + 1, 0) if k + 1 < NQ // 2 else None, (k, 1))
        dl = den_s[...]
        safe = jnp.logical_and(jnp.min(dl[0:1]) >= DEN_LO, jnp.max(dl[1:2]) <= DEN_HI)
        safe = jnp.logical_and(safe, wv_ok)
        finish()

        @pl.when(jnp.logical_not(safe))
        def _():
            def redo(k, carry):
                for par in range(2):
                    for j in range(4):
                        stage_a_safe(k, par, j, pb[par])
                        stage_b(mslot, k, par, j, pb[par])
                return carry
            lax.fori_loop(0, NQ // 2, redo, 0)
            finish()
        return carry

    lax.fori_loop(0, NSEG, seg_body, 0)
    out_copy(NSEG - 2).start()
    post(NSEG - 1, 3)
    out_copy(NSEG - 1).start()

    for c in e_copies:
        c.wait()
    best = best_s[0]
    for s in range(1, NSEG):
        cand = best_s[s]
        best = jnp.where(cand[0:1, 0:1] > best[0:1, 0:1], cand, best)
    idx = jnp.clip(best[1, 0].astype(i32), 0, S - 1)
    blk = idx // 128
    col = idx - blk * 128
    onehot = ((_iota((16, 128), 1) == col) & (_iota((16, 128), 0) == 0)).astype(bf)
    ln = ((h_s[blk] - st_s[blk, 0:1]) * st_s[blk, 1:2]).astype(bf)
    xs = _dot_nt(onehot, ln).astype(bf)
    gate = _dot(xs, wg_s[...])
    up = _dot(xs, wu_s[...])
    act = (gate * jax.nn.sigmoid(gate) * up).astype(bf)
    y = _dot_nt(act, wd_s[...]) * jax.nn.sigmoid(best[0:1, 0:1])
    yt = jnp.broadcast_to(y[0:1], (128, D)).T
    for s in range(NSEG):
        out_copy(s).wait()
    seg = blk // 4
    c0 = pl.multiple_of((blk - seg * 4) * 128, 128)
    cur = out_s[seg, :, pl.ds(c0, 128)].astype(f32)
    hit = _iota((D, 128), 1) == col
    fin_s[...] = (cur + jnp.where(hit, yt, 0.0)).astype(bf)
    fin = cp(fin_s, out_hbm.at[:, pl.ds(pl.multiple_of(blk * 128, 128), 128)], sems.at[15])
    fin.start()
    fin.wait()


@jax.jit
def pallas_sequential_preLN__memory_aug_infini_attn__moe_arch_mod__prompt_kernel(
    A_x, A_wq, A_wk, A_wv, A_wo, A_beta, B_x, B_w_r, B_w_gate, B_w_up, B_w_down,
):
    hbm = pl.BlockSpec(memory_space=pltpu.HBM)
    vm = pltpu.VMEM
    x_t = A_x.reshape(S, D).T
    out_t = pl.pallas_call(
        _kernel,
        out_shape=jax.ShapeDtypeStruct((D, S), bf),
        in_specs=[hbm] * 5 + [pl.BlockSpec(memory_space=pltpu.VMEM)] * 2 + [hbm] * 3,
        out_specs=hbm,
        scratch_shapes=[
            vm((NSEG, DP, L), bf), vm((DP, D), bf), vm((DP, D), bf), vm((DP, D), bf), vm((D, D), bf),
            vm((D, F), bf), vm((D, F), bf), vm((D, F), bf),
            vm((DP // 2, 128), u32), vm((D // 2, DP), u32), vm((D // 2, D), u32),
            vm((L // 2, DP), u32), vm((4, 8, 128), f32), vm((4, 128, 128), f32),
            vm((NQ, L // 2, 128), u32), vm((NQ, L // 2, 128), u32),
            vm((NQ, L // 2, 128), u32), vm((NQ, L // 2, 128), u32),
            vm((D // 2, L), u32),
            vm((640, 512), u32), vm((640, 512), u32), vm((16, D, 128), f32),
            vm((D, L), f32), vm((NQ, 80, 128), f32), vm((2, NQ, 40, 128), u32),
            vm((H, 1, 128), f32), vm((D, 128), f32), vm((8, 128), f32), vm((NSEG, D, L), bf),
            vm((16, 8, 128), f32),
            vm((NSEG, 8, 128), f32), vm((8, 128), f32), vm((D, 128), bf),
            pltpu.SemaphoreType.DMA((16,)),
        ],
        compiler_params=pltpu.CompilerParams(vmem_limit_bytes=100 * 1024 * 1024),
        name="infini_moe",
    )(x_t, A_wq, A_wk, A_wv, A_wo, A_beta, B_w_r, B_w_gate, B_w_up, B_w_down.T)
    return out_t.T.reshape(1, S, D)
```

```python
import jax
import jax.numpy as jnp
from jax import lax
from jax.experimental import pallas as pl
from jax.experimental.pallas import tpu as pltpu

S, D, H, DH = 2048, 576, 32, 18
NSEG, L, F = 4, 512, 4608
DP = 640
NQ = 8
QW = 4 * DH
bf, u32, f32, i32 = jnp.bfloat16, jnp.uint32, jnp.float32, jnp.int32
LOG2E = 1.4426950408889634
QSCALE = DH ** -0.5 * LOG2E
MASKB = -1000000000.0 * LOG2E
EPS = 1e-5
NT = (((1,), (1,)), ((), ()))
ONES2 = 0x3F803F80
DEN_LO, DEN_HI, WV_MAX = 2.0 ** -60, 2.0 ** 60, 2.0 ** 40


def _tobf(x):
    return pltpu.bitcast(x, bf)


def _tou(x):
    return pltpu.bitcast(x, u32)


def _pack(x):
    return pltpu.bitcast(x.astype(bf), u32)


def _dot(a, b):
    return jnp.dot(a, b, preferred_element_type=f32)


def _dot_nt(a, b):
    return lax.dot_general(a, b, NT, preferred_element_type=f32)


def _phi(t):
    return jnp.where(t > 0, t + 1.0, jnp.exp(t))


def _rowsum(parts):
    acc = [jnp.sum(p.reshape(p.shape[0] // 8, 8, 128), axis=0) for p in parts]
    while len(acc) > 1:
        acc = [acc[i] + acc[i + 1] for i in range(0, len(acc), 2)]
    return jnp.sum(acc[0], axis=0, keepdims=True)


def _ln_stats(rows, x0, w=None):
    d = [rows(144 * g, 144 * (g + 1)) - x0 for g in range(4)]
    m1 = _rowsum(d) * (1.0 / D)
    m2 = _rowsum([v * v for v in d]) * (1.0 / D)
    var = jnp.maximum(m2 - m1 * m1, 0.0)
    rstd = lax.rsqrt(var + EPS)
    if w is None:
        return x0 + m1, rstd
    dw = _rowsum([d[g] * w[0][144 * g:144 * (g + 1)] for g in range(4)])
    return x0 + m1, rstd, (dw - m1 * w[1]) * rstd


def _hi_lo(v):
    hi = v.astype(bf).astype(f32)
    return hi, (v - hi).astype(bf).astype(f32)


def _iota(shape, dim):
    return lax.broadcasted_iota(i32, shape, dim)


def _al(x, n):
    return x if isinstance(x, int) else pl.multiple_of(x, n)


def _kernel(x_hbm, wq_hbm, wk_hbm, wv_hbm, wo_hbm, beta_ref, wr_ref,
            wg_hbm, wu_hbm, wd_hbm, out_hbm,
            x_s, wq_s, wk_s, wv_s, wo_s, wg_s, wu_s, wd_s,
            w4_u, wvt_u, wot_u, xn_u, rs_s, rc_s, qx, kx, pqx, pkx, vt_u,
            p0, p1, h_s, ot_s, m_f, m_u, g_s, wr_s, wrs_s, out_s, st_s, best_s, den_s, fin_s,
            sems):
    cp = pltpu.make_async_copy

    def x_copy(s):
        return cp(x_hbm.at[:, pl.ds(_al(s * L, L), L)], x_s.at[s, pl.ds(0, D), :], sems.at[s])

    def out_copy(s):
        return cp(out_s.at[s], out_hbm.at[:, pl.ds(_al(s * L, L), L)], sems.at[11 + s])

    def prep(s, t):
        c = 128 * t
        mean, rstd = _ln_stats(lambda a, b: x_s[s, a:b, pl.ds(c, 128)].astype(f32),
                               x_s[s, 0:16, pl.ds(c, 128)].astype(f32)[0:1])
        mh, ml = _hi_lo(mean)
        r16 = _iota((16, 128), 0)
        x_s[s, D:D + 16, pl.ds(c, 128)] = jnp.where(
            r16 < 2, mh, jnp.where(r16 == 2, ml, 0.0)).astype(bf)
        rs_s[t, 0:1] = rstd
        rc_s[t] = jnp.broadcast_to(rstd, (128, 128)).T
        xn_u[pl.ds(64 * t, 64), :] = _tou(x_s[s, :, pl.ds(c, 128)].T)

    def augment(w_ref):
        ones = jnp.ones((16, D), bf)
        hi, lo = _hi_lo(_dot(ones, w_ref[0:D, :])[0:1])
        r16 = _iota((16, D), 0)
        w_ref[D:D + 16, :] = jnp.where((r16 == 0) | (r16 == 2), -hi,
                                       jnp.where(r16 == 1, -lo, 0.0)).astype(bf)

    top = pl.ds(0, D)
    w_copies = [cp(wq_hbm, wq_s.at[top, :], sems.at[4]), cp(wk_hbm, wk_s.at[top, :], sems.at[5]),
                cp(wv_hbm, wv_s.at[top, :], sems.at[6]), cp(wo_hbm, wo_s, sems.at[7])]
    e_copies = [cp(wg_hbm, wg_s, sems.at[8]), cp(wu_hbm, wu_s, sems.at[9]),
                cp(wd_hbm, wd_s, sems.at[10])]

    x_copy(0).start()
    for c in w_copies:
        c.start()
    for s in range(1, NSEG):
        x_copy(s).start()

    g32 = jax.nn.sigmoid(beta_ref[...].astype(f32)).reshape(1, H)
    sel = _iota((H, H), 1) == _iota((H, H), 0)
    gcol = jnp.sum(jnp.where(sel, g32, 0.0), axis=1, keepdims=True)
    for h in range(H):
        g_s[h] = jnp.broadcast_to(gcol[h:h + 1], (1, 128))
    wr_s[...] = jnp.broadcast_to(wr_ref[...].astype(f32).reshape(1, D), (128, D)).T
    m_f[...] = jnp.zeros_like(m_f)
    wrs_s[...] = jnp.broadcast_to(jnp.sum(wr_s[...], axis=0, keepdims=True), (8, 128))
    den_s[...] = jnp.ones_like(den_s)

    for w_ref in (wq_s, wk_s, wv_s):
        w_ref[D + 16:DP, :] = jnp.zeros((DP - D - 16, D), bf)
    for s in range(NSEG):
        x_s[s, D + 16:DP, :] = jnp.zeros((DP - D - 16, L), bf)

    lane1 = _iota((1, 128), 1)
    causal = _iota((128, 128), 0) <= _iota((128, 128), 1)

    def proj(s, t):
        rows = pl.ds(64 * t, 64)
        xn = _tobf(xn_u[rows, :])
        rc = rc_s[t]
        rc4 = jnp.concatenate([rc] * 4, axis=1)
        q = _dot(xn, wq_s[:, 0:512]) * rc4
        k = _dot(xn, wk_s[:, 0:512]) * rc4
        r4 = _dot(xn, _tobf(w4_u[...])) * rc
        k4 = pltpu.roll(r4, 64, 1)
        for src, last, raw_ref, phi_ref, sc in ((q, r4, qx, pqx, QSCALE), (k, k4, kx, pkx, None)):
            tiles = [src[:, 128 * i:128 * (i + 1)] for i in range(4)] + [last]
            raw = [_pack(v * sc if sc is not None else v) for v in tiles]
            ph = [_pack(_phi(v)) for v in tiles]
            for c in range(NQ):
                i = c // 2
                if c % 2 == 0:
                    raw_ref[c, rows, :] = raw[i]
                    phi_ref[c, rows, :] = ph[i]
                else:
                    keep = lane1 >= (QW * c) % 128
                    raw_ref[c, rows, :] = jnp.where(keep, raw[i], raw[i + 1])
                    phi_ref[c, rows, :] = jnp.where(keep, ph[i], ph[i + 1])

    def proj_v(s, t):
        vt = _dot(_tobf(wvt_u[...]), x_s[s, :, pl.ds(128 * t, 128)]) * rs_s[t, 0:1]
        vt_u[:, pl.ds(128 * t, 128)] = _pack(vt)

    def scores(k, par, j):
        c = 2 * k + par
        lms = []
        for i in range(4):
            st = (2 * QW * k + QW * par + DH * i) % 128
            lms.append(jnp.where(((lane1 - st) & 127) < DH, jnp.uint32(0xFFFFFFFF), jnp.uint32(0)))
        q = qx[c, pl.ds(64 * j, 64), :]
        qm = _tobf(jnp.concatenate([q & lms[i] for i in range(4)], axis=0))
        kk = _tobf(kx[c, pl.ds(0, 64 * (j + 1)), :])
        return _dot_nt(kk, qm)

    def stage_a(k, par, j, p_ref):
        p = jnp.exp2(scores(k, par, j))
        pd = jnp.concatenate([jnp.where(causal, p[128 * j:, 128 * i:128 * (i + 1)], 0.0)
                              for i in range(4)], axis=1)
        off = 64 * (j * (j + 1) // 2)
        if j > 0:
            p_ref[pl.ds(off, 64 * j), :] = _pack(p[:128 * j])
        p_ref[pl.ds(off + 64 * j, 64), :] = _pack(pd)

    def stage_a_safe(k, par, j, p_ref):
        s = scores(k, par, j)
        bias = jnp.where(causal, 0.0, MASKB).astype(f32)
        sd = s[128 * j:] + jnp.concatenate([bias] * 4, axis=1)
        s = sd if j == 0 else jnp.concatenate([s[:128 * j], sd], axis=0)
        p = jnp.exp2(s - jnp.max(s, axis=0, keepdims=True))
        p_ref[pl.ds(64 * (j * (j + 1) // 2), 64 * (j + 1)), :] = _pack(p)

    def stage_b(use_mem, k, par, j, p_ref):
        c = 2 * k + par
        base = QW * par
        mwin = base - base % 16
        moff = base - mwin
        zrow = 72 if moff == 0 else 0
        srow = _iota((8, 128), 0)
        grow = [g_s[4 * c + i] for i in range(4)]
        off = 64 * (j * (j + 1) // 2)
        if use_mem:
            mem = _dot_nt(_tobf(m_u[c]), _tobf(pqx[c, pl.ds(64 * j, 64), :]))
        accs, rds, rms = [], [], []
        dlo, dhi = den_s[0:1], den_s[1:2]
        for i in range(4):
            r0 = base + DH * i
            w = r0 - r0 % 16
            o = r0 - w
            vt = vt_u[pl.ds(_al(QW * k + w // 2, 8), 16), pl.ds(0, 128 * (j + 1))]
            orow = 15 if o < 14 else 0
            vt = jnp.where(_iota(vt.shape, 0) == orow, jnp.uint32(ONES2), vt)
            p = _tobf(p_ref[pl.ds(off, 64 * (j + 1)), pl.ds(128 * i, 128)])
            acc = _dot(_tobf(vt), p)
            den = acc[2 * orow:2 * orow + 1]
            dlo, dhi = jnp.minimum(dlo, den), jnp.maximum(dhi, den)
            rds.append((1.0 - grow[i]) / den)
            if use_mem:
                rms.append(grow[i] / (mem[zrow + i:zrow + i + 1] + 1e-6))
            a0 = o - o % 8
            accs.append(acc[a0:a0 + 24])
        den_s[0:1] = dlo
        den_s[1:2] = dhi
        for v in range(9):
            lo_h, hi_h = (8 * v) // DH, (8 * v + 7) // DH

            def piece(h):
                a = accs[h][8 * (v - (DH * h) // 8):8 * (v - (DH * h) // 8) + 8]
                if not use_mem:
                    return a * rds[h]
                return a * rds[h] + mem[moff + 8 * v:moff + 8 * v + 8] * rms[h]
            val = piece(lo_h)
            if hi_h != lo_h:
                val = jnp.where(srow < DH * hi_h - 8 * v, val, piece(hi_h))
            ot_s[pl.ds(_al(2 * QW * k + base + 8 * v, 8), 8), pl.ds(128 * j, 128)] = val

    def mem_update(k, par):
        c = 2 * k + par
        base = QW * par
        mwin = base - base % 16
        moff = base - mwin
        zrow = 72 if moff == 0 else 0
        vw = vt_u[pl.ds(_al(QW * k + mwin // 2, 8), 40), :]
        rr = _iota(vw.shape, 0)
        isz = (rr >= 36) if moff == 0 else (rr < 4)
        vw = jnp.where(isz, jnp.uint32(ONES2), vw)
        upd = _dot(_tobf(vw), _tobf(pkx[c]))
        r80 = _iota((80, 128), 0)
        l80 = (_iota((80, 128), 1) - (2 * QW * k + base)) & 127
        hrow = jnp.where((r80 >= zrow) & (r80 < zrow + 8), r80 - zrow, (r80 - moff) // DH)
        keep = (l80 >= DH * hrow) & (l80 < DH * hrow + DH) & (hrow < 4) & (hrow >= 0)
        mnew = m_f[c] + jnp.where(keep, upd, 0.0)
        m_f[c] = mnew
        m_u[c] = _pack(mnew)

    pb = (p0, p1)

    def step(use_mem, update, a, b):
        for j in range(4):
            if b is not None:
                stage_b(use_mem, b[0], b[1], j, pb[b[1]])
                if j == 3 and update:
                    mem_update(b[0], b[1])
            if a is not None:
                stage_a(a[0], a[1], j, pb[a[1]])

    def out_proj(s, t):
        c = 128 * t
        o = ot_s[:, pl.ds(c, 128)].astype(bf)
        h = x_s[s, 0:D, pl.ds(c, 128)].astype(f32) + _dot(_tobf(wot_u[...]), o)
        h_s[4 * s + t] = h
        mean, rstd, sc = _ln_stats(lambda a, b: h[a:b], h[0:1], (wr_s[...], wrs_s[0:1]))
        st_s[4 * s + t, 0:1] = mean
        st_s[4 * s + t, 1:2] = rstd
        smax = jnp.max(sc, axis=1, keepdims=True)
        pos = (lane1 + (s * L + c)).astype(f32)
        sidx = jnp.min(jnp.where(sc == smax, pos, 1e9), axis=1, keepdims=True)
        new = jnp.concatenate([jnp.broadcast_to(smax, (1, 128)), jnp.broadcast_to(sidx, (1, 128)),
                               jnp.zeros((6, 128), f32)], axis=0)
        if t == 0:
            best_s[s] = new
        else:
            old = best_s[s]
            best_s[s] = jnp.where(smax > old[0:1, 0:1], new, old)

    def post(s, t):
        rstd = st_s[4 * s + t, 1:2]
        a = 1.0 + rstd
        b = st_s[4 * s + t, 0:1] * rstd
        out_s[s, :, pl.ds(128 * t, 128)] = (h_s[4 * s + t] * a - b).astype(bf)

    def finish(s):
        for t in range(4):
            out_proj(s, t)
            if t < 3:
                post(s, t)

    def attention(s):
        use_mem, update = s > 0, s < NSEG - 1
        step(use_mem, update, (0, 0), None)
        for k in range(NQ // 2):
            step(use_mem, update, (k, 1), (k, 0))
            step(use_mem, update, (k + 1, 0) if k + 1 < NQ // 2 else None, (k, 1))

    x_copy(0).wait()
    for t in range(4):
        prep(0, t)
    w_copies[0].wait()
    augment(wq_s)
    w_copies[1].wait()
    augment(wk_s)
    w4_u[...] = _tou(jnp.concatenate([wq_s[:, 512:D], wk_s[:, 512:D]], axis=1))
    for t in range(4):
        proj(0, t)
    for c in e_copies:
        c.start()
    w_copies[2].wait()
    augment(wv_s)
    wvt_u[...] = _tou(wv_s[...].T)
    wv_ok = jnp.max(jnp.abs(wv_s[0:D, :].astype(f32))) < WV_MAX
    for t in range(4):
        proj_v(0, t)
    w_copies[3].wait()
    wot_u[...] = _tou(wo_s[...].T)
    attention(0)
    for s in range(1, NSEG):
        x_copy(s).wait()
    finish(0)

    for s in range(1, NSEG):
        post(s - 1, 3)
        for t in range(4):
            prep(s, t)
        for t in range(4):
            proj_v(s, t)
        for t in range(4):
            proj(s, t)
        out_copy(s - 1).start()
        attention(s)
        finish(s)
    post(NSEG - 1, 3)
    out_copy(NSEG - 1).start()

    dl = den_s[...]
    safe = jnp.logical_and(jnp.min(dl[0:1]) >= DEN_LO, jnp.max(dl[1:2]) <= DEN_HI)
    safe = jnp.logical_and(safe, wv_ok)

    @pl.when(jnp.logical_not(safe))
    def _():
        for s in range(NSEG):
            out_copy(s).wait()
        m_f[...] = jnp.zeros_like(m_f)
        m_u[...] = jnp.zeros_like(m_u)

        def seg_redo(s, carry):
            for t in range(4):
                prep(s, t)
                proj_v(s, t)
                proj(s, t)

            def quads(k, carry):
                for par in range(2):
                    for j in range(4):
                        stage_a_safe(k, par, j, pb[par])
                        stage_b(True, k, par, j, pb[par])
                    mem_update(k, par)
                return carry
            lax.fori_loop(0, NQ // 2, quads, 0)
            finish(s)
            post(s, 3)
            out_copy(s).start()
            return carry
        lax.fori_loop(0, NSEG, seg_redo, 0)

    for c in e_copies:
        c.wait()
    best = best_s[0]
    for s in range(1, NSEG):
        cand = best_s[s]
        best = jnp.where(cand[0:1, 0:1] > best[0:1, 0:1], cand, best)
    idx = jnp.clip(best[1, 0].astype(i32), 0, S - 1)
    blk = idx // 128
    col = idx - blk * 128
    onehot = ((_iota((16, 128), 1) == col) & (_iota((16, 128), 0) == 0)).astype(bf)
    ln = ((h_s[blk] - st_s[blk, 0:1]) * st_s[blk, 1:2]).astype(bf)
    xs = _dot_nt(onehot, ln).astype(bf)
    gate = _dot(xs, wg_s[...])
    up = _dot(xs, wu_s[...])
    act = (gate * jax.nn.sigmoid(gate) * up).astype(bf)
    y = _dot_nt(act, wd_s[...]) * jax.nn.sigmoid(best[0:1, 0:1])
    yt = jnp.broadcast_to(y[0:1], (128, D)).T
    for s in range(NSEG):
        out_copy(s).wait()
    seg = blk // 4
    c0 = pl.multiple_of((blk - seg * 4) * 128, 128)
    cur = out_s[seg, :, pl.ds(c0, 128)].astype(f32)
    hit = _iota((D, 128), 1) == col
    fin_s[...] = (cur + jnp.where(hit, yt, 0.0)).astype(bf)
    fin = cp(fin_s, out_hbm.at[:, pl.ds(pl.multiple_of(blk * 128, 128), 128)], sems.at[15])
    fin.start()
    fin.wait()


@jax.jit
def pallas_sequential_preLN__memory_aug_infini_attn__moe_arch_mod__prompt_kernel(
    A_x, A_wq, A_wk, A_wv, A_wo, A_beta, B_x, B_w_r, B_w_gate, B_w_up, B_w_down,
):
    hbm = pl.BlockSpec(memory_space=pltpu.HBM)
    vm = pltpu.VMEM
    x_t = A_x.reshape(S, D).T
    out_t = pl.pallas_call(
        _kernel,
        out_shape=jax.ShapeDtypeStruct((D, S), bf),
        in_specs=[hbm] * 5 + [pl.BlockSpec(memory_space=pltpu.VMEM)] * 2 + [hbm] * 3,
        out_specs=hbm,
        scratch_shapes=[
            vm((NSEG, DP, L), bf), vm((DP, D), bf), vm((DP, D), bf), vm((DP, D), bf), vm((D, D), bf),
            vm((D, F), bf), vm((D, F), bf), vm((D, F), bf),
            vm((DP // 2, 128), u32), vm((D // 2, DP), u32), vm((D // 2, D), u32),
            vm((L // 2, DP), u32), vm((4, 8, 128), f32), vm((4, 128, 128), f32),
            vm((NQ, L // 2, 128), u32), vm((NQ, L // 2, 128), u32),
            vm((NQ, L // 2, 128), u32), vm((NQ, L // 2, 128), u32),
            vm((D // 2, L), u32),
            vm((640, 512), u32), vm((640, 512), u32), vm((16, D, 128), f32),
            vm((D, L), f32), vm((NQ, 80, 128), f32), vm((NQ, 40, 128), u32),
            vm((H, 1, 128), f32), vm((D, 128), f32), vm((8, 128), f32), vm((NSEG, D, L), bf),
            vm((16, 8, 128), f32),
            vm((NSEG, 8, 128), f32), vm((8, 128), f32), vm((D, 128), bf),
            pltpu.SemaphoreType.DMA((16,)),
        ],
        compiler_params=pltpu.CompilerParams(vmem_limit_bytes=100 * 1024 * 1024),
        name="infini_moe",
    )(x_t, A_wq, A_wk, A_wv, A_wo, A_beta, B_w_r, B_w_gate, B_w_up, B_w_down.T)
    return out_t.T.reshape(1, S, D)
```

```python
import jax
import jax.numpy as jnp
from jax import lax
from jax.experimental import pallas as pl
from jax.experimental.pallas import tpu as pltpu

S, D, H, DH = 2048, 576, 32, 18
NSEG, L, F = 4, 512, 4608
DP = 640
NQ = 8
QW = 4 * DH
bf, u32, f32, i32 = jnp.bfloat16, jnp.uint32, jnp.float32, jnp.int32
LOG2E = 1.4426950408889634
QSCALE = DH ** -0.5 * LOG2E
MASKB = -1000000000.0 * LOG2E
EPS = 1e-5
NT = (((1,), (1,)), ((), ()))
ONES2 = 0x3F803F80
DEN_LO, DEN_HI, WV_MAX = 2.0 ** -60, 2.0 ** 60, 2.0 ** 40


def _tobf(x):
    return pltpu.bitcast(x, bf)


def _tou(x):
    return pltpu.bitcast(x, u32)


def _pack(x):
    return pltpu.bitcast(x.astype(bf), u32)


def _dot(a, b):
    return jnp.dot(a, b, preferred_element_type=f32)


def _dot_nt(a, b):
    return lax.dot_general(a, b, NT, preferred_element_type=f32)


def _phi(t):
    return jnp.where(t > 0, t + 1.0, jnp.exp(t))


def _rowsum(parts):
    acc = [jnp.sum(p.reshape(p.shape[0] // 8, 8, 128), axis=0) for p in parts]
    while len(acc) > 1:
        acc = [acc[i] + acc[i + 1] for i in range(0, len(acc), 2)]
    return jnp.sum(acc[0], axis=0, keepdims=True)


def _ln_stats(rows, w=None):
    d = [rows(144 * g, 144 * (g + 1)) for g in range(4)]
    m1 = _rowsum(d) * (1.0 / D)
    m2 = _rowsum([v * v for v in d]) * (1.0 / D)
    var = jnp.maximum(m2 - m1 * m1, 0.0)
    rstd = lax.rsqrt(var + EPS)
    if w is None:
        return m1, rstd
    dw = _rowsum([d[g] * w[0][144 * g:144 * (g + 1)] for g in range(4)])
    return m1, rstd, (dw - m1 * w[1]) * rstd


def _hi_lo(v):
    hi = v.astype(bf).astype(f32)
    return hi, (v - hi).astype(bf).astype(f32)


def _iota(shape, dim):
    return lax.broadcasted_iota(i32, shape, dim)


def _al(x, n):
    return x if isinstance(x, int) else pl.multiple_of(x, n)


def _kernel(x_hbm, wq_hbm, wk_hbm, wv_hbm, wo_hbm, beta_ref, wr_ref,
            wg_hbm, wu_hbm, wd_hbm, out_hbm,
            x_s, wq_s, wk_s, wv_s, wo_s, wg_s, wu_s, wd_s,
            w4_u, wvt_u, wot_u, xn_u, rs_s, rc_s, qx, kx, pqx, pkx, vt_u,
            p0, p1, h_s, ot_s, m_f, m_u, g_s, wr_s, wrs_s, out_s, st_s, best_s, den_s, fin_s,
            sems):
    cp = pltpu.make_async_copy

    def x_copy(s):
        return cp(x_hbm.at[:, pl.ds(_al(s * L, L), L)], x_s.at[s, pl.ds(0, D), :], sems.at[s])

    def out_copy(s):
        return cp(out_s.at[s], out_hbm.at[:, pl.ds(_al(s * L, L), L)], sems.at[11 + s])

    def prep(s, t):
        c = 128 * t
        mean, rstd = _ln_stats(lambda a, b: x_s[s, a:b, pl.ds(c, 128)].astype(f32))
        mh, ml = _hi_lo(mean)
        r16 = _iota((16, 128), 0)
        x_s[s, D:D + 16, pl.ds(c, 128)] = jnp.where(
            r16 < 2, mh, jnp.where(r16 == 2, ml, 0.0)).astype(bf)
        rs_s[t, 0:1] = rstd
        rc_s[t] = jnp.broadcast_to(rstd, (128, 128)).T
        xn_u[pl.ds(64 * t, 64), :] = _tou(x_s[s, :, pl.ds(c, 128)].T)

    def augment(w_ref):
        ones = jnp.ones((16, D), bf)
        hi, lo = _hi_lo(_dot(ones, w_ref[0:D, :])[0:1])
        r16 = _iota((16, D), 0)
        w_ref[D:D + 16, :] = jnp.where((r16 == 0) | (r16 == 2), -hi,
                                       jnp.where(r16 == 1, -lo, 0.0)).astype(bf)

    top = pl.ds(0, D)
    w_copies = [cp(wq_hbm, wq_s.at[top, :], sems.at[4]), cp(wk_hbm, wk_s.at[top, :], sems.at[5]),
                cp(wv_hbm, wv_s.at[top, :], sems.at[6]), cp(wo_hbm, wo_s, sems.at[7])]
    e_copies = [cp(wg_hbm, wg_s, sems.at[8]), cp(wu_hbm, wu_s, sems.at[9]),
                cp(wd_hbm, wd_s, sems.at[10])]

    x_copy(0).start()
    w_copies[0].start()

    g32 = jax.nn.sigmoid(beta_ref[...].astype(f32)).reshape(1, H)
    sel = _iota((H, H), 1) == _iota((H, H), 0)
    gcol = jnp.sum(jnp.where(sel, g32, 0.0), axis=1, keepdims=True)
    for h in range(H):
        g_s[h] = jnp.broadcast_to(gcol[h:h + 1], (1, 128))
    wr_s[...] = jnp.broadcast_to(wr_ref[...].astype(f32).reshape(1, D), (128, D)).T
    m_f[...] = jnp.zeros_like(m_f)
    wrs_s[...] = jnp.broadcast_to(jnp.sum(wr_s[...], axis=0, keepdims=True), (8, 128))
    den_s[...] = jnp.ones_like(den_s)

    for w_ref in (wq_s, wk_s, wv_s):
        w_ref[D + 16:DP, :] = jnp.zeros((DP - D - 16, D), bf)
    for s in range(NSEG):
        x_s[s, D + 16:DP, :] = jnp.zeros((DP - D - 16, L), bf)

    lane1 = _iota((1, 128), 1)
    causal = _iota((128, 128), 0) <= _iota((128, 128), 1)

    def proj_q(t):
        rows = pl.ds(64 * t, 64)
        q = _dot(_tobf(xn_u[rows, :]), wq_s[:, 0:512]) * jnp.concatenate([rc_s[t]] * 4, axis=1)
        tiles = [q[:, 128 * i:128 * (i + 1)] for i in range(4)]
        raw = [_pack(v * QSCALE) for v in tiles]
        ph = [_pack(_phi(v)) for v in tiles]
        for c in range(NQ):
            i = c // 2
            if c % 2 == 0 or c == NQ - 1:
                qx[c, rows, :] = raw[i]
                pqx[c, rows, :] = ph[i]
            else:
                keep = lane1 >= (QW * c) % 128
                qx[c, rows, :] = jnp.where(keep, raw[i], raw[i + 1])
                pqx[c, rows, :] = jnp.where(keep, ph[i], ph[i + 1])

    def proj_k(t):
        rows = pl.ds(64 * t, 64)
        xn = _tobf(xn_u[rows, :])
        rc = rc_s[t]
        k = _dot(xn, wk_s[:, 0:512]) * jnp.concatenate([rc] * 4, axis=1)
        r4 = _dot(xn, _tobf(w4_u[...])) * rc
        tiles = [k[:, 128 * i:128 * (i + 1)] for i in range(4)] + [pltpu.roll(r4, 64, 1)]
        raw = [_pack(v) for v in tiles]
        ph = [_pack(_phi(v)) for v in tiles]
        for c in range(NQ):
            i = c // 2
            if c % 2 == 0:
                kx[c, rows, :] = raw[i]
                pkx[c, rows, :] = ph[i]
            else:
                keep = lane1 >= (QW * c) % 128
                kx[c, rows, :] = jnp.where(keep, raw[i], raw[i + 1])
                pkx[c, rows, :] = jnp.where(keep, ph[i], ph[i + 1])
        keep = lane1 >= (QW * (NQ - 1)) % 128
        qx[NQ - 1, rows, :] = jnp.where(keep, qx[NQ - 1, rows, :], _pack(r4 * QSCALE))
        pqx[NQ - 1, rows, :] = jnp.where(keep, pqx[NQ - 1, rows, :], _pack(_phi(r4)))

    def proj_v(s, t):
        vt = _dot(_tobf(wvt_u[...]), x_s[s, :, pl.ds(128 * t, 128)]) * rs_s[t, 0:1]
        vt_u[:, pl.ds(128 * t, 128)] = _pack(vt)

    def masked_q(k, par, j):
        q = qx[2 * k + par, pl.ds(64 * j, 64), :]
        out = []
        for i in range(4):
            st = (2 * QW * k + QW * par + DH * i) % 128
            out.append(q & jnp.where(((lane1 - st) & 127) < DH, jnp.uint32(0xFFFFFFFF),
                                     jnp.uint32(0)))
        return out

    def scores(k, par, j):
        qm = _tobf(jnp.concatenate(masked_q(k, par, j), axis=0))
        kk = _tobf(kx[2 * k + par, pl.ds(0, 64 * (j + 1)), :])
        return _dot_nt(kk, qm)

    r64, l64 = _iota((64, 128), 0), _iota((64, 128), 1)
    lo_nat = (l64 >= 64) | (r64 <= l64)
    lo_swp = (l64 < 64) | (r64 <= l64 - 64)
    hi_even = (l64 < 64) & (r64 <= l64)
    hi_odd = (l64 >= 64) & (r64 <= l64 - 64)

    def stage_a(k, par, j, p_ref):
        c = 2 * k + par
        qm = masked_q(k, par, j)
        w1 = [jnp.concatenate([qm[i][32:], qm[i][:32]], axis=0) if i % 2 == 0 else qm[i]
              for i in range(4)]
        w2 = [qm[i][32:] for i in range(4)]
        n1 = 128 * j + 64
        p1 = jnp.exp2(_dot_nt(_tobf(kx[c, pl.ds(0, n1 // 2), :]),
                              _tobf(jnp.concatenate(w1, axis=0))))
        p2 = jnp.exp2(_dot_nt(_tobf(kx[c, pl.ds(n1 // 2, 32), :]),
                              _tobf(jnp.concatenate(w2, axis=0))))
        off = 64 * (j * (j + 1) // 2)
        if j > 0:
            p_ref[pl.ds(off, 64 * j), :] = _pack(p1[:128 * j])
        lo = [jnp.where(lo_swp if i % 2 == 0 else lo_nat,
                        p1[128 * j:, 128 * i:128 * (i + 1)], 0.0) for i in range(4)]
        hi = [jnp.where(hi_even if i % 2 == 0 else hi_odd,
                        p2[:, 128 * (i // 2):128 * (i // 2 + 1)], 0.0) for i in range(4)]
        p_ref[pl.ds(off + 64 * j, 32), :] = _pack(jnp.concatenate(lo, axis=1))
        p_ref[pl.ds(off + 64 * j + 32, 32), :] = _pack(jnp.concatenate(hi, axis=1))

    def stage_a_safe(k, par, j, p_ref):
        s = scores(k, par, j)
        bias = jnp.where(causal, 0.0, MASKB).astype(f32)
        sd = s[128 * j:] + jnp.concatenate([bias] * 4, axis=1)
        s = sd if j == 0 else jnp.concatenate([s[:128 * j], sd], axis=0)
        p = jnp.exp2(s - jnp.max(s, axis=0, keepdims=True))
        p_ref[pl.ds(64 * (j * (j + 1) // 2), 64 * (j + 1)), :] = _pack(p)

    def stage_b(use_mem, k, par, j, p_ref, swapped=True):
        c = 2 * k + par
        base = QW * par
        mwin = base - base % 16
        moff = base - mwin
        zrow = 72 if moff == 0 else 0
        srow = _iota((8, 128), 0)
        grow = [g_s[4 * c + i] for i in range(4)]
        off = 64 * (j * (j + 1) // 2)
        if use_mem:
            mem = _dot_nt(_tobf(m_u[c]), _tobf(pqx[c, pl.ds(64 * j, 64), :]))
        accs, rds, rms = [], [], []
        dlo, dhi = den_s[0:1], den_s[1:2]
        for i in range(4):
            r0 = base + DH * i
            w = r0 - r0 % 16
            o = r0 - w
            vt = vt_u[pl.ds(_al(QW * k + w // 2, 8), 16), pl.ds(0, 128 * (j + 1))]
            orow = 15 if o < 14 else 0
            vt = jnp.where(_iota(vt.shape, 0) == orow, jnp.uint32(ONES2), vt)
            p = _tobf(p_ref[pl.ds(off, 64 * (j + 1)), pl.ds(128 * i, 128)])
            acc = _dot(_tobf(vt), p)
            if swapped and i % 2 == 0:
                acc = pltpu.roll(acc, 64, 1)
            den = acc[2 * orow:2 * orow + 1]
            dlo, dhi = jnp.minimum(dlo, den), jnp.maximum(dhi, den)
            rds.append((1.0 - grow[i]) / den)
            if use_mem:
                rms.append(grow[i] / (mem[zrow + i:zrow + i + 1] + 1e-6))
            a0 = o - o % 8
            accs.append(acc[a0:a0 + 24])
        den_s[0:1] = dlo
        den_s[1:2] = dhi
        for v in range(9):
            lo_h, hi_h = (8 * v) // DH, (8 * v + 7) // DH

            def piece(h):
                a = accs[h][8 * (v - (DH * h) // 8):8 * (v - (DH * h) // 8) + 8]
                if not use_mem:
                    return a * rds[h]
                return a * rds[h] + mem[moff + 8 * v:moff + 8 * v + 8] * rms[h]
            val = piece(lo_h)
            if hi_h != lo_h:
                val = jnp.where(srow < DH * hi_h - 8 * v, val, piece(hi_h))
            ot_s[pl.ds(_al(2 * QW * k + base + 8 * v, 8), 8), pl.ds(128 * j, 128)] = val

    def mem_update(k, par):
        c = 2 * k + par
        base = QW * par
        mwin = base - base % 16
        moff = base - mwin
        zrow = 72 if moff == 0 else 0
        vw = vt_u[pl.ds(_al(QW * k + mwin // 2, 8), 40), :]
        rr = _iota(vw.shape, 0)
        isz = (rr >= 36) if moff == 0 else (rr < 4)
        vw = jnp.where(isz, jnp.uint32(ONES2), vw)
        upd = _dot(_tobf(vw), _tobf(pkx[c]))
        r80 = _iota((80, 128), 0)
        l80 = (_iota((80, 128), 1) - (2 * QW * k + base)) & 127
        hrow = jnp.where((r80 >= zrow) & (r80 < zrow + 8), r80 - zrow, (r80 - moff) // DH)
        keep = (l80 >= DH * hrow) & (l80 < DH * hrow + DH) & (hrow < 4) & (hrow >= 0)
        mnew = m_f[c] + jnp.where(keep, upd, 0.0)
        m_f[c] = mnew
        m_u[c] = _pack(mnew)

    pb = (p0, p1)

    def step(use_mem, update, a, b):
        for j in range(4):
            if b is not None:
                stage_b(use_mem, b[0], b[1], j, pb[b[1]])
                if j == 3 and update:
                    mem_update(b[0], b[1])
            if a is not None:
                stage_a(a[0], a[1], j, pb[a[1]])

    def out_proj(s, t):
        c = 128 * t
        o = ot_s[:, pl.ds(c, 128)].astype(bf)
        h = x_s[s, 0:D, pl.ds(c, 128)].astype(f32) + _dot(_tobf(wot_u[...]), o)
        h_s[4 * s + t] = h
        mean, rstd, sc = _ln_stats(lambda a, b: h[a:b], (wr_s[...], wrs_s[0:1]))
        st_s[4 * s + t, 0:1] = mean
        st_s[4 * s + t, 1:2] = rstd
        smax = jnp.max(sc, axis=1, keepdims=True)
        pos = (lane1 + (s * L + c)).astype(f32)
        sidx = jnp.min(jnp.where(sc == smax, pos, 1e9), axis=1, keepdims=True)
        new = jnp.concatenate([jnp.broadcast_to(smax, (1, 128)), jnp.broadcast_to(sidx, (1, 128)),
                               jnp.zeros((6, 128), f32)], axis=0)
        if t == 0:
            best_s[s] = new
        else:
            old = best_s[s]
            best_s[s] = jnp.where(smax > old[0:1, 0:1], new, old)

    def post(s, t):
        rstd = st_s[4 * s + t, 1:2]
        a = 1.0 + rstd
        b = st_s[4 * s + t, 0:1] * rstd
        out_s[s, :, pl.ds(128 * t, 128)] = (h_s[4 * s + t] * a - b).astype(bf)

    def finish(s):
        for t in range(4):
            out_proj(s, t)
            if t < 3:
                post(s, t)

    def attention(s):
        use_mem, update = s > 0, s < NSEG - 1
        step(use_mem, update, (0, 0), None)
        for k in range(NQ // 2):
            step(use_mem, update, (k, 1), (k, 0))
            step(use_mem, update, (k + 1, 0) if k + 1 < NQ // 2 else None, (k, 1))

    x_copy(0).wait()
    w_copies[1].start()
    for t in range(4):
        prep(0, t)
    w_copies[0].wait()
    w_copies[2].start()
    augment(wq_s)
    for t in range(4):
        proj_q(t)
    w_copies[1].wait()
    w_copies[3].start()
    for s in range(1, NSEG):
        x_copy(s).start()
    augment(wk_s)
    w4_u[...] = _tou(jnp.concatenate([wq_s[:, 512:D], wk_s[:, 512:D]], axis=1))
    for t in range(2):
        proj_k(t)
    w_copies[2].wait()
    for c in e_copies:
        c.start()
    augment(wv_s)
    wvt_u[...] = _tou(wv_s[...].T)
    wv_ok = jnp.max(jnp.abs(wv_s[0:D, :].astype(f32))) < WV_MAX
    for t in range(2, 4):
        proj_k(t)
    w_copies[3].wait()
    wot_u[...] = _tou(wo_s[...].T)
    for t in range(4):
        proj_v(0, t)
    attention(0)
    for s in range(1, NSEG):
        x_copy(s).wait()
    finish(0)

    for s in range(1, NSEG):
        post(s - 1, 3)
        for t in range(4):
            prep(s, t)
        for t in range(4):
            proj_v(s, t)
        for t in range(4):
            proj_q(t)
            proj_k(t)
        out_copy(s - 1).start()
        attention(s)
        finish(s)
    post(NSEG - 1, 3)
    out_copy(NSEG - 1).start()

    dl = den_s[...]
    safe = jnp.logical_and(jnp.min(dl[0:1]) >= DEN_LO, jnp.max(dl[1:2]) <= DEN_HI)
    safe = jnp.logical_and(safe, wv_ok)

    @pl.when(jnp.logical_not(safe))
    def _():
        for s in range(NSEG):
            out_copy(s).wait()
        m_f[...] = jnp.zeros_like(m_f)
        m_u[...] = jnp.zeros_like(m_u)

        def seg_redo(s, carry):
            for t in range(4):
                prep(s, t)
                proj_v(s, t)
                proj_q(t)
                proj_k(t)

            def quads(k, carry):
                for par in range(2):
                    for j in range(4):
                        stage_a_safe(k, par, j, pb[par])
                        stage_b(True, k, par, j, pb[par], swapped=False)
                    mem_update(k, par)
                return carry
            lax.fori_loop(0, NQ // 2, quads, 0)
            finish(s)
            post(s, 3)
            out_copy(s).start()
            return carry
        lax.fori_loop(0, NSEG, seg_redo, 0)

    for c in e_copies:
        c.wait()
    best = best_s[0]
    for s in range(1, NSEG):
        cand = best_s[s]
        best = jnp.where(cand[0:1, 0:1] > best[0:1, 0:1], cand, best)
    idx = jnp.clip(best[1, 0].astype(i32), 0, S - 1)
    blk = idx // 128
    col = idx - blk * 128
    onehot = ((_iota((16, 128), 1) == col) & (_iota((16, 128), 0) == 0)).astype(bf)
    ln = ((h_s[blk] - st_s[blk, 0:1]) * st_s[blk, 1:2]).astype(bf)
    xs = _dot_nt(onehot, ln).astype(bf)
    gate = _dot(xs, wg_s[...])
    up = _dot(xs, wu_s[...])
    act = (gate * jax.nn.sigmoid(gate) * up).astype(bf)
    y = _dot_nt(act, wd_s[...]) * jax.nn.sigmoid(best[0:1, 0:1])
    yt = jnp.broadcast_to(y[0:1], (128, D)).T
    for s in range(NSEG):
        out_copy(s).wait()
    seg = blk // 4
    c0 = pl.multiple_of((blk - seg * 4) * 128, 128)
    cur = out_s[seg, :, pl.ds(c0, 128)].astype(f32)
    hit = _iota((D, 128), 1) == col
    fin_s[...] = (cur + jnp.where(hit, yt, 0.0)).astype(bf)
    fin = cp(fin_s, out_hbm.at[:, pl.ds(pl.multiple_of(blk * 128, 128), 128)], sems.at[15])
    fin.start()
    fin.wait()


@jax.jit
def pallas_sequential_preLN__memory_aug_infini_attn__moe_arch_mod__prompt_kernel(
    A_x, A_wq, A_wk, A_wv, A_wo, A_beta, B_x, B_w_r, B_w_gate, B_w_up, B_w_down,
):
    hbm = pl.BlockSpec(memory_space=pltpu.HBM)
    vm = pltpu.VMEM
    x_t = A_x.reshape(S, D).T
    out_t = pl.pallas_call(
        _kernel,
        out_shape=jax.ShapeDtypeStruct((D, S), bf),
        in_specs=[hbm] * 5 + [pl.BlockSpec(memory_space=pltpu.VMEM)] * 2 + [hbm] * 3,
        out_specs=hbm,
        scratch_shapes=[
            vm((NSEG, DP, L), bf), vm((DP, D), bf), vm((DP, D), bf), vm((DP, D), bf), vm((D, D), bf),
            vm((D, F), bf), vm((D, F), bf), vm((D, F), bf),
            vm((DP // 2, 128), u32), vm((D // 2, DP), u32), vm((D // 2, D), u32),
            vm((L // 2, DP), u32), vm((4, 8, 128), f32), vm((4, 128, 128), f32),
            vm((NQ, L // 2, 128), u32), vm((NQ, L // 2, 128), u32),
            vm((NQ, L // 2, 128), u32), vm((NQ, L // 2, 128), u32),
            vm((D // 2, L), u32),
            vm((640, 512), u32), vm((640, 512), u32), vm((16, D, 128), f32),
            vm((D, L), f32), vm((NQ, 80, 128), f32), vm((NQ, 40, 128), u32),
            vm((H, 1, 128), f32), vm((D, 128), f32), vm((8, 128), f32), vm((NSEG, D, L), bf),
            vm((16, 8, 128), f32),
            vm((NSEG, 8, 128), f32), vm((8, 128), f32), vm((D, 128), bf),
            pltpu.SemaphoreType.DMA((16,)),
        ],
        compiler_params=pltpu.CompilerParams(vmem_limit_bytes=100 * 1024 * 1024),
        name="infini_moe",
    )(x_t, A_wq, A_wk, A_wv, A_wo, A_beta, B_w_r, B_w_gate, B_w_up, B_w_down.T)
    return out_t.T.reshape(1, S, D)
```

```python
import jax
import jax.numpy as jnp
from jax import lax
from jax.experimental import pallas as pl
from jax.experimental.pallas import tpu as pltpu

S, D, H, DH = 2048, 576, 32, 18
NSEG, L, F = 4, 512, 4608
DP = 640
NQ = 8
QW = 4 * DH
bf, u32, f32, i32 = jnp.bfloat16, jnp.uint32, jnp.float32, jnp.int32
LOG2E = 1.4426950408889634
QSCALE = DH ** -0.5 * LOG2E
MASKB = -1000000000.0 * LOG2E
EPS = 1e-5
NT = (((1,), (1,)), ((), ()))
ONES2 = 0x3F803F80
DEN_LO, DEN_HI, WV_MAX = 2.0 ** -60, 2.0 ** 60, 2.0 ** 40


def _tobf(x):
    return pltpu.bitcast(x, bf)


def _tou(x):
    return pltpu.bitcast(x, u32)


def _pack(x):
    return pltpu.bitcast(x.astype(bf), u32)


def _dot(a, b):
    return jnp.dot(a, b, preferred_element_type=f32)


def _dot_nt(a, b):
    return lax.dot_general(a, b, NT, preferred_element_type=f32)


def _phi(t):
    return jnp.where(t > 0, t + 1.0, jnp.exp(t))


def _rowsum(parts):
    acc = [jnp.sum(p.reshape(p.shape[0] // 8, 8, 128), axis=0) for p in parts]
    while len(acc) > 1:
        acc = [acc[i] + acc[i + 1] for i in range(0, len(acc), 2)]
    return jnp.sum(acc[0], axis=0, keepdims=True)


def _ln_stats(rows, w=None):
    d = [rows(144 * g, 144 * (g + 1)) for g in range(4)]
    m1 = _rowsum(d) * (1.0 / D)
    m2 = _rowsum([v * v for v in d]) * (1.0 / D)
    var = jnp.maximum(m2 - m1 * m1, 0.0)
    rstd = lax.rsqrt(var + EPS)
    if w is None:
        return m1, rstd
    dw = _rowsum([d[g] * w[0][144 * g:144 * (g + 1)] for g in range(4)])
    return m1, rstd, (dw - m1 * w[1]) * rstd


def _hi_lo(v):
    hi = v.astype(bf).astype(f32)
    return hi, (v - hi).astype(bf).astype(f32)


def _iota(shape, dim):
    return lax.broadcasted_iota(i32, shape, dim)


def _al(x, n):
    return x if isinstance(x, int) else pl.multiple_of(x, n)


def _kernel(x_hbm, wq_hbm, wk_hbm, wv_hbm, wo_hbm, beta_hbm, wr_hbm,
            wg_hbm, wu_hbm, wd_hbm, out_hbm,
            x_s, wq_s, wk_s, wv_s, wo_s, wg_s, wu_s, wd_s,
            w4_u, wvt_u, wot_u, xn_u, rs_s, rc_s, qx, kx, pqx, pkx, vt_u,
            p0, p1, h_s, ot_s, m_f, m_u, g_s, wr_s, wrs_s, out_s, st_s, best_s, den_s, fin_s,
            beta_ref, wr_ref, sems):
    cp = pltpu.make_async_copy

    def x_copy(s):
        return cp(x_hbm.at[:, pl.ds(_al(s * L, L), L)], x_s.at[s, pl.ds(0, D), :], sems.at[s])

    def out_copy(s):
        return cp(out_s.at[s], out_hbm.at[:, pl.ds(_al(s * L, L), L)], sems.at[11 + s])

    def prep(s, t):
        c = 128 * t
        mean, rstd = _ln_stats(lambda a, b: x_s[s, a:b, pl.ds(c, 128)].astype(f32))
        mh, ml = _hi_lo(mean)
        r16 = _iota((16, 128), 0)
        x_s[s, D:D + 16, pl.ds(c, 128)] = jnp.where(
            r16 < 2, mh, jnp.where(r16 == 2, ml, 0.0)).astype(bf)
        rs_s[t, 0:1] = rstd
        rc_s[t] = jnp.broadcast_to(rstd, (128, 128)).T
        xn_u[pl.ds(64 * t, 64), :] = _tou(x_s[s, :, pl.ds(c, 128)].T)

    def augment(w_ref):
        ones = jnp.ones((16, D), bf)
        hi, lo = _hi_lo(_dot(ones, w_ref[0:D, :])[0:1])
        r16 = _iota((16, D), 0)
        w_ref[D:D + 16, :] = jnp.where((r16 == 0) | (r16 == 2), -hi,
                                       jnp.where(r16 == 1, -lo, 0.0)).astype(bf)

    top = pl.ds(0, D)
    w_copies = [cp(wq_hbm, wq_s.at[top, :], sems.at[4]), cp(wk_hbm, wk_s.at[top, :], sems.at[5]),
                cp(wv_hbm, wv_s.at[top, :], sems.at[6]), cp(wo_hbm, wo_s, sems.at[7])]
    e_copies = [cp(wg_hbm, wg_s, sems.at[8]), cp(wu_hbm, wu_s, sems.at[9]),
                cp(wd_hbm, wd_s, sems.at[10])]

    small = [cp(beta_hbm, beta_ref, sems.at[16]), cp(wr_hbm, wr_ref, sems.at[17])]
    x_copy(0).start()
    w_copies[0].start()
    for c in small:
        c.start()

    m_f[...] = jnp.zeros_like(m_f)
    den_s[...] = jnp.ones_like(den_s)

    for w_ref in (wq_s, wk_s, wv_s):
        w_ref[D + 16:DP, :] = jnp.zeros((DP - D - 16, D), bf)
    for s in range(NSEG):
        x_s[s, D + 16:DP, :] = jnp.zeros((DP - D - 16, L), bf)

    lane1 = _iota((1, 128), 1)
    causal = _iota((128, 128), 0) <= _iota((128, 128), 1)

    def proj_q(t):
        rows = pl.ds(64 * t, 64)
        q = _dot(_tobf(xn_u[rows, :]), wq_s[:, 0:512]) * jnp.concatenate([rc_s[t]] * 4, axis=1)
        tiles = [q[:, 128 * i:128 * (i + 1)] for i in range(4)]
        raw = [_pack(v * QSCALE) for v in tiles]
        ph = [_pack(_phi(v)) for v in tiles]
        for c in range(NQ):
            i = c // 2
            if c % 2 == 0 or c == NQ - 1:
                qx[c, rows, :] = raw[i]
                pqx[c, rows, :] = ph[i]
            else:
                keep = lane1 >= (QW * c) % 128
                qx[c, rows, :] = jnp.where(keep, raw[i], raw[i + 1])
                pqx[c, rows, :] = jnp.where(keep, ph[i], ph[i + 1])

    def proj_k(t):
        rows = pl.ds(64 * t, 64)
        xn = _tobf(xn_u[rows, :])
        rc = rc_s[t]
        k = _dot(xn, wk_s[:, 0:512]) * jnp.concatenate([rc] * 4, axis=1)
        r4 = _dot(xn, _tobf(w4_u[...])) * rc
        tiles = [k[:, 128 * i:128 * (i + 1)] for i in range(4)] + [pltpu.roll(r4, 64, 1)]
        raw = [_pack(v) for v in tiles]
        ph = [_pack(_phi(v)) for v in tiles]
        for c in range(NQ):
            i = c // 2
            if c % 2 == 0:
                kx[c, rows, :] = raw[i]
                pkx[c, rows, :] = ph[i]
            else:
                keep = lane1 >= (QW * c) % 128
                kx[c, rows, :] = jnp.where(keep, raw[i], raw[i + 1])
                pkx[c, rows, :] = jnp.where(keep, ph[i], ph[i + 1])
        keep = lane1 >= (QW * (NQ - 1)) % 128
        qx[NQ - 1, rows, :] = jnp.where(keep, qx[NQ - 1, rows, :], _pack(r4 * QSCALE))
        pqx[NQ - 1, rows, :] = jnp.where(keep, pqx[NQ - 1, rows, :], _pack(_phi(r4)))

    def proj_v(s, t):
        vt = _dot(_tobf(wvt_u[...]), x_s[s, :, pl.ds(128 * t, 128)]) * rs_s[t, 0:1]
        vt_u[:, pl.ds(128 * t, 128)] = _pack(vt)

    def masked_q(k, par, j):
        q = qx[2 * k + par, pl.ds(64 * j, 64), :]
        out = []
        for i in range(4):
            st = (2 * QW * k + QW * par + DH * i) % 128
            out.append(q & jnp.where(((lane1 - st) & 127) < DH, jnp.uint32(0xFFFFFFFF),
                                     jnp.uint32(0)))
        return out

    def scores(k, par, j):
        qm = _tobf(jnp.concatenate(masked_q(k, par, j), axis=0))
        kk = _tobf(kx[2 * k + par, pl.ds(0, 64 * (j + 1)), :])
        return _dot_nt(kk, qm)

    r64, l64 = _iota((64, 128), 0), _iota((64, 128), 1)
    lo_nat = (l64 >= 64) | (r64 <= l64)
    lo_swp = (l64 < 64) | (r64 <= l64 - 64)
    hi_even = (l64 < 64) & (r64 <= l64)
    hi_odd = (l64 >= 64) & (r64 <= l64 - 64)

    def stage_a(k, par, j, p_ref):
        c = 2 * k + par
        qm = masked_q(k, par, j)
        w1 = [jnp.concatenate([qm[i][32:], qm[i][:32]], axis=0) if i % 2 == 0 else qm[i]
              for i in range(4)]
        w2 = [qm[i][32:] for i in range(4)]
        n1 = 128 * j + 64
        p1 = jnp.exp2(_dot_nt(_tobf(kx[c, pl.ds(0, n1 // 2), :]),
                              _tobf(jnp.concatenate(w1, axis=0))))
        p2 = jnp.exp2(_dot_nt(_tobf(kx[c, pl.ds(n1 // 2, 32), :]),
                              _tobf(jnp.concatenate(w2, axis=0))))
        off = 64 * (j * (j + 1) // 2)
        if j > 0:
            p_ref[pl.ds(off, 64 * j), :] = _pack(p1[:128 * j])
        lo = [jnp.where(lo_swp if i % 2 == 0 else lo_nat,
                        p1[128 * j:, 128 * i:128 * (i + 1)], 0.0) for i in range(4)]
        hi = [jnp.where(hi_even if i % 2 == 0 else hi_odd,
                        p2[:, 128 * (i // 2):128 * (i // 2 + 1)], 0.0) for i in range(4)]
        p_ref[pl.ds(off + 64 * j, 32), :] = _pack(jnp.concatenate(lo, axis=1))
        p_ref[pl.ds(off + 64 * j + 32, 32), :] = _pack(jnp.concatenate(hi, axis=1))

    def stage_a_safe(k, par, j, p_ref):
        s = scores(k, par, j)
        bias = jnp.where(causal, 0.0, MASKB).astype(f32)
        sd = s[128 * j:] + jnp.concatenate([bias] * 4, axis=1)
        s = sd if j == 0 else jnp.concatenate([s[:128 * j], sd], axis=0)
        p = jnp.exp2(s - jnp.max(s, axis=0, keepdims=True))
        p_ref[pl.ds(64 * (j * (j + 1) // 2), 64 * (j + 1)), :] = _pack(p)

    def stage_b(use_mem, k, par, j, p_ref, swapped=True):
        c = 2 * k + par
        base = QW * par
        mwin = base - base % 16
        moff = base - mwin
        zrow = 72 if moff == 0 else 0
        srow = _iota((8, 128), 0)
        grow = [g_s[4 * c + i] for i in range(4)]
        off = 64 * (j * (j + 1) // 2)
        if use_mem:
            mem = _dot_nt(_tobf(m_u[c]), _tobf(pqx[c, pl.ds(64 * j, 64), :]))
        accs, rds, rms = [], [], []
        dlo, dhi = den_s[0:1], den_s[1:2]
        for i in range(4):
            r0 = base + DH * i
            w = r0 - r0 % 16
            o = r0 - w
            vt = vt_u[pl.ds(_al(QW * k + w // 2, 8), 16), pl.ds(0, 128 * (j + 1))]
            orow = 15 if o < 14 else 0
            vt = jnp.where(_iota(vt.shape, 0) == orow, jnp.uint32(ONES2), vt)
            p = _tobf(p_ref[pl.ds(off, 64 * (j + 1)), pl.ds(128 * i, 128)])
            acc = _dot(_tobf(vt), p)
            if swapped and i % 2 == 0:
                acc = pltpu.roll(acc, 64, 1)
            den = acc[2 * orow:2 * orow + 1]
            dlo, dhi = jnp.minimum(dlo, den), jnp.maximum(dhi, den)
            rds.append((1.0 - grow[i]) / den)
            if use_mem:
                rms.append(grow[i] / (mem[zrow + i:zrow + i + 1] + 1e-6))
            a0 = o - o % 8
            accs.append(acc[a0:a0 + 24])
        den_s[0:1] = dlo
        den_s[1:2] = dhi
        for v in range(9):
            lo_h, hi_h = (8 * v) // DH, (8 * v + 7) // DH

            def piece(h):
                a = accs[h][8 * (v - (DH * h) // 8):8 * (v - (DH * h) // 8) + 8]
                if not use_mem:
                    return a * rds[h]
                return a * rds[h] + mem[moff + 8 * v:moff + 8 * v + 8] * rms[h]
            val = piece(lo_h)
            if hi_h != lo_h:
                val = jnp.where(srow < DH * hi_h - 8 * v, val, piece(hi_h))
            ot_s[pl.ds(_al(2 * QW * k + base + 8 * v, 8), 8), pl.ds(128 * j, 128)] = val

    def mem_update(k, par):
        c = 2 * k + par
        base = QW * par
        mwin = base - base % 16
        moff = base - mwin
        zrow = 72 if moff == 0 else 0
        vw = vt_u[pl.ds(_al(QW * k + mwin // 2, 8), 40), :]
        rr = _iota(vw.shape, 0)
        isz = (rr >= 36) if moff == 0 else (rr < 4)
        vw = jnp.where(isz, jnp.uint32(ONES2), vw)
        upd = _dot(_tobf(vw), _tobf(pkx[c]))
        r80 = _iota((80, 128), 0)
        l80 = (_iota((80, 128), 1) - (2 * QW * k + base)) & 127
        hrow = jnp.where((r80 >= zrow) & (r80 < zrow + 8), r80 - zrow, (r80 - moff) // DH)
        keep = (l80 >= DH * hrow) & (l80 < DH * hrow + DH) & (hrow < 4) & (hrow >= 0)
        mnew = m_f[c] + jnp.where(keep, upd, 0.0)
        m_f[c] = mnew
        m_u[c] = _pack(mnew)

    pb = (p0, p1)

    def step(use_mem, update, a, b):
        for j in range(4):
            if b is not None:
                stage_b(use_mem, b[0], b[1], j, pb[b[1]])
                if j == 3 and update:
                    mem_update(b[0], b[1])
            if a is not None:
                stage_a(a[0], a[1], j, pb[a[1]])

    def out_proj(s, t):
        c = 128 * t
        o = ot_s[:, pl.ds(c, 128)].astype(bf)
        h = x_s[s, 0:D, pl.ds(c, 128)].astype(f32) + _dot(_tobf(wot_u[...]), o)
        h_s[4 * s + t] = h
        mean, rstd, sc = _ln_stats(lambda a, b: h[a:b], (wr_s[...], wrs_s[0:1]))
        st_s[4 * s + t, 0:1] = mean
        st_s[4 * s + t, 1:2] = rstd
        smax = jnp.max(sc, axis=1, keepdims=True)
        pos = (lane1 + (s * L + c)).astype(f32)
        sidx = jnp.min(jnp.where(sc == smax, pos, 1e9), axis=1, keepdims=True)
        new = jnp.concatenate([jnp.broadcast_to(smax, (1, 128)), jnp.broadcast_to(sidx, (1, 128)),
                               jnp.zeros((6, 128), f32)], axis=0)
        if t == 0:
            best_s[s] = new
        else:
            old = best_s[s]
            best_s[s] = jnp.where(smax > old[0:1, 0:1], new, old)

    def post(s, t):
        rstd = st_s[4 * s + t, 1:2]
        a = 1.0 + rstd
        b = st_s[4 * s + t, 0:1] * rstd
        out_s[s, :, pl.ds(128 * t, 128)] = (h_s[4 * s + t] * a - b).astype(bf)

    def finish(s):
        for t in range(4):
            out_proj(s, t)
            if t < 3:
                post(s, t)

    def attention(s):
        use_mem, update = s > 0, s < NSEG - 1
        step(use_mem, update, (0, 0), None)
        for k in range(NQ // 2):
            step(use_mem, update, (k, 1), (k, 0))
            step(use_mem, update, (k + 1, 0) if k + 1 < NQ // 2 else None, (k, 1))

    x_copy(0).wait()
    w_copies[1].start()
    for t in range(4):
        prep(0, t)
    w_copies[0].wait()
    w_copies[2].start()
    augment(wq_s)
    for t in range(4):
        proj_q(t)
    w_copies[1].wait()
    w_copies[3].start()
    for s in range(1, NSEG):
        x_copy(s).start()
    augment(wk_s)
    w4_u[...] = _tou(jnp.concatenate([wq_s[:, 512:D], wk_s[:, 512:D]], axis=1))
    for t in range(2):
        proj_k(t)
    w_copies[2].wait()
    for c in e_copies:
        c.start()
    augment(wv_s)
    wvt_u[...] = _tou(wv_s[...].T)
    wv_ok = jnp.max(jnp.abs(wv_s[0:D, :].astype(f32))) < WV_MAX
    for t in range(2, 4):
        proj_k(t)
    w_copies[3].wait()
    for c in small:
        c.wait()
    g32 = jax.nn.sigmoid(beta_ref[...].astype(f32)).reshape(1, H)
    sel = _iota((H, H), 1) == _iota((H, H), 0)
    gcol = jnp.sum(jnp.where(sel, g32, 0.0), axis=1, keepdims=True)
    for h in range(H):
        g_s[h] = jnp.broadcast_to(gcol[h:h + 1], (1, 128))
    wr_s[...] = jnp.broadcast_to(wr_ref[...].astype(f32).reshape(1, D), (128, D)).T
    wrs_s[...] = jnp.broadcast_to(jnp.sum(wr_s[...], axis=0, keepdims=True), (8, 128))
    wot_u[...] = _tou(wo_s[...].T)
    for t in range(4):
        proj_v(0, t)
    attention(0)
    for s in range(1, NSEG):
        x_copy(s).wait()
    finish(0)

    for s in range(1, NSEG):
        post(s - 1, 3)
        for t in range(4):
            prep(s, t)
        for t in range(4):
            proj_v(s, t)
        for t in range(4):
            proj_q(t)
            proj_k(t)
        out_copy(s - 1).start()
        attention(s)
        finish(s)
    post(NSEG - 1, 3)
    out_copy(NSEG - 1).start()

    dl = den_s[...]
    safe = jnp.logical_and(jnp.min(dl[0:1]) >= DEN_LO, jnp.max(dl[1:2]) <= DEN_HI)
    safe = jnp.logical_and(safe, wv_ok)

    @pl.when(jnp.logical_not(safe))
    def _():
        for s in range(NSEG):
            out_copy(s).wait()
        m_f[...] = jnp.zeros_like(m_f)
        m_u[...] = jnp.zeros_like(m_u)

        def seg_redo(s, carry):
            for t in range(4):
                prep(s, t)
                proj_v(s, t)
                proj_q(t)
                proj_k(t)

            def quads(k, carry):
                for par in range(2):
                    for j in range(4):
                        stage_a_safe(k, par, j, pb[par])
                        stage_b(True, k, par, j, pb[par], swapped=False)
                    mem_update(k, par)
                return carry
            lax.fori_loop(0, NQ // 2, quads, 0)
            finish(s)
            post(s, 3)
            out_copy(s).start()
            return carry
        lax.fori_loop(0, NSEG, seg_redo, 0)

    for c in e_copies:
        c.wait()
    best = best_s[0]
    for s in range(1, NSEG):
        cand = best_s[s]
        best = jnp.where(cand[0:1, 0:1] > best[0:1, 0:1], cand, best)
    idx = jnp.clip(best[1, 0].astype(i32), 0, S - 1)
    blk = idx // 128
    col = idx - blk * 128
    onehot = ((_iota((16, 128), 1) == col) & (_iota((16, 128), 0) == 0)).astype(bf)
    ln = ((h_s[blk] - st_s[blk, 0:1]) * st_s[blk, 1:2]).astype(bf)
    xs = _dot_nt(onehot, ln).astype(bf)
    gate = _dot(xs, wg_s[...])
    up = _dot(xs, wu_s[...])
    act = (gate * jax.nn.sigmoid(gate) * up).astype(bf)
    y = _dot_nt(act, wd_s[...]) * jax.nn.sigmoid(best[0:1, 0:1])
    yt = jnp.broadcast_to(y[0:1], (128, D)).T
    for s in range(NSEG):
        out_copy(s).wait()
    seg = blk // 4
    c0 = pl.multiple_of((blk - seg * 4) * 128, 128)
    cur = out_s[seg, :, pl.ds(c0, 128)].astype(f32)
    hit = _iota((D, 128), 1) == col
    fin_s[...] = (cur + jnp.where(hit, yt, 0.0)).astype(bf)
    fin = cp(fin_s, out_hbm.at[:, pl.ds(pl.multiple_of(blk * 128, 128), 128)], sems.at[15])
    fin.start()
    fin.wait()


@jax.jit
def pallas_sequential_preLN__memory_aug_infini_attn__moe_arch_mod__prompt_kernel(
    A_x, A_wq, A_wk, A_wv, A_wo, A_beta, B_x, B_w_r, B_w_gate, B_w_up, B_w_down,
):
    hbm = pl.BlockSpec(memory_space=pltpu.HBM)
    vm = pltpu.VMEM
    x_t = A_x.reshape(S, D).T
    out_t = pl.pallas_call(
        _kernel,
        out_shape=jax.ShapeDtypeStruct((D, S), bf),
        in_specs=[hbm] * 10,
        out_specs=hbm,
        scratch_shapes=[
            vm((NSEG, DP, L), bf), vm((DP, D), bf), vm((DP, D), bf), vm((DP, D), bf), vm((D, D), bf),
            vm((D, F), bf), vm((D, F), bf), vm((D, F), bf),
            vm((DP // 2, 128), u32), vm((D // 2, DP), u32), vm((D // 2, D), u32),
            vm((L // 2, DP), u32), vm((4, 8, 128), f32), vm((4, 128, 128), f32),
            vm((NQ, L // 2, 128), u32), vm((NQ, L // 2, 128), u32),
            vm((NQ, L // 2, 128), u32), vm((NQ, L // 2, 128), u32),
            vm((D // 2, L), u32),
            vm((640, 512), u32), vm((640, 512), u32), vm((16, D, 128), f32),
            vm((D, L), f32), vm((NQ, 80, 128), f32), vm((NQ, 40, 128), u32),
            vm((H, 1, 128), f32), vm((D, 128), f32), vm((8, 128), f32), vm((NSEG, D, L), bf),
            vm((16, 8, 128), f32),
            vm((NSEG, 8, 128), f32), vm((8, 128), f32), vm((D, 128), bf),
            vm((H,), bf), vm((D,), bf),
            pltpu.SemaphoreType.DMA((18,)),
        ],
        compiler_params=pltpu.CompilerParams(vmem_limit_bytes=100 * 1024 * 1024),
        name="infini_moe",
    )(x_t, A_wq, A_wk, A_wv, A_wo, A_beta, B_w_r, B_w_gate, B_w_up, B_w_down.T)
    return out_t.T.reshape(1, S, D)
```

```python
import jax
import jax.numpy as jnp
from jax import lax
from jax.experimental import pallas as pl
from jax.experimental.pallas import tpu as pltpu

S, D, H, DH = 2048, 576, 32, 18
NSEG, L, F = 4, 512, 4608
DP = 640
NQ = 8
QW = 4 * DH
bf, u32, f32, i32 = jnp.bfloat16, jnp.uint32, jnp.float32, jnp.int32
LOG2E = 1.4426950408889634
QSCALE = DH ** -0.5 * LOG2E
MASKB = -1000000000.0 * LOG2E
EPS = 1e-5
NT = (((1,), (1,)), ((), ()))
ONES2 = 0x3F803F80
GU_VPU = 11
DN_VPU = 26
DEN_LO, DEN_HI, WV_MAX = 2.0 ** -60, 2.0 ** 60, 2.0 ** 40


def _tobf(x):
    return pltpu.bitcast(x, bf)


def _tou(x):
    return pltpu.bitcast(x, u32)


def _pack(x):
    return pltpu.bitcast(x.astype(bf), u32)


def _dot(a, b):
    return jnp.dot(a, b, preferred_element_type=f32)


def _dot_nt(a, b):
    return lax.dot_general(a, b, NT, preferred_element_type=f32)


def _phi(t):
    return jnp.where(t > 0, t + 1.0, jnp.exp(t))


def _rowsum(parts):
    acc = [jnp.sum(p.reshape(p.shape[0] // 8, 8, 128), axis=0) for p in parts]
    while len(acc) > 1:
        acc = [acc[i] + acc[i + 1] for i in range(0, len(acc), 2)]
    return jnp.sum(acc[0], axis=0, keepdims=True)


def _ln_stats(rows, w=None):
    d = [rows(144 * g, 144 * (g + 1)) for g in range(4)]
    m1 = _rowsum(d) * (1.0 / D)
    m2 = _rowsum([v * v for v in d]) * (1.0 / D)
    var = jnp.maximum(m2 - m1 * m1, 0.0)
    rstd = lax.rsqrt(var + EPS)
    if w is None:
        return m1, rstd
    dw = _rowsum([d[g] * w[0][144 * g:144 * (g + 1)] for g in range(4)])
    return m1, rstd, (dw - m1 * w[1]) * rstd


def _hi_lo(v):
    hi = v.astype(bf).astype(f32)
    return hi, (v - hi).astype(bf).astype(f32)


def _iota(shape, dim):
    return lax.broadcasted_iota(i32, shape, dim)


def _al(x, n):
    return x if isinstance(x, int) else pl.multiple_of(x, n)


def _kernel(x_hbm, wq_hbm, wk_hbm, wv_hbm, wo_hbm, beta_hbm, wr_hbm,
            wg_hbm, wu_hbm, wd_hbm, out_hbm,
            x_s, wq_s, wk_s, wv_s, wo_s, wg_s, wu_s, wd_s,
            w4_u, wvt_u, wot_u, xn_u, rs_s, rc_s, qx, kx, pqx, pkx, vt_u,
            p0, p1, h_s, ot_s, m_f, m_u, g_s, wr_s, wrs_s, out_s, st_s, best_s, den_s, fin_s,
            beta_ref, wr_ref, sems):
    cp = pltpu.make_async_copy

    def x_copy(s):
        return cp(x_hbm.at[:, pl.ds(_al(s * L, L), L)], x_s.at[s, pl.ds(0, D), :], sems.at[s])

    def out_copy(s):
        return cp(out_s.at[s], out_hbm.at[:, pl.ds(_al(s * L, L), L)], sems.at[11 + s])

    def prep(s, t):
        c = 128 * t
        mean, rstd = _ln_stats(lambda a, b: x_s[s, a:b, pl.ds(c, 128)].astype(f32))
        mh, ml = _hi_lo(mean)
        r16 = _iota((16, 128), 0)
        x_s[s, D:D + 16, pl.ds(c, 128)] = jnp.where(
            r16 < 2, mh, jnp.where(r16 == 2, ml, 0.0)).astype(bf)
        rs_s[t, 0:1] = rstd
        rc_s[t] = jnp.broadcast_to(rstd, (128, 128)).T
        xn_u[pl.ds(64 * t, 64), :] = _tou(x_s[s, :, pl.ds(c, 128)].T)

    def augment(w_ref):
        ones = jnp.ones((16, D), bf)
        hi, lo = _hi_lo(_dot(ones, w_ref[0:D, :])[0:1])
        r16 = _iota((16, D), 0)
        w_ref[D:D + 16, :] = jnp.where((r16 == 0) | (r16 == 2), -hi,
                                       jnp.where(r16 == 1, -lo, 0.0)).astype(bf)

    top = pl.ds(0, D)
    w_copies = [cp(wq_hbm, wq_s.at[top, :], sems.at[4]), cp(wk_hbm, wk_s.at[top, :], sems.at[5]),
                cp(wv_hbm, wv_s.at[top, :], sems.at[6]), cp(wo_hbm, wo_s, sems.at[7])]
    e_copies = [cp(wg_hbm, wg_s, sems.at[8]), cp(wu_hbm, wu_s, sems.at[9]),
                cp(wd_hbm, wd_s, sems.at[10])]

    small = [cp(beta_hbm, beta_ref, sems.at[16]), cp(wr_hbm, wr_ref, sems.at[17])]
    x_copy(0).start()
    w_copies[0].start()
    for c in small:
        c.start()

    m_f[...] = jnp.zeros_like(m_f)
    den_s[...] = jnp.ones_like(den_s)

    for w_ref in (wq_s, wk_s, wv_s):
        w_ref[D + 16:DP, :] = jnp.zeros((DP - D - 16, D), bf)
    for s in range(NSEG):
        x_s[s, D + 16:DP, :] = jnp.zeros((DP - D - 16, L), bf)

    lane1 = _iota((1, 128), 1)
    causal = _iota((128, 128), 0) <= _iota((128, 128), 1)

    def proj_q(t):
        rows = pl.ds(64 * t, 64)
        q = _dot(_tobf(xn_u[rows, :]), wq_s[:, 0:512]) * jnp.concatenate([rc_s[t]] * 4, axis=1)
        tiles = [q[:, 128 * i:128 * (i + 1)] for i in range(4)]
        raw = [_pack(v * QSCALE) for v in tiles]
        ph = [_pack(_phi(v)) for v in tiles]
        for c in range(NQ):
            i = c // 2
            if c % 2 == 0 or c == NQ - 1:
                qx[c, rows, :] = raw[i]
                pqx[c, rows, :] = ph[i]
            else:
                keep = lane1 >= (QW * c) % 128
                qx[c, rows, :] = jnp.where(keep, raw[i], raw[i + 1])
                pqx[c, rows, :] = jnp.where(keep, ph[i], ph[i + 1])

    def proj_k(t):
        rows = pl.ds(64 * t, 64)
        xn = _tobf(xn_u[rows, :])
        rc = rc_s[t]
        k = _dot(xn, wk_s[:, 0:512]) * jnp.concatenate([rc] * 4, axis=1)
        r4 = _dot(xn, _tobf(w4_u[...])) * rc
        tiles = [k[:, 128 * i:128 * (i + 1)] for i in range(4)] + [pltpu.roll(r4, 64, 1)]
        raw = [_pack(v) for v in tiles]
        ph = [_pack(_phi(v)) for v in tiles]
        for c in range(NQ):
            i = c // 2
            if c % 2 == 0:
                kx[c, rows, :] = raw[i]
                pkx[c, rows, :] = ph[i]
            else:
                keep = lane1 >= (QW * c) % 128
                kx[c, rows, :] = jnp.where(keep, raw[i], raw[i + 1])
                pkx[c, rows, :] = jnp.where(keep, ph[i], ph[i + 1])
        keep = lane1 >= (QW * (NQ - 1)) % 128
        qx[NQ - 1, rows, :] = jnp.where(keep, qx[NQ - 1, rows, :], _pack(r4 * QSCALE))
        pqx[NQ - 1, rows, :] = jnp.where(keep, pqx[NQ - 1, rows, :], _pack(_phi(r4)))

    def proj_v(s, t):
        vt = _dot(_tobf(wvt_u[...]), x_s[s, :, pl.ds(128 * t, 128)]) * rs_s[t, 0:1]
        vt_u[:, pl.ds(128 * t, 128)] = _pack(vt)

    def masked_q(k, par, j):
        q = qx[2 * k + par, pl.ds(64 * j, 64), :]
        out = []
        for i in range(4):
            st = (2 * QW * k + QW * par + DH * i) % 128
            out.append(q & jnp.where(((lane1 - st) & 127) < DH, jnp.uint32(0xFFFFFFFF),
                                     jnp.uint32(0)))
        return out

    def scores(k, par, j):
        qm = _tobf(jnp.concatenate(masked_q(k, par, j), axis=0))
        kk = _tobf(kx[2 * k + par, pl.ds(0, 64 * (j + 1)), :])
        return _dot_nt(kk, qm)

    r64, l64 = _iota((64, 128), 0), _iota((64, 128), 1)
    lo_nat = (l64 >= 64) | (r64 <= l64)
    lo_swp = (l64 < 64) | (r64 <= l64 - 64)
    hi_even = (l64 < 64) & (r64 <= l64)
    hi_odd = (l64 >= 64) & (r64 <= l64 - 64)

    def stage_a(k, par, j, p_ref):
        c = 2 * k + par
        qm = masked_q(k, par, j)
        w1 = [jnp.concatenate([qm[i][32:], qm[i][:32]], axis=0) if i % 2 == 0 else qm[i]
              for i in range(4)]
        w2 = [qm[i][32:] for i in range(4)]
        n1 = 128 * j + 64
        p1 = jnp.exp2(_dot_nt(_tobf(kx[c, pl.ds(0, n1 // 2), :]),
                              _tobf(jnp.concatenate(w1, axis=0))))
        p2 = jnp.exp2(_dot_nt(_tobf(kx[c, pl.ds(n1 // 2, 32), :]),
                              _tobf(jnp.concatenate(w2, axis=0))))
        off = 64 * (j * (j + 1) // 2)
        if j > 0:
            p_ref[pl.ds(off, 64 * j), :] = _pack(p1[:128 * j])
        lo = [jnp.where(lo_swp if i % 2 == 0 else lo_nat,
                        p1[128 * j:, 128 * i:128 * (i + 1)], 0.0) for i in range(4)]
        hi = [jnp.where(hi_even if i % 2 == 0 else hi_odd,
                        p2[:, 128 * (i // 2):128 * (i // 2 + 1)], 0.0) for i in range(4)]
        p_ref[pl.ds(off + 64 * j, 32), :] = _pack(jnp.concatenate(lo, axis=1))
        p_ref[pl.ds(off + 64 * j + 32, 32), :] = _pack(jnp.concatenate(hi, axis=1))

    def stage_a_safe(k, par, j, p_ref):
        s = scores(k, par, j)
        bias = jnp.where(causal, 0.0, MASKB).astype(f32)
        sd = s[128 * j:] + jnp.concatenate([bias] * 4, axis=1)
        s = sd if j == 0 else jnp.concatenate([s[:128 * j], sd], axis=0)
        p = jnp.exp2(s - jnp.max(s, axis=0, keepdims=True))
        p_ref[pl.ds(64 * (j * (j + 1) // 2), 64 * (j + 1)), :] = _pack(p)

    def stage_b(use_mem, k, par, j, p_ref, swapped=True):
        c = 2 * k + par
        base = QW * par
        mwin = base - base % 16
        moff = base - mwin
        zrow = 72 if moff == 0 else 0
        srow = _iota((8, 128), 0)
        grow = [g_s[4 * c + i] for i in range(4)]
        off = 64 * (j * (j + 1) // 2)
        if use_mem:
            mem = _dot_nt(_tobf(m_u[c]), _tobf(pqx[c, pl.ds(64 * j, 64), :]))
        accs, rds, rms = [], [], []
        dlo, dhi = den_s[0:1], den_s[1:2]
        for i in range(4):
            r0 = base + DH * i
            w = r0 - r0 % 16
            o = r0 - w
            vt = vt_u[pl.ds(_al(QW * k + w // 2, 8), 16), pl.ds(0, 128 * (j + 1))]
            orow = 15 if o < 14 else 0
            vt = jnp.where(_iota(vt.shape, 0) == orow, jnp.uint32(ONES2), vt)
            p = _tobf(p_ref[pl.ds(off, 64 * (j + 1)), pl.ds(128 * i, 128)])
            acc = _dot(_tobf(vt), p)
            if swapped and i % 2 == 0:
                acc = pltpu.roll(acc, 64, 1)
            den = acc[2 * orow:2 * orow + 1]
            dlo, dhi = jnp.minimum(dlo, den), jnp.maximum(dhi, den)
            rds.append((1.0 - grow[i]) / den)
            if use_mem:
                rms.append(grow[i] / (mem[zrow + i:zrow + i + 1] + 1e-6))
            a0 = o - o % 8
            accs.append(acc[a0:a0 + 24])
        den_s[0:1] = dlo
        den_s[1:2] = dhi
        for v in range(9):
            lo_h, hi_h = (8 * v) // DH, (8 * v + 7) // DH

            def piece(h):
                a = accs[h][8 * (v - (DH * h) // 8):8 * (v - (DH * h) // 8) + 8]
                if not use_mem:
                    return a * rds[h]
                return a * rds[h] + mem[moff + 8 * v:moff + 8 * v + 8] * rms[h]
            val = piece(lo_h)
            if hi_h != lo_h:
                val = jnp.where(srow < DH * hi_h - 8 * v, val, piece(hi_h))
            ot_s[pl.ds(_al(2 * QW * k + base + 8 * v, 8), 8), pl.ds(128 * j, 128)] = val

    def mem_update(k, par):
        c = 2 * k + par
        base = QW * par
        mwin = base - base % 16
        moff = base - mwin
        zrow = 72 if moff == 0 else 0
        vw = vt_u[pl.ds(_al(QW * k + mwin // 2, 8), 40), :]
        rr = _iota(vw.shape, 0)
        isz = (rr >= 36) if moff == 0 else (rr < 4)
        vw = jnp.where(isz, jnp.uint32(ONES2), vw)
        upd = _dot(_tobf(vw), _tobf(pkx[c]))
        r80 = _iota((80, 128), 0)
        l80 = (_iota((80, 128), 1) - (2 * QW * k + base)) & 127
        hrow = jnp.where((r80 >= zrow) & (r80 < zrow + 8), r80 - zrow, (r80 - moff) // DH)
        keep = (l80 >= DH * hrow) & (l80 < DH * hrow + DH) & (hrow < 4) & (hrow >= 0)
        mnew = m_f[c] + jnp.where(keep, upd, 0.0)
        m_f[c] = mnew
        m_u[c] = _pack(mnew)

    pb = (p0, p1)

    def step(use_mem, update, a, b):
        for j in range(4):
            if b is not None:
                stage_b(use_mem, b[0], b[1], j, pb[b[1]])
                if j == 3 and update:
                    mem_update(b[0], b[1])
            if a is not None:
                stage_a(a[0], a[1], j, pb[a[1]])

    def out_proj(s, t):
        c = 128 * t
        o = ot_s[:, pl.ds(c, 128)].astype(bf)
        h = x_s[s, 0:D, pl.ds(c, 128)].astype(f32) + _dot(_tobf(wot_u[...]), o)
        h_s[4 * s + t] = h
        mean, rstd, sc = _ln_stats(lambda a, b: h[a:b], (wr_s[...], wrs_s[0:1]))
        st_s[4 * s + t, 0:1] = mean
        st_s[4 * s + t, 1:2] = rstd
        smax = jnp.max(sc, axis=1, keepdims=True)
        pos = (lane1 + (s * L + c)).astype(f32)
        sidx = jnp.min(jnp.where(sc == smax, pos, 1e9), axis=1, keepdims=True)
        new = jnp.concatenate([jnp.broadcast_to(smax, (1, 128)), jnp.broadcast_to(sidx, (1, 128)),
                               jnp.zeros((6, 128), f32)], axis=0)
        if t == 0:
            best_s[s] = new
        else:
            old = best_s[s]
            best_s[s] = jnp.where(smax > old[0:1, 0:1], new, old)

    def post(s, t):
        rstd = st_s[4 * s + t, 1:2]
        a = 1.0 + rstd
        b = st_s[4 * s + t, 0:1] * rstd
        out_s[s, :, pl.ds(128 * t, 128)] = (h_s[4 * s + t] * a - b).astype(bf)

    def finish(s):
        for t in range(4):
            out_proj(s, t)
            if t < 3:
                post(s, t)

    def attention(s):
        use_mem, update = s > 0, s < NSEG - 1
        step(use_mem, update, (0, 0), None)
        for k in range(NQ // 2):
            step(use_mem, update, (k, 1), (k, 0))
            step(use_mem, update, (k + 1, 0) if k + 1 < NQ // 2 else None, (k, 1))

    x_copy(0).wait()
    w_copies[1].start()
    for t in range(4):
        prep(0, t)
    w_copies[0].wait()
    w_copies[2].start()
    augment(wq_s)
    for t in range(4):
        proj_q(t)
    w_copies[1].wait()
    w_copies[3].start()
    for s in range(1, NSEG):
        x_copy(s).start()
    augment(wk_s)
    w4_u[...] = _tou(jnp.concatenate([wq_s[:, 512:D], wk_s[:, 512:D]], axis=1))
    for t in range(2):
        proj_k(t)
    w_copies[2].wait()
    for c in e_copies:
        c.start()
    augment(wv_s)
    wvt_u[...] = _tou(wv_s[...].T)
    wv_ok = jnp.max(jnp.abs(wv_s[0:D, :].astype(f32))) < WV_MAX
    for t in range(2, 4):
        proj_k(t)
    w_copies[3].wait()
    for c in small:
        c.wait()
    g32 = jax.nn.sigmoid(beta_ref[...].astype(f32)).reshape(1, H)
    sel = _iota((H, H), 1) == _iota((H, H), 0)
    gcol = jnp.sum(jnp.where(sel, g32, 0.0), axis=1, keepdims=True)
    for h in range(H):
        g_s[h] = jnp.broadcast_to(gcol[h:h + 1], (1, 128))
    wr_s[...] = jnp.broadcast_to(wr_ref[...].astype(f32).reshape(1, D), (128, D)).T
    wrs_s[...] = jnp.broadcast_to(jnp.sum(wr_s[...], axis=0, keepdims=True), (8, 128))
    wot_u[...] = _tou(wo_s[...].T)
    for t in range(4):
        proj_v(0, t)
    attention(0)
    for s in range(1, NSEG):
        x_copy(s).wait()
    finish(0)

    for s in range(1, NSEG):
        post(s - 1, 3)
        for t in range(4):
            prep(s, t)
        for t in range(4):
            proj_v(s, t)
        for t in range(4):
            proj_q(t)
            proj_k(t)
        out_copy(s - 1).start()
        attention(s)
        finish(s)
    post(NSEG - 1, 3)
    out_copy(NSEG - 1).start()

    dl = den_s[...]
    safe = jnp.logical_and(jnp.min(dl[0:1]) >= DEN_LO, jnp.max(dl[1:2]) <= DEN_HI)
    safe = jnp.logical_and(safe, wv_ok)

    @pl.when(jnp.logical_not(safe))
    def _():
        for s in range(NSEG):
            out_copy(s).wait()
        m_f[...] = jnp.zeros_like(m_f)
        m_u[...] = jnp.zeros_like(m_u)

        def seg_redo(s, carry):
            for t in range(4):
                prep(s, t)
                proj_v(s, t)
                proj_q(t)
                proj_k(t)

            def quads(k, carry):
                for par in range(2):
                    for j in range(4):
                        stage_a_safe(k, par, j, pb[par])
                        stage_b(True, k, par, j, pb[par], swapped=False)
                    mem_update(k, par)
                return carry
            lax.fori_loop(0, NQ // 2, quads, 0)
            finish(s)
            post(s, 3)
            out_copy(s).start()
            return carry
        lax.fori_loop(0, NSEG, seg_redo, 0)

    for c in e_copies:
        c.wait()
    best = best_s[0]
    for s in range(1, NSEG):
        cand = best_s[s]
        best = jnp.where(cand[0:1, 0:1] > best[0:1, 0:1], cand, best)
    idx = jnp.clip(best[1, 0].astype(i32), 0, S - 1)
    blk = idx // 128
    col = idx - blk * 128
    onehot = ((_iota((16, 128), 1) == col) & (_iota((16, 128), 0) == 0)).astype(bf)
    ln = ((h_s[blk] - st_s[blk, 0:1]) * st_s[blk, 1:2]).astype(bf)
    xs = _dot_nt(onehot, ln).astype(bf)
    pick = (_iota((128, 128), 0) == col).astype(bf)
    xcol = _dot(ln, pick)
    fm = F - 128 * GU_VPU

    def first_layer(w_ref):
        acc = jnp.zeros((8, 128 * GU_VPU), f32)
        for i in range(D // 8):
            w = w_ref[8 * i:8 * i + 8, fm:F].astype(f32)
            acc = acc + w * jnp.concatenate([xcol[8 * i:8 * i + 8]] * GU_VPU, axis=1)
        return jnp.concatenate([_dot(xs, w_ref[:, 0:fm])[0:1],
                                jnp.sum(acc, axis=0, keepdims=True)], axis=1)
    gate = first_layer(wg_s)
    up = first_layer(wu_s)
    act = (gate * jax.nn.sigmoid(gate) * up).astype(bf)
    actf = act.astype(f32)
    fd = F - 128 * DN_VPU
    y = _dot_nt(jnp.broadcast_to(act[:, 0:fd], (16, fd)), wd_s[:, 0:fd])
    parts = []
    for i in range(D // 8):
        w = wd_s[8 * i:8 * i + 8, fd:F].astype(f32) * actf[:, fd:F]
        tot = w[:, 0:128]
        for c in range(1, DN_VPU):
            tot = tot + w[:, 128 * c:128 * (c + 1)]
        parts.append(tot)
    yv = jnp.sum(jnp.concatenate(parts, axis=0), axis=1, keepdims=True)
    yt = (jnp.broadcast_to(y[0:1], (128, D)).T + yv) * jax.nn.sigmoid(best[0:1, 0:1])
    for s in range(NSEG):
        out_copy(s).wait()
    seg = blk // 4
    c0 = pl.multiple_of((blk - seg * 4) * 128, 128)
    cur = out_s[seg, :, pl.ds(c0, 128)].astype(f32)
    hit = _iota((D, 128), 1) == col
    fin_s[...] = (cur + jnp.where(hit, yt, 0.0)).astype(bf)
    fin = cp(fin_s, out_hbm.at[:, pl.ds(pl.multiple_of(blk * 128, 128), 128)], sems.at[15])
    fin.start()
    fin.wait()


@jax.jit
def pallas_sequential_preLN__memory_aug_infini_attn__moe_arch_mod__prompt_kernel(
    A_x, A_wq, A_wk, A_wv, A_wo, A_beta, B_x, B_w_r, B_w_gate, B_w_up, B_w_down,
):
    hbm = pl.BlockSpec(memory_space=pltpu.HBM)
    vm = pltpu.VMEM
    x_t = A_x.reshape(S, D).T
    out_t = pl.pallas_call(
        _kernel,
        out_shape=jax.ShapeDtypeStruct((D, S), bf),
        in_specs=[hbm] * 10,
        out_specs=hbm,
        scratch_shapes=[
            vm((NSEG, DP, L), bf), vm((DP, D), bf), vm((DP, D), bf), vm((DP, D), bf), vm((D, D), bf),
            vm((D, F), bf), vm((D, F), bf), vm((D, F), bf),
            vm((DP // 2, 128), u32), vm((D // 2, DP), u32), vm((D // 2, D), u32),
            vm((L // 2, DP), u32), vm((4, 8, 128), f32), vm((4, 128, 128), f32),
            vm((NQ, L // 2, 128), u32), vm((NQ, L // 2, 128), u32),
            vm((NQ, L // 2, 128), u32), vm((NQ, L // 2, 128), u32),
            vm((D // 2, L), u32),
            vm((640, 512), u32), vm((640, 512), u32), vm((16, D, 128), f32),
            vm((D, L), f32), vm((NQ, 80, 128), f32), vm((NQ, 40, 128), u32),
            vm((H, 1, 128), f32), vm((D, 128), f32), vm((8, 128), f32), vm((NSEG, D, L), bf),
            vm((16, 8, 128), f32),
            vm((NSEG, 8, 128), f32), vm((8, 128), f32), vm((D, 128), bf),
            vm((H,), bf), vm((D,), bf),
            pltpu.SemaphoreType.DMA((18,)),
        ],
        compiler_params=pltpu.CompilerParams(vmem_limit_bytes=100 * 1024 * 1024),
        name="infini_moe",
    )(x_t, A_wq, A_wk, A_wv, A_wo, A_beta, B_w_r, B_w_gate, B_w_up, B_w_down.T)
    return out_t.T.reshape(1, S, D)
```

```python
import jax
import jax.numpy as jnp
from jax import lax
from jax.experimental import pallas as pl
from jax.experimental.pallas import tpu as pltpu

S, D, H, DH = 2048, 576, 32, 18
NSEG, L, F = 4, 512, 4608
DP = 640
NQ = 8
QW = 4 * DH
bf, u32, f32, i32 = jnp.bfloat16, jnp.uint32, jnp.float32, jnp.int32
LOG2E = 1.4426950408889634
QSCALE = DH ** -0.5 * LOG2E
MASKB = -1000000000.0 * LOG2E
EPS = 1e-5
NT = (((1,), (1,)), ((), ()))
ONES2 = 0x3F803F80
GU_VPU = 11
DN_VPU = 26
DEN_LO, DEN_HI, WV_MAX = 2.0 ** -60, 2.0 ** 60, 2.0 ** 40


def _tobf(x):
    return pltpu.bitcast(x, bf)


def _tou(x):
    return pltpu.bitcast(x, u32)


def _pack(x):
    return pltpu.bitcast(x.astype(bf), u32)


def _dot(a, b):
    return jnp.dot(a, b, preferred_element_type=f32)


def _dot_nt(a, b):
    return lax.dot_general(a, b, NT, preferred_element_type=f32)


def _phi(t):
    return jnp.where(t > 0, t + 1.0, jnp.exp(t))


def _rowsum(parts):
    acc = [jnp.sum(p.reshape(p.shape[0] // 8, 8, 128), axis=0) for p in parts]
    while len(acc) > 1:
        acc = [acc[i] + acc[i + 1] for i in range(0, len(acc), 2)]
    return jnp.sum(acc[0], axis=0, keepdims=True)


def _ln_stats(rows, w=None):
    d = [rows(144 * g, 144 * (g + 1)) for g in range(4)]
    m1 = _rowsum(d) * (1.0 / D)
    m2 = _rowsum([v * v for v in d]) * (1.0 / D)
    var = jnp.maximum(m2 - m1 * m1, 0.0)
    rstd = lax.rsqrt(var + EPS)
    if w is None:
        return m1, rstd
    dw = _rowsum([d[g] * w[0][144 * g:144 * (g + 1)] for g in range(4)])
    return m1, rstd, (dw - m1 * w[1]) * rstd


def _hi_lo(v):
    hi = v.astype(bf).astype(f32)
    return hi, (v - hi).astype(bf).astype(f32)


def _iota(shape, dim):
    return lax.broadcasted_iota(i32, shape, dim)


def _al(x, n):
    return x if isinstance(x, int) else pl.multiple_of(x, n)


def _kernel(x_hbm, wq_hbm, wk_hbm, wv_hbm, wo_hbm, beta_hbm, wr_hbm,
            wg_hbm, wu_hbm, wd_hbm, out_hbm,
            x_s, wq_s, wk_s, wv_s, wo_s, wg_s, wu_s, wd_s,
            w4_u, wvt_u, wot_u, xn_u, rs_s, rc_s, qx, kx, pqx, pkx, vt_u,
            p0, p1, h_s, ot_s, m_f, m_u, g_s, wr_s, wrs_s, out_s, st_s, best_s, den_s, fin_s,
            beta_ref, wr_ref, sems):
    cp = pltpu.make_async_copy

    def x_copy(s):
        return cp(x_hbm.at[:, pl.ds(_al(s * L, L), L)], x_s.at[s, pl.ds(0, D), :], sems.at[s])

    def out_copy(s):
        return cp(out_s.at[s], out_hbm.at[:, pl.ds(_al(s * L, L), L)], sems.at[11 + s])

    def prep(s, t):
        c = 128 * t
        mean, rstd = _ln_stats(lambda a, b: x_s[s, a:b, pl.ds(c, 128)].astype(f32))
        mh, ml = _hi_lo(mean)
        r16 = _iota((16, 128), 0)
        x_s[s, D:D + 16, pl.ds(c, 128)] = jnp.where(
            r16 < 2, mh, jnp.where(r16 == 2, ml, 0.0)).astype(bf)
        rs_s[t, 0:1] = rstd
        rc_s[t] = jnp.broadcast_to(rstd, (128, 128)).T
        xn_u[pl.ds(64 * t, 64), :] = _tou(x_s[s, :, pl.ds(c, 128)].T)

    def augment(w_ref):
        ones = jnp.ones((16, D), bf)
        hi, lo = _hi_lo(_dot(ones, w_ref[0:D, :])[0:1])
        r16 = _iota((16, D), 0)
        w_ref[D:D + 16, :] = jnp.where((r16 == 0) | (r16 == 2), -hi,
                                       jnp.where(r16 == 1, -lo, 0.0)).astype(bf)

    top = pl.ds(0, D)
    w_copies = [cp(wq_hbm, wq_s.at[top, :], sems.at[4]), cp(wk_hbm, wk_s.at[top, :], sems.at[5]),
                cp(wv_hbm, wv_s.at[top, :], sems.at[6]), cp(wo_hbm, wo_s, sems.at[7])]
    e_copies = [cp(wg_hbm, wg_s, sems.at[8]), cp(wu_hbm, wu_s, sems.at[9]),
                cp(wd_hbm, wd_s, sems.at[10])]

    small = [cp(beta_hbm, beta_ref, sems.at[16]), cp(wr_hbm, wr_ref, sems.at[17])]
    x_copy(0).start()
    w_copies[0].start()
    for c in small:
        c.start()

    m_f[...] = jnp.zeros_like(m_f)
    den_s[...] = jnp.ones_like(den_s)

    for w_ref in (wq_s, wk_s, wv_s):
        w_ref[D + 16:DP, :] = jnp.zeros((DP - D - 16, D), bf)
    for s in range(NSEG):
        x_s[s, D + 16:DP, :] = jnp.zeros((DP - D - 16, L), bf)

    lane1 = _iota((1, 128), 1)
    causal = _iota((128, 128), 0) <= _iota((128, 128), 1)

    def proj_q(t):
        rows = pl.ds(64 * t, 64)
        q = _dot(_tobf(xn_u[rows, :]), wq_s[:, 0:512]) * jnp.concatenate([rc_s[t]] * 4, axis=1)
        tiles = [q[:, 128 * i:128 * (i + 1)] for i in range(4)]
        raw = [_pack(v * QSCALE) for v in tiles]
        ph = [_pack(_phi(v)) for v in tiles]
        for c in range(NQ):
            i = c // 2
            if c % 2 == 0 or c == NQ - 1:
                qx[c, rows, :] = raw[i]
                pqx[c, rows, :] = ph[i]
            else:
                keep = lane1 >= (QW * c) % 128
                qx[c, rows, :] = jnp.where(keep, raw[i], raw[i + 1])
                pqx[c, rows, :] = jnp.where(keep, ph[i], ph[i + 1])

    def proj_k(t):
        rows = pl.ds(64 * t, 64)
        xn = _tobf(xn_u[rows, :])
        rc = rc_s[t]
        k = _dot(xn, wk_s[:, 0:512]) * jnp.concatenate([rc] * 4, axis=1)
        r4 = _dot(xn, _tobf(w4_u[...])) * rc
        tiles = [k[:, 128 * i:128 * (i + 1)] for i in range(4)] + [pltpu.roll(r4, 64, 1)]
        raw = [_pack(v) for v in tiles]
        ph = [_pack(_phi(v)) for v in tiles]
        for c in range(NQ):
            i = c // 2
            if c % 2 == 0:
                kx[c, rows, :] = raw[i]
                pkx[c, rows, :] = ph[i]
            else:
                keep = lane1 >= (QW * c) % 128
                kx[c, rows, :] = jnp.where(keep, raw[i], raw[i + 1])
                pkx[c, rows, :] = jnp.where(keep, ph[i], ph[i + 1])
        keep = lane1 >= (QW * (NQ - 1)) % 128
        qx[NQ - 1, rows, :] = jnp.where(keep, qx[NQ - 1, rows, :], _pack(r4 * QSCALE))
        pqx[NQ - 1, rows, :] = jnp.where(keep, pqx[NQ - 1, rows, :], _pack(_phi(r4)))

    def proj_v(s, t):
        vt = _dot(_tobf(wvt_u[...]), x_s[s, :, pl.ds(128 * t, 128)]) * rs_s[t, 0:1]
        vt_u[:, pl.ds(128 * t, 128)] = _pack(vt)

    def masked_q(k, par, j):
        q = qx[2 * k + par, pl.ds(64 * j, 64), :]
        out = []
        for i in range(4):
            st = (2 * QW * k + QW * par + DH * i) % 128
            out.append(q & jnp.where(((lane1 - st) & 127) < DH, jnp.uint32(0xFFFFFFFF),
                                     jnp.uint32(0)))
        return out

    def scores(k, par, j):
        qm = _tobf(jnp.concatenate(masked_q(k, par, j), axis=0))
        kk = _tobf(kx[2 * k + par, pl.ds(0, 64 * (j + 1)), :])
        return _dot_nt(kk, qm)

    r64, l64 = _iota((64, 128), 0), _iota((64, 128), 1)
    lo_nat = (l64 >= 64) | (r64 <= l64)
    lo_swp = (l64 < 64) | (r64 <= l64 - 64)
    hi_even = (l64 < 64) & (r64 <= l64)
    hi_odd = (l64 >= 64) & (r64 <= l64 - 64)

    def stage_a(k, par, j, p_ref):
        c = 2 * k + par
        qm = masked_q(k, par, j)
        w1 = [jnp.concatenate([qm[i][32:], qm[i][:32]], axis=0) if i % 2 == 0 else qm[i]
              for i in range(4)]
        w2 = [qm[i][32:] for i in range(4)]
        n1 = 128 * j + 64
        p1 = jnp.exp2(_dot_nt(_tobf(kx[c, pl.ds(0, n1 // 2), :]),
                              _tobf(jnp.concatenate(w1, axis=0))))
        p2 = jnp.exp2(_dot_nt(_tobf(kx[c, pl.ds(n1 // 2, 32), :]),
                              _tobf(jnp.concatenate(w2, axis=0))))
        off = 64 * (j * (j + 1) // 2)
        if j > 0:
            p_ref[pl.ds(off, 64 * j), :] = _pack(p1[:128 * j])
        lo = [jnp.where(lo_swp if i % 2 == 0 else lo_nat,
                        p1[128 * j:, 128 * i:128 * (i + 1)], 0.0) for i in range(4)]
        hi = [jnp.where(hi_even if i % 2 == 0 else hi_odd,
                        p2[:, 128 * (i // 2):128 * (i // 2 + 1)], 0.0) for i in range(4)]
        p_ref[pl.ds(off + 64 * j, 32), :] = _pack(jnp.concatenate(lo, axis=1))
        p_ref[pl.ds(off + 64 * j + 32, 32), :] = _pack(jnp.concatenate(hi, axis=1))

    def stage_a_safe(k, par, j, p_ref):
        s = scores(k, par, j)
        bias = jnp.where(causal, 0.0, MASKB).astype(f32)
        sd = s[128 * j:] + jnp.concatenate([bias] * 4, axis=1)
        s = sd if j == 0 else jnp.concatenate([s[:128 * j], sd], axis=0)
        p = jnp.exp2(s - jnp.max(s, axis=0, keepdims=True))
        p_ref[pl.ds(64 * (j * (j + 1) // 2), 64 * (j + 1)), :] = _pack(p)

    def stage_b(use_mem, oslot, k, par, j, p_ref, swapped=True):
        c = 2 * k + par
        base = QW * par
        mwin = base - base % 16
        moff = base - mwin
        zrow = 72 if moff == 0 else 0
        srow = _iota((8, 128), 0)
        grow = [g_s[4 * c + i] for i in range(4)]
        off = 64 * (j * (j + 1) // 2)
        if use_mem:
            mem = _dot_nt(_tobf(m_u[c]), _tobf(pqx[c, pl.ds(64 * j, 64), :]))
        accs, rds, rms = [], [], []
        dlo, dhi = den_s[0:1], den_s[1:2]
        for i in range(4):
            r0 = base + DH * i
            w = r0 - r0 % 16
            o = r0 - w
            vt = vt_u[pl.ds(_al(QW * k + w // 2, 8), 16), pl.ds(0, 128 * (j + 1))]
            orow = 15 if o < 14 else 0
            vt = jnp.where(_iota(vt.shape, 0) == orow, jnp.uint32(ONES2), vt)
            p = _tobf(p_ref[pl.ds(off, 64 * (j + 1)), pl.ds(128 * i, 128)])
            acc = _dot(_tobf(vt), p)
            if swapped and i % 2 == 0:
                acc = pltpu.roll(acc, 64, 1)
            den = acc[2 * orow:2 * orow + 1]
            dlo, dhi = jnp.minimum(dlo, den), jnp.maximum(dhi, den)
            rds.append((1.0 - grow[i]) / den)
            if use_mem:
                rms.append(grow[i] / (mem[zrow + i:zrow + i + 1] + 1e-6))
            a0 = o - o % 8
            accs.append(acc[a0:a0 + 24])
        den_s[0:1] = dlo
        den_s[1:2] = dhi
        for v in range(9):
            lo_h, hi_h = (8 * v) // DH, (8 * v + 7) // DH

            def piece(h):
                a = accs[h][8 * (v - (DH * h) // 8):8 * (v - (DH * h) // 8) + 8]
                if not use_mem:
                    return a * rds[h]
                return a * rds[h] + mem[moff + 8 * v:moff + 8 * v + 8] * rms[h]
            val = piece(lo_h)
            if hi_h != lo_h:
                val = jnp.where(srow < DH * hi_h - 8 * v, val, piece(hi_h))
            ot_s[oslot, pl.ds(_al(2 * QW * k + base + 8 * v, 8), 8), pl.ds(128 * j, 128)] = val

    def mem_update(k, par):
        c = 2 * k + par
        base = QW * par
        mwin = base - base % 16
        moff = base - mwin
        zrow = 72 if moff == 0 else 0
        vw = vt_u[pl.ds(_al(QW * k + mwin // 2, 8), 40), :]
        rr = _iota(vw.shape, 0)
        isz = (rr >= 36) if moff == 0 else (rr < 4)
        vw = jnp.where(isz, jnp.uint32(ONES2), vw)
        upd = _dot(_tobf(vw), _tobf(pkx[c]))
        r80 = _iota((80, 128), 0)
        l80 = (_iota((80, 128), 1) - (2 * QW * k + base)) & 127
        hrow = jnp.where((r80 >= zrow) & (r80 < zrow + 8), r80 - zrow, (r80 - moff) // DH)
        keep = (l80 >= DH * hrow) & (l80 < DH * hrow + DH) & (hrow < 4) & (hrow >= 0)
        mnew = m_f[c] + jnp.where(keep, upd, 0.0)
        m_f[c] = mnew
        m_u[c] = _pack(mnew)

    pb = (p0, p1)

    def step(use_mem, update, oslot, a, b):
        for j in range(4):
            if b is not None:
                stage_b(use_mem, oslot, b[0], b[1], j, pb[b[1]])
                if j == 3 and update:
                    mem_update(b[0], b[1])
            if a is not None:
                stage_a(a[0], a[1], j, pb[a[1]])

    def out_proj(s, t):
        c = 128 * t
        o = ot_s[s % 2, :, pl.ds(c, 128)].astype(bf)
        h = x_s[s, 0:D, pl.ds(c, 128)].astype(f32) + _dot(_tobf(wot_u[...]), o)
        h_s[4 * s + t] = h
        mean, rstd, sc = _ln_stats(lambda a, b: h[a:b], (wr_s[...], wrs_s[0:1]))
        st_s[4 * s + t, 0:1] = mean
        st_s[4 * s + t, 1:2] = rstd
        smax = jnp.max(sc, axis=1, keepdims=True)
        pos = (lane1 + (s * L + c)).astype(f32)
        sidx = jnp.min(jnp.where(sc == smax, pos, 1e9), axis=1, keepdims=True)
        new = jnp.concatenate([jnp.broadcast_to(smax, (1, 128)), jnp.broadcast_to(sidx, (1, 128)),
                               jnp.zeros((6, 128), f32)], axis=0)
        if t == 0:
            best_s[s] = new
        else:
            old = best_s[s]
            best_s[s] = jnp.where(smax > old[0:1, 0:1], new, old)

    def post(s, t):
        rstd = st_s[4 * s + t, 1:2]
        a = 1.0 + rstd
        b = st_s[4 * s + t, 0:1] * rstd
        out_s[s, :, pl.ds(128 * t, 128)] = (h_s[4 * s + t] * a - b).astype(bf)

    def finish(s):
        for t in range(4):
            out_proj(s, t)
            if t < 3:
                post(s, t)

    def attention(s):
        use_mem, update, o = s > 0, s < NSEG - 1, s % 2
        step(use_mem, update, o, (0, 0), None)
        for k in range(NQ // 2):
            step(use_mem, update, o, (k, 1), (k, 0))
            if s > 0:
                out_proj(s - 1, k)
                post(s - 1, k)
            step(use_mem, update, o, (k + 1, 0) if k + 1 < NQ // 2 else None, (k, 1))
        if s > 0:
            out_copy(s - 1).start()

    x_copy(0).wait()
    w_copies[1].start()
    for t in range(4):
        prep(0, t)
    w_copies[0].wait()
    w_copies[2].start()
    augment(wq_s)
    for t in range(4):
        proj_q(t)
    w_copies[1].wait()
    w_copies[3].start()
    for s in range(1, NSEG):
        x_copy(s).start()
    augment(wk_s)
    w4_u[...] = _tou(jnp.concatenate([wq_s[:, 512:D], wk_s[:, 512:D]], axis=1))
    for t in range(2):
        proj_k(t)
    w_copies[2].wait()
    augment(wv_s)
    wvt_u[...] = _tou(wv_s[...].T)
    wv_ok = jnp.max(jnp.abs(wv_s[0:D, :].astype(f32))) < WV_MAX
    for t in range(2, 4):
        proj_k(t)
    w_copies[3].wait()
    for c in small:
        c.wait()
    g32 = jax.nn.sigmoid(beta_ref[...].astype(f32)).reshape(1, H)
    sel = _iota((H, H), 1) == _iota((H, H), 0)
    gcol = jnp.sum(jnp.where(sel, g32, 0.0), axis=1, keepdims=True)
    for h in range(H):
        g_s[h] = jnp.broadcast_to(gcol[h:h + 1], (1, 128))
    wr_s[...] = jnp.broadcast_to(wr_ref[...].astype(f32).reshape(1, D), (128, D)).T
    wrs_s[...] = jnp.broadcast_to(jnp.sum(wr_s[...], axis=0, keepdims=True), (8, 128))
    wot_u[...] = _tou(wo_s[...].T)
    for t in range(4):
        proj_v(0, t)
    attention(0)
    for s in range(1, NSEG):
        x_copy(s).wait()

    for s in range(1, NSEG):
        e_copies[s - 1].start()
        for t in range(4):
            prep(s, t)
        for t in range(4):
            proj_v(s, t)
        for t in range(4):
            proj_q(t)
            proj_k(t)
        attention(s)
    finish(NSEG - 1)
    post(NSEG - 1, 3)
    out_copy(NSEG - 1).start()

    dl = den_s[...]
    safe = jnp.logical_and(jnp.min(dl[0:1]) >= DEN_LO, jnp.max(dl[1:2]) <= DEN_HI)
    safe = jnp.logical_and(safe, wv_ok)

    @pl.when(jnp.logical_not(safe))
    def _():
        for s in range(NSEG):
            out_copy(s).wait()
        m_f[...] = jnp.zeros_like(m_f)
        m_u[...] = jnp.zeros_like(m_u)

        def seg_redo(s, carry):
            for t in range(4):
                prep(s, t)
                proj_v(s, t)
                proj_q(t)
                proj_k(t)

            def quads(k, carry):
                for par in range(2):
                    for j in range(4):
                        stage_a_safe(k, par, j, pb[par])
                        stage_b(True, s % 2, k, par, j, pb[par], swapped=False)
                    mem_update(k, par)
                return carry
            lax.fori_loop(0, NQ // 2, quads, 0)
            finish(s)
            post(s, 3)
            out_copy(s).start()
            return carry
        lax.fori_loop(0, NSEG, seg_redo, 0)

    for c in e_copies:
        c.wait()
    best = best_s[0]
    for s in range(1, NSEG):
        cand = best_s[s]
        best = jnp.where(cand[0:1, 0:1] > best[0:1, 0:1], cand, best)
    idx = jnp.clip(best[1, 0].astype(i32), 0, S - 1)
    blk = idx // 128
    col = idx - blk * 128
    onehot = ((_iota((16, 128), 1) == col) & (_iota((16, 128), 0) == 0)).astype(bf)
    ln = ((h_s[blk] - st_s[blk, 0:1]) * st_s[blk, 1:2]).astype(bf)
    xs = _dot_nt(onehot, ln).astype(bf)
    pick = (_iota((128, 128), 0) == col).astype(bf)
    xcol = _dot(ln, pick)
    fm = F - 128 * GU_VPU

    def first_layer(w_ref):
        acc = jnp.zeros((8, 128 * GU_VPU), f32)
        for i in range(D // 8):
            w = w_ref[8 * i:8 * i + 8, fm:F].astype(f32)
            acc = acc + w * jnp.concatenate([xcol[8 * i:8 * i + 8]] * GU_VPU, axis=1)
        return jnp.concatenate([_dot(xs, w_ref[:, 0:fm])[0:1],
                                jnp.sum(acc, axis=0, keepdims=True)], axis=1)
    gate = first_layer(wg_s)
    up = first_layer(wu_s)
    act = (gate * jax.nn.sigmoid(gate) * up).astype(bf)
    actf = act.astype(f32)
    fd = F - 128 * DN_VPU
    y = _dot_nt(jnp.broadcast_to(act[:, 0:fd], (16, fd)), wd_s[:, 0:fd])
    parts = []
    for i in range(D // 8):
        w = wd_s[8 * i:8 * i + 8, fd:F].astype(f32) * actf[:, fd:F]
        tot = w[:, 0:128]
        for c in range(1, DN_VPU):
            tot = tot + w[:, 128 * c:128 * (c + 1)]
        parts.append(tot)
    yv = jnp.sum(jnp.concatenate(parts, axis=0), axis=1, keepdims=True)
    yt = (jnp.broadcast_to(y[0:1], (128, D)).T + yv) * jax.nn.sigmoid(best[0:1, 0:1])
    for s in range(NSEG):
        out_copy(s).wait()
    seg = blk // 4
    c0 = pl.multiple_of((blk - seg * 4) * 128, 128)
    cur = out_s[seg, :, pl.ds(c0, 128)].astype(f32)
    hit = _iota((D, 128), 1) == col
    fin_s[...] = (cur + jnp.where(hit, yt, 0.0)).astype(bf)
    fin = cp(fin_s, out_hbm.at[:, pl.ds(pl.multiple_of(blk * 128, 128), 128)], sems.at[15])
    fin.start()
    fin.wait()


@jax.jit
def pallas_sequential_preLN__memory_aug_infini_attn__moe_arch_mod__prompt_kernel(
    A_x, A_wq, A_wk, A_wv, A_wo, A_beta, B_x, B_w_r, B_w_gate, B_w_up, B_w_down,
):
    hbm = pl.BlockSpec(memory_space=pltpu.HBM)
    vm = pltpu.VMEM
    x_t = A_x.reshape(S, D).T
    out_t = pl.pallas_call(
        _kernel,
        out_shape=jax.ShapeDtypeStruct((D, S), bf),
        in_specs=[hbm] * 10,
        out_specs=hbm,
        scratch_shapes=[
            vm((NSEG, DP, L), bf), vm((DP, D), bf), vm((DP, D), bf), vm((DP, D), bf), vm((D, D), bf),
            vm((D, F), bf), vm((D, F), bf), vm((D, F), bf),
            vm((DP // 2, 128), u32), vm((D // 2, DP), u32), vm((D // 2, D), u32),
            vm((L // 2, DP), u32), vm((4, 8, 128), f32), vm((4, 128, 128), f32),
            vm((NQ, L // 2, 128), u32), vm((NQ, L // 2, 128), u32),
            vm((NQ, L // 2, 128), u32), vm((NQ, L // 2, 128), u32),
            vm((D // 2, L), u32),
            vm((640, 512), u32), vm((640, 512), u32), vm((16, D, 128), f32),
            vm((2, D, L), f32), vm((NQ, 80, 128), f32), vm((NQ, 40, 128), u32),
            vm((H, 1, 128), f32), vm((D, 128), f32), vm((8, 128), f32), vm((NSEG, D, L), bf),
            vm((16, 8, 128), f32),
            vm((NSEG, 8, 128), f32), vm((8, 128), f32), vm((D, 128), bf),
            vm((H,), bf), vm((D,), bf),
            pltpu.SemaphoreType.DMA((18,)),
        ],
        compiler_params=pltpu.CompilerParams(vmem_limit_bytes=100 * 1024 * 1024),
        name="infini_moe",
    )(x_t, A_wq, A_wk, A_wv, A_wo, A_beta, B_w_r, B_w_gate, B_w_up, B_w_down.T)
    return out_t.T.reshape(1, S, D)
```

```python
import jax
import jax.numpy as jnp
from jax import lax
from jax.experimental import pallas as pl
from jax.experimental.pallas import tpu as pltpu

S, D, H, DH = 2048, 576, 32, 18
NSEG, L, F = 4, 512, 4608
DP = 640
NQ = 8
QW = 4 * DH
bf, u32, f32, i32 = jnp.bfloat16, jnp.uint32, jnp.float32, jnp.int32
LOG2E = 1.4426950408889634
QSCALE = DH ** -0.5 * LOG2E
MASKB = -1000000000.0 * LOG2E
EPS = 1e-5
NT = (((1,), (1,)), ((), ()))
ONES2 = 0x3F803F80
GU_VPU = 11
DN_VPU = 26
DEN_LO, DEN_HI, WV_MAX = 2.0 ** -60, 2.0 ** 60, 2.0 ** 40


def _tobf(x):
    return pltpu.bitcast(x, bf)


def _tou(x):
    return pltpu.bitcast(x, u32)


def _pack(x):
    return pltpu.bitcast(x.astype(bf), u32)


def _dot(a, b):
    return jnp.dot(a, b, preferred_element_type=f32)


def _dot_nt(a, b):
    return lax.dot_general(a, b, NT, preferred_element_type=f32)


def _phi(t):
    return jnp.where(t > 0, t + 1.0, jnp.exp(t))


def _rowsum(parts):
    acc = [jnp.sum(p.reshape(p.shape[0] // 8, 8, 128), axis=0) for p in parts]
    while len(acc) > 1:
        acc = [acc[i] + acc[i + 1] for i in range(0, len(acc), 2)]
    return jnp.sum(acc[0], axis=0, keepdims=True)


def _ln_stats(rows, w=None):
    d = [rows(144 * g, 144 * (g + 1)) for g in range(4)]
    m1 = _rowsum(d) * (1.0 / D)
    m2 = _rowsum([v * v for v in d]) * (1.0 / D)
    var = jnp.maximum(m2 - m1 * m1, 0.0)
    rstd = lax.rsqrt(var + EPS)
    if w is None:
        return m1, rstd
    dw = _rowsum([d[g] * w[0][144 * g:144 * (g + 1)] for g in range(4)])
    return m1, rstd, (dw - m1 * w[1]) * rstd


def _hi_lo(v):
    hi = v.astype(bf).astype(f32)
    return hi, (v - hi).astype(bf).astype(f32)


def _iota(shape, dim):
    return lax.broadcasted_iota(i32, shape, dim)


def _al(x, n):
    return x if isinstance(x, int) else pl.multiple_of(x, n)


def _kernel(x_hbm, wq_hbm, wk_hbm, wv_hbm, wo_hbm, beta_hbm, wr_hbm,
            wg_hbm, wu_hbm, wd_hbm, out_hbm,
            x_s, wq_s, wk_s, wv_s, wo_s, wg_s, wu_s, wd_s,
            w4_u, wvt_u, wot_u, xn_u, rs_s, rc_s, qx, kx, pqx, pkx, vt_u,
            p0, p1, h_s, ot_s, m_f, m_u, g_s, wr_s, wrs_s, out_s, st_s, best_s, den_s, fin_s,
            beta_ref, wr_ref, sems):
    cp = pltpu.make_async_copy

    def x_copy(s):
        return cp(x_hbm.at[:, pl.ds(_al(s * L, L), L)], x_s.at[s, pl.ds(0, D), :], sems.at[s])

    def out_copy(s):
        return cp(out_s.at[s], out_hbm.at[:, pl.ds(_al(s * L, L), L)], sems.at[11 + s])

    def prep(s, t):
        c = 128 * t
        mean, rstd = _ln_stats(lambda a, b: x_s[s, a:b, pl.ds(c, 128)].astype(f32))
        mh, ml = _hi_lo(mean)
        r16 = _iota((16, 128), 0)
        x_s[s, D:D + 16, pl.ds(c, 128)] = jnp.where(
            r16 < 2, mh, jnp.where(r16 == 2, ml, 0.0)).astype(bf)
        rs_s[t, 0:1] = rstd
        rc_s[t] = jnp.broadcast_to(rstd, (128, 128)).T
        xn_u[pl.ds(64 * t, 64), :] = _tou(x_s[s, :, pl.ds(c, 128)].T)

    def augment(w_ref, a=0, b=D):
        ones = jnp.ones((16, D), bf)
        hi, lo = _hi_lo(_dot(ones, w_ref[0:D, a:b])[0:1])
        r16 = _iota((16, b - a), 0)
        w_ref[D:D + 16, a:b] = jnp.where((r16 == 0) | (r16 == 2), -hi,
                                         jnp.where(r16 == 1, -lo, 0.0)).astype(bf)

    top = pl.ds(0, D)
    w_copies = [None, cp(wk_hbm, wk_s.at[top, :], sems.at[5]),
                cp(wv_hbm, wv_s.at[top, :], sems.at[6]), cp(wo_hbm, wo_s, sems.at[7])]
    e_copies = [cp(wg_hbm, wg_s, sems.at[8]), cp(wu_hbm, wu_s, sems.at[9]),
                cp(wd_hbm, wd_s, sems.at[10])]

    small = [cp(beta_hbm, beta_ref, sems.at[16]), cp(wr_hbm, wr_ref, sems.at[17])]
    half = [cp(x_hbm.at[:, pl.ds(256 * i, 256)], x_s.at[0, top, pl.ds(256 * i, 256)],
               sems.at[18 * i]) for i in range(2)]
    wq_lo = cp(wq_hbm.at[:, pl.ds(0, 512)], wq_s.at[top, pl.ds(0, 512)], sems.at[4])
    wq_hi = cp(wq_hbm.at[:, pl.ds(512, D - 512)], wq_s.at[top, pl.ds(512, D - 512)], sems.at[19])
    half[0].start()
    wq_lo.start()
    half[1].start()
    for c in small:
        c.start()

    m_f[...] = jnp.zeros_like(m_f)
    den_s[...] = jnp.ones_like(den_s)

    for w_ref in (wq_s, wk_s, wv_s):
        w_ref[D + 16:DP, :] = jnp.zeros((DP - D - 16, D), bf)
    for s in range(NSEG):
        x_s[s, D + 16:DP, :] = jnp.zeros((DP - D - 16, L), bf)

    lane1 = _iota((1, 128), 1)
    causal = _iota((128, 128), 0) <= _iota((128, 128), 1)

    def proj_q(t):
        rows = pl.ds(64 * t, 64)
        q = _dot(_tobf(xn_u[rows, :]), wq_s[:, 0:512]) * jnp.concatenate([rc_s[t]] * 4, axis=1)
        tiles = [q[:, 128 * i:128 * (i + 1)] for i in range(4)]
        raw = [_pack(v * QSCALE) for v in tiles]
        ph = [_pack(_phi(v)) for v in tiles]
        for c in range(NQ):
            i = c // 2
            if c % 2 == 0 or c == NQ - 1:
                qx[c, rows, :] = raw[i]
                pqx[c, rows, :] = ph[i]
            else:
                keep = lane1 >= (QW * c) % 128
                qx[c, rows, :] = jnp.where(keep, raw[i], raw[i + 1])
                pqx[c, rows, :] = jnp.where(keep, ph[i], ph[i + 1])

    def proj_k(t):
        rows = pl.ds(64 * t, 64)
        xn = _tobf(xn_u[rows, :])
        rc = rc_s[t]
        k = _dot(xn, wk_s[:, 0:512]) * jnp.concatenate([rc] * 4, axis=1)
        r4 = _dot(xn, _tobf(w4_u[...])) * rc
        tiles = [k[:, 128 * i:128 * (i + 1)] for i in range(4)] + [pltpu.roll(r4, 64, 1)]
        raw = [_pack(v) for v in tiles]
        ph = [_pack(_phi(v)) for v in tiles]
        for c in range(NQ):
            i = c // 2
            if c % 2 == 0:
                kx[c, rows, :] = raw[i]
                pkx[c, rows, :] = ph[i]
            else:
                keep = lane1 >= (QW * c) % 128
                kx[c, rows, :] = jnp.where(keep, raw[i], raw[i + 1])
                pkx[c, rows, :] = jnp.where(keep, ph[i], ph[i + 1])
        keep = lane1 >= (QW * (NQ - 1)) % 128
        qx[NQ - 1, rows, :] = jnp.where(keep, qx[NQ - 1, rows, :], _pack(r4 * QSCALE))
        pqx[NQ - 1, rows, :] = jnp.where(keep, pqx[NQ - 1, rows, :], _pack(_phi(r4)))

    def proj_v(s, t):
        vt = _dot(_tobf(wvt_u[...]), x_s[s, :, pl.ds(128 * t, 128)]) * rs_s[t, 0:1]
        vt_u[:, pl.ds(128 * t, 128)] = _pack(vt)

    def masked_q(k, par, j):
        q = qx[2 * k + par, pl.ds(64 * j, 64), :]
        out = []
        for i in range(4):
            st = (2 * QW * k + QW * par + DH * i) % 128
            out.append(q & jnp.where(((lane1 - st) & 127) < DH, jnp.uint32(0xFFFFFFFF),
                                     jnp.uint32(0)))
        return out

    def scores(k, par, j):
        qm = _tobf(jnp.concatenate(masked_q(k, par, j), axis=0))
        kk = _tobf(kx[2 * k + par, pl.ds(0, 64 * (j + 1)), :])
        return _dot_nt(kk, qm)

    r64, l64 = _iota((64, 128), 0), _iota((64, 128), 1)
    lo_nat = (l64 >= 64) | (r64 <= l64)
    lo_swp = (l64 < 64) | (r64 <= l64 - 64)
    hi_even = (l64 < 64) & (r64 <= l64)
    hi_odd = (l64 >= 64) & (r64 <= l64 - 64)

    def stage_a(k, par, j, p_ref):
        c = 2 * k + par
        qm = masked_q(k, par, j)
        w1 = [jnp.concatenate([qm[i][32:], qm[i][:32]], axis=0) if i % 2 == 0 else qm[i]
              for i in range(4)]
        w2 = [qm[i][32:] for i in range(4)]
        n1 = 128 * j + 64
        p1 = jnp.exp2(_dot_nt(_tobf(kx[c, pl.ds(0, n1 // 2), :]),
                              _tobf(jnp.concatenate(w1, axis=0))))
        p2 = jnp.exp2(_dot_nt(_tobf(kx[c, pl.ds(n1 // 2, 32), :]),
                              _tobf(jnp.concatenate(w2, axis=0))))
        off = 64 * (j * (j + 1) // 2)
        if j > 0:
            p_ref[pl.ds(off, 64 * j), :] = _pack(p1[:128 * j])
        lo = [jnp.where(lo_swp if i % 2 == 0 else lo_nat,
                        p1[128 * j:, 128 * i:128 * (i + 1)], 0.0) for i in range(4)]
        hi = [jnp.where(hi_even if i % 2 == 0 else hi_odd,
                        p2[:, 128 * (i // 2):128 * (i // 2 + 1)], 0.0) for i in range(4)]
        p_ref[pl.ds(off + 64 * j, 32), :] = _pack(jnp.concatenate(lo, axis=1))
        p_ref[pl.ds(off + 64 * j + 32, 32), :] = _pack(jnp.concatenate(hi, axis=1))

    def stage_a_safe(k, par, j, p_ref):
        s = scores(k, par, j)
        bias = jnp.where(causal, 0.0, MASKB).astype(f32)
        sd = s[128 * j:] + jnp.concatenate([bias] * 4, axis=1)
        s = sd if j == 0 else jnp.concatenate([s[:128 * j], sd], axis=0)
        p = jnp.exp2(s - jnp.max(s, axis=0, keepdims=True))
        p_ref[pl.ds(64 * (j * (j + 1) // 2), 64 * (j + 1)), :] = _pack(p)

    def stage_b(use_mem, oslot, k, par, j, p_ref, swapped=True):
        c = 2 * k + par
        base = QW * par
        mwin = base - base % 16
        moff = base - mwin
        zrow = 72 if moff == 0 else 0
        srow = _iota((8, 128), 0)
        grow = [g_s[4 * c + i] for i in range(4)]
        off = 64 * (j * (j + 1) // 2)
        if use_mem:
            mem = _dot_nt(_tobf(m_u[c]), _tobf(pqx[c, pl.ds(64 * j, 64), :]))
        accs, rds, rms = [], [], []
        dlo, dhi = den_s[0:1], den_s[1:2]
        for i in range(4):
            r0 = base + DH * i
            w = r0 - r0 % 16
            o = r0 - w
            vt = vt_u[pl.ds(_al(QW * k + w // 2, 8), 16), pl.ds(0, 128 * (j + 1))]
            orow = 15 if o < 14 else 0
            vt = jnp.where(_iota(vt.shape, 0) == orow, jnp.uint32(ONES2), vt)
            p = _tobf(p_ref[pl.ds(off, 64 * (j + 1)), pl.ds(128 * i, 128)])
            acc = _dot(_tobf(vt), p)
            if swapped and i % 2 == 0:
                acc = pltpu.roll(acc, 64, 1)
            den = acc[2 * orow:2 * orow + 1]
            dlo, dhi = jnp.minimum(dlo, den), jnp.maximum(dhi, den)
            rds.append((1.0 - grow[i]) / den)
            if use_mem:
                rms.append(grow[i] / (mem[zrow + i:zrow + i + 1] + 1e-6))
            a0 = o - o % 8
            accs.append(acc[a0:a0 + 24])
        den_s[0:1] = dlo
        den_s[1:2] = dhi
        for v in range(9):
            lo_h, hi_h = (8 * v) // DH, (8 * v + 7) // DH

            def piece(h):
                a = accs[h][8 * (v - (DH * h) // 8):8 * (v - (DH * h) // 8) + 8]
                if not use_mem:
                    return a * rds[h]
                return a * rds[h] + mem[moff + 8 * v:moff + 8 * v + 8] * rms[h]
            val = piece(lo_h)
            if hi_h != lo_h:
                val = jnp.where(srow < DH * hi_h - 8 * v, val, piece(hi_h))
            ot_s[oslot, pl.ds(_al(2 * QW * k + base + 8 * v, 8), 8), pl.ds(128 * j, 128)] = val

    def mem_update(k, par):
        c = 2 * k + par
        base = QW * par
        mwin = base - base % 16
        moff = base - mwin
        zrow = 72 if moff == 0 else 0
        vw = vt_u[pl.ds(_al(QW * k + mwin // 2, 8), 40), :]
        rr = _iota(vw.shape, 0)
        isz = (rr >= 36) if moff == 0 else (rr < 4)
        vw = jnp.where(isz, jnp.uint32(ONES2), vw)
        upd = _dot(_tobf(vw), _tobf(pkx[c]))
        r80 = _iota((80, 128), 0)
        l80 = (_iota((80, 128), 1) - (2 * QW * k + base)) & 127
        hrow = jnp.where((r80 >= zrow) & (r80 < zrow + 8), r80 - zrow, (r80 - moff) // DH)
        keep = (l80 >= DH * hrow) & (l80 < DH * hrow + DH) & (hrow < 4) & (hrow >= 0)
        mnew = m_f[c] + jnp.where(keep, upd, 0.0)
        m_f[c] = mnew
        m_u[c] = _pack(mnew)

    pb = (p0, p1)

    def step(use_mem, update, oslot, a, b):
        for j in range(4):
            if b is not None:
                stage_b(use_mem, oslot, b[0], b[1], j, pb[b[1]])
                if j == 3 and update:
                    mem_update(b[0], b[1])
            if a is not None:
                stage_a(a[0], a[1], j, pb[a[1]])

    def out_proj(s, t):
        c = 128 * t
        o = ot_s[s % 2, :, pl.ds(c, 128)].astype(bf)
        h = x_s[s, 0:D, pl.ds(c, 128)].astype(f32) + _dot(_tobf(wot_u[...]), o)
        h_s[4 * s + t] = h
        mean, rstd, sc = _ln_stats(lambda a, b: h[a:b], (wr_s[...], wrs_s[0:1]))
        st_s[4 * s + t, 0:1] = mean
        st_s[4 * s + t, 1:2] = rstd
        smax = jnp.max(sc, axis=1, keepdims=True)
        pos = (lane1 + (s * L + c)).astype(f32)
        sidx = jnp.min(jnp.where(sc == smax, pos, 1e9), axis=1, keepdims=True)
        new = jnp.concatenate([jnp.broadcast_to(smax, (1, 128)), jnp.broadcast_to(sidx, (1, 128)),
                               jnp.zeros((6, 128), f32)], axis=0)
        if t == 0:
            best_s[s] = new
        else:
            old = best_s[s]
            best_s[s] = jnp.where(smax > old[0:1, 0:1], new, old)

    def post(s, t):
        rstd = st_s[4 * s + t, 1:2]
        a = 1.0 + rstd
        b = st_s[4 * s + t, 0:1] * rstd
        out_s[s, :, pl.ds(128 * t, 128)] = (h_s[4 * s + t] * a - b).astype(bf)

    def finish(s):
        for t in range(4):
            out_proj(s, t)
            if t < 3:
                post(s, t)

    def attention(s):
        use_mem, update, o = s > 0, s < NSEG - 1, s % 2
        step(use_mem, update, o, (0, 0), None)
        for k in range(NQ // 2):
            step(use_mem, update, o, (k, 1), (k, 0))
            if s > 0:
                out_proj(s - 1, k)
                post(s - 1, k)
            step(use_mem, update, o, (k + 1, 0) if k + 1 < NQ // 2 else None, (k, 1))
        if s > 0:
            out_copy(s - 1).start()

    half[0].wait()
    for t in range(2):
        prep(0, t)
    wq_lo.wait()
    w_copies[1].start()
    wq_hi.start()
    augment(wq_s, 0, 512)
    for t in range(2):
        proj_q(t)
    half[1].wait()
    w_copies[2].start()
    for t in range(2, 4):
        prep(0, t)
        proj_q(t)
    w_copies[1].wait()
    wq_hi.wait()
    augment(wq_s, 512, D)
    w_copies[3].start()
    for s in range(1, NSEG):
        x_copy(s).start()
    augment(wk_s)
    w4_u[...] = _tou(jnp.concatenate([wq_s[:, 512:D], wk_s[:, 512:D]], axis=1))
    for t in range(2):
        proj_k(t)
    w_copies[2].wait()
    augment(wv_s)
    wvt_u[...] = _tou(wv_s[...].T)
    wv_ok = jnp.max(jnp.abs(wv_s[0:D, :].astype(f32))) < WV_MAX
    for t in range(2, 4):
        proj_k(t)
    w_copies[3].wait()
    for c in small:
        c.wait()
    g32 = jax.nn.sigmoid(beta_ref[...].astype(f32)).reshape(1, H)
    sel = _iota((H, H), 1) == _iota((H, H), 0)
    gcol = jnp.sum(jnp.where(sel, g32, 0.0), axis=1, keepdims=True)
    for h in range(H):
        g_s[h] = jnp.broadcast_to(gcol[h:h + 1], (1, 128))
    wr_s[...] = jnp.broadcast_to(wr_ref[...].astype(f32).reshape(1, D), (128, D)).T
    wrs_s[...] = jnp.broadcast_to(jnp.sum(wr_s[...], axis=0, keepdims=True), (8, 128))
    wot_u[...] = _tou(wo_s[...].T)
    for t in range(4):
        proj_v(0, t)
    attention(0)
    for s in range(1, NSEG):
        x_copy(s).wait()

    for s in range(1, NSEG):
        e_copies[s - 1].start()
        for t in range(4):
            prep(s, t)
        for t in range(4):
            proj_v(s, t)
        for t in range(4):
            proj_q(t)
            proj_k(t)
        attention(s)
    finish(NSEG - 1)
    post(NSEG - 1, 3)
    out_copy(NSEG - 1).start()

    dl = den_s[...]
    safe = jnp.logical_and(jnp.min(dl[0:1]) >= DEN_LO, jnp.max(dl[1:2]) <= DEN_HI)
    safe = jnp.logical_and(safe, wv_ok)

    @pl.when(jnp.logical_not(safe))
    def _():
        for s in range(NSEG):
            out_copy(s).wait()
        m_f[...] = jnp.zeros_like(m_f)
        m_u[...] = jnp.zeros_like(m_u)

        def seg_redo(s, carry):
            for t in range(4):
                prep(s, t)
                proj_v(s, t)
                proj_q(t)
                proj_k(t)

            def quads(k, carry):
                for par in range(2):
                    for j in range(4):
                        stage_a_safe(k, par, j, pb[par])
                        stage_b(True, s % 2, k, par, j, pb[par], swapped=False)
                    mem_update(k, par)
                return carry
            lax.fori_loop(0, NQ // 2, quads, 0)
            finish(s)
            post(s, 3)
            out_copy(s).start()
            return carry
        lax.fori_loop(0, NSEG, seg_redo, 0)

    for c in e_copies:
        c.wait()
    best = best_s[0]
    for s in range(1, NSEG):
        cand = best_s[s]
        best = jnp.where(cand[0:1, 0:1] > best[0:1, 0:1], cand, best)
    idx = jnp.clip(best[1, 0].astype(i32), 0, S - 1)
    blk = idx // 128
    col = idx - blk * 128
    onehot = ((_iota((16, 128), 1) == col) & (_iota((16, 128), 0) == 0)).astype(bf)
    ln = ((h_s[blk] - st_s[blk, 0:1]) * st_s[blk, 1:2]).astype(bf)
    xs = _dot_nt(onehot, ln).astype(bf)
    pick = (_iota((128, 128), 0) == col).astype(bf)
    xcol = _dot(ln, pick)
    fm = F - 128 * GU_VPU

    def first_layer(w_ref):
        acc = jnp.zeros((8, 128 * GU_VPU), f32)
        for i in range(D // 8):
            w = w_ref[8 * i:8 * i + 8, fm:F].astype(f32)
            acc = acc + w * jnp.concatenate([xcol[8 * i:8 * i + 8]] * GU_VPU, axis=1)
        return jnp.concatenate([_dot(xs, w_ref[:, 0:fm])[0:1],
                                jnp.sum(acc, axis=0, keepdims=True)], axis=1)
    gate = first_layer(wg_s)
    up = first_layer(wu_s)
    act = (gate * jax.nn.sigmoid(gate) * up).astype(bf)
    actf = act.astype(f32)
    fd = F - 128 * DN_VPU
    y = _dot_nt(jnp.broadcast_to(act[:, 0:fd], (16, fd)), wd_s[:, 0:fd])
    parts = []
    for i in range(D // 8):
        w = wd_s[8 * i:8 * i + 8, fd:F].astype(f32) * actf[:, fd:F]
        tot = w[:, 0:128]
        for c in range(1, DN_VPU):
            tot = tot + w[:, 128 * c:128 * (c + 1)]
        parts.append(tot)
    yv = jnp.sum(jnp.concatenate(parts, axis=0), axis=1, keepdims=True)
    yt = (jnp.broadcast_to(y[0:1], (128, D)).T + yv) * jax.nn.sigmoid(best[0:1, 0:1])
    for s in range(NSEG):
        out_copy(s).wait()
    seg = blk // 4
    c0 = pl.multiple_of((blk - seg * 4) * 128, 128)
    cur = out_s[seg, :, pl.ds(c0, 128)].astype(f32)
    hit = _iota((D, 128), 1) == col
    fin_s[...] = (cur + jnp.where(hit, yt, 0.0)).astype(bf)
    fin = cp(fin_s, out_hbm.at[:, pl.ds(pl.multiple_of(blk * 128, 128), 128)], sems.at[15])
    fin.start()
    fin.wait()


@jax.jit
def pallas_sequential_preLN__memory_aug_infini_attn__moe_arch_mod__prompt_kernel(
    A_x, A_wq, A_wk, A_wv, A_wo, A_beta, B_x, B_w_r, B_w_gate, B_w_up, B_w_down,
):
    hbm = pl.BlockSpec(memory_space=pltpu.HBM)
    vm = pltpu.VMEM
    x_t = A_x.reshape(S, D).T
    out_t = pl.pallas_call(
        _kernel,
        out_shape=jax.ShapeDtypeStruct((D, S), bf),
        in_specs=[hbm] * 10,
        out_specs=hbm,
        scratch_shapes=[
            vm((NSEG, DP, L), bf), vm((DP, D), bf), vm((DP, D), bf), vm((DP, D), bf), vm((D, D), bf),
            vm((D, F), bf), vm((D, F), bf), vm((D, F), bf),
            vm((DP // 2, 128), u32), vm((D // 2, DP), u32), vm((D // 2, D), u32),
            vm((L // 2, DP), u32), vm((4, 8, 128), f32), vm((4, 128, 128), f32),
            vm((NQ, L // 2, 128), u32), vm((NQ, L // 2, 128), u32),
            vm((NQ, L // 2, 128), u32), vm((NQ, L // 2, 128), u32),
            vm((D // 2, L), u32),
            vm((640, 512), u32), vm((640, 512), u32), vm((16, D, 128), f32),
            vm((2, D, L), f32), vm((NQ, 80, 128), f32), vm((NQ, 40, 128), u32),
            vm((H, 1, 128), f32), vm((D, 128), f32), vm((8, 128), f32), vm((NSEG, D, L), bf),
            vm((16, 8, 128), f32),
            vm((NSEG, 8, 128), f32), vm((8, 128), f32), vm((D, 128), bf),
            vm((H,), bf), vm((D,), bf),
            pltpu.SemaphoreType.DMA((20,)),
        ],
        compiler_params=pltpu.CompilerParams(vmem_limit_bytes=100 * 1024 * 1024),
        name="infini_moe",
    )(x_t, A_wq, A_wk, A_wv, A_wo, A_beta, B_w_r, B_w_gate, B_w_up, B_w_down.T)
    return out_t.T.reshape(1, S, D)
```

```python
import jax
import jax.numpy as jnp
from jax import lax
from jax.experimental import pallas as pl
from jax.experimental.pallas import tpu as pltpu

S, D, H, DH = 2048, 576, 32, 18
NSEG, L, F = 4, 512, 4608
DP = 640
NQ = 8
QW = 4 * DH
bf, u32, f32, i32 = jnp.bfloat16, jnp.uint32, jnp.float32, jnp.int32
LOG2E = 1.4426950408889634
QSCALE = DH ** -0.5 * LOG2E
MASKB = -1000000000.0 * LOG2E
EPS = 1e-5
NT = (((1,), (1,)), ((), ()))
ONES2 = 0x3F803F80
GU_VPU = 11
DN_VPU = 26
DEN_LO, DEN_HI, WV_MAX = 2.0 ** -60, 2.0 ** 60, 2.0 ** 40


def _tobf(x):
    return pltpu.bitcast(x, bf)


def _tou(x):
    return pltpu.bitcast(x, u32)


def _pack(x):
    return pltpu.bitcast(x.astype(bf), u32)


def _dot(a, b):
    return jnp.dot(a, b, preferred_element_type=f32)


def _dot_nt(a, b):
    return lax.dot_general(a, b, NT, preferred_element_type=f32)


def _phi(t):
    return jnp.where(t > 0, t + 1.0, jnp.exp(t))


def _rowsum(parts):
    acc = [jnp.sum(p.reshape(p.shape[0] // 8, 8, 128), axis=0) for p in parts]
    while len(acc) > 1:
        acc = [acc[i] + acc[i + 1] for i in range(0, len(acc), 2)]
    return jnp.sum(acc[0], axis=0, keepdims=True)


def _ln_stats(rows, w=None):
    d = [rows(144 * g, 144 * (g + 1)) for g in range(4)]
    m1 = _rowsum(d) * (1.0 / D)
    m2 = _rowsum([v * v for v in d]) * (1.0 / D)
    var = jnp.maximum(m2 - m1 * m1, 0.0)
    rstd = lax.rsqrt(var + EPS)
    if w is None:
        return m1, rstd
    dw = _rowsum([d[g] * w[0][144 * g:144 * (g + 1)] for g in range(4)])
    return m1, rstd, (dw - m1 * w[1]) * rstd


def _hi_lo(v):
    hi = v.astype(bf).astype(f32)
    return hi, (v - hi).astype(bf).astype(f32)


def _iota(shape, dim):
    return lax.broadcasted_iota(i32, shape, dim)


def _al(x, n):
    return x if isinstance(x, int) else pl.multiple_of(x, n)


def _kernel(x_hbm, wq_hbm, wk_hbm, wv_hbm, wo_hbm, beta_hbm, wr_hbm,
            wg_hbm, wu_hbm, wd_hbm, out_hbm,
            x_s, wq_s, wk_s, wv_s, wo_s, wg_s, wu_s, wd_s,
            w4_u, wvt_u, wot_u, xn_u, rs_s, rc_s, qx, kx, pqx, pkx, vt_u,
            p0, p1, h_s, ot_s, m_f, m_u, g_s, wr_s, wrs_s, out_s, st_s, best_s, den_s, fin_s,
            beta_ref, wr_ref, sems):
    cp = pltpu.make_async_copy

    def x_copy(s):
        return cp(x_hbm.at[:, pl.ds(_al(s * L, L), L)], x_s.at[s, pl.ds(0, D), :], sems.at[s])

    def out_copy(s):
        return cp(out_s.at[s], out_hbm.at[:, pl.ds(_al(s * L, L), L)], sems.at[11 + s])

    def prep(s, t):
        c = 128 * t
        mean, rstd = _ln_stats(lambda a, b: x_s[s, a:b, pl.ds(c, 128)].astype(f32))
        mh, ml = _hi_lo(mean)
        r16 = _iota((16, 128), 0)
        x_s[s, D:D + 16, pl.ds(c, 128)] = jnp.where(
            r16 < 2, mh, jnp.where(r16 == 2, ml, 0.0)).astype(bf)
        rs_s[t, 0:1] = rstd
        rc_s[t] = jnp.broadcast_to(rstd, (128, 128)).T
        xn_u[pl.ds(64 * t, 64), :] = _tou(x_s[s, :, pl.ds(c, 128)].T)

    def augment(w_ref, a=0, b=D):
        ones = jnp.ones((16, D), bf)
        hi, lo = _hi_lo(_dot(ones, w_ref[0:D, a:b])[0:1])
        r16 = _iota((16, b - a), 0)
        w_ref[D:D + 16, a:b] = jnp.where((r16 == 0) | (r16 == 2), -hi,
                                         jnp.where(r16 == 1, -lo, 0.0)).astype(bf)

    top = pl.ds(0, D)
    w_copies = [None, cp(wk_hbm, wk_s.at[top, :], sems.at[5]),
                cp(wv_hbm, wv_s.at[top, :], sems.at[6]), cp(wo_hbm, wo_s, sems.at[7])]
    e_copies = [cp(wg_hbm, wg_s, sems.at[8]), cp(wu_hbm, wu_s, sems.at[9]),
                cp(wd_hbm, wd_s, sems.at[10])]

    small = [cp(beta_hbm, beta_ref, sems.at[16]), cp(wr_hbm, wr_ref, sems.at[17])]
    half = [cp(x_hbm.at[:, pl.ds(256 * i, 256)], x_s.at[0, top, pl.ds(256 * i, 256)],
               sems.at[18 * i]) for i in range(2)]
    wq_lo = cp(wq_hbm.at[:, pl.ds(0, 512)], wq_s.at[top, pl.ds(0, 512)], sems.at[4])
    wq_hi = cp(wq_hbm.at[:, pl.ds(512, D - 512)], wq_s.at[top, pl.ds(512, D - 512)], sems.at[19])
    half[0].start()
    wq_lo.start()
    half[1].start()
    for c in small:
        c.start()

    m_f[...] = jnp.zeros_like(m_f)
    den_s[...] = jnp.ones_like(den_s)

    for w_ref in (wq_s, wk_s, wv_s):
        w_ref[D + 16:DP, :] = jnp.zeros((DP - D - 16, D), bf)
    for s in range(NSEG):
        x_s[s, D + 16:DP, :] = jnp.zeros((DP - D - 16, L), bf)

    lane1 = _iota((1, 128), 1)
    causal = _iota((128, 128), 0) <= _iota((128, 128), 1)

    def proj_q(t):
        rows = pl.ds(64 * t, 64)
        q = _dot(_tobf(xn_u[rows, :]), wq_s[:, 0:512]) * jnp.concatenate([rc_s[t]] * 4, axis=1)
        tiles = [q[:, 128 * i:128 * (i + 1)] for i in range(4)]
        raw = [_pack(v * QSCALE) for v in tiles]
        ph = [_pack(_phi(v)) for v in tiles]
        for c in range(NQ):
            i = c // 2
            if c % 2 == 0 or c == NQ - 1:
                qx[c, rows, :] = raw[i]
                pqx[c, rows, :] = ph[i]
            else:
                keep = lane1 >= (QW * c) % 128
                qx[c, rows, :] = jnp.where(keep, raw[i], raw[i + 1])
                pqx[c, rows, :] = jnp.where(keep, ph[i], ph[i + 1])

    def proj_k(t):
        rows = pl.ds(64 * t, 64)
        xn = _tobf(xn_u[rows, :])
        rc = rc_s[t]
        k = _dot(xn, wk_s[:, 0:512]) * jnp.concatenate([rc] * 4, axis=1)
        r4 = _dot(xn, _tobf(w4_u[...])) * rc
        tiles = [k[:, 128 * i:128 * (i + 1)] for i in range(4)] + [pltpu.roll(r4, 64, 1)]
        raw = [_pack(v) for v in tiles]
        ph = [_pack(_phi(v)) for v in tiles]
        for c in range(NQ):
            i = c // 2
            if c % 2 == 0:
                kx[c, rows, :] = raw[i]
                pkx[c, rows, :] = ph[i]
            else:
                keep = lane1 >= (QW * c) % 128
                kx[c, rows, :] = jnp.where(keep, raw[i], raw[i + 1])
                pkx[c, rows, :] = jnp.where(keep, ph[i], ph[i + 1])
        keep = lane1 >= (QW * (NQ - 1)) % 128
        qx[NQ - 1, rows, :] = jnp.where(keep, qx[NQ - 1, rows, :], _pack(r4 * QSCALE))
        pqx[NQ - 1, rows, :] = jnp.where(keep, pqx[NQ - 1, rows, :], _pack(_phi(r4)))

    def proj_v(s, t):
        vt = _dot(_tobf(wvt_u[...]), x_s[s, :, pl.ds(128 * t, 128)]) * rs_s[t, 0:1]
        vt_u[:, pl.ds(128 * t, 128)] = _pack(vt)

    def masked_q(k, par, j):
        q = qx[2 * k + par, pl.ds(64 * j, 64), :]
        out = []
        for i in range(4):
            st = (2 * QW * k + QW * par + DH * i) % 128
            out.append(q & jnp.where(((lane1 - st) & 127) < DH, jnp.uint32(0xFFFFFFFF),
                                     jnp.uint32(0)))
        return out

    def scores(k, par, j):
        qm = _tobf(jnp.concatenate(masked_q(k, par, j), axis=0))
        kk = _tobf(kx[2 * k + par, pl.ds(0, 64 * (j + 1)), :])
        return _dot_nt(kk, qm)

    r64, l64 = _iota((64, 128), 0), _iota((64, 128), 1)
    lo_nat = (l64 >= 64) | (r64 <= l64)
    lo_swp = (l64 < 64) | (r64 <= l64 - 64)
    hi_even = (l64 < 64) & (r64 <= l64)
    hi_odd = (l64 >= 64) & (r64 <= l64 - 64)

    def stage_a(k, par, j, p_ref):
        c = 2 * k + par
        qm = masked_q(k, par, j)
        w1 = [jnp.concatenate([qm[i][32:], qm[i][:32]], axis=0) if i % 2 == 0 else qm[i]
              for i in range(4)]
        w2 = [qm[i][32:] for i in range(4)]
        n1 = 128 * j + 64
        p1 = jnp.exp2(_dot_nt(_tobf(kx[c, pl.ds(0, n1 // 2), :]),
                              _tobf(jnp.concatenate(w1, axis=0))))
        p2 = jnp.exp2(_dot_nt(_tobf(kx[c, pl.ds(n1 // 2, 32), :]),
                              _tobf(jnp.concatenate(w2, axis=0))))
        off = 64 * (j * (j + 1) // 2)
        if j > 0:
            p_ref[pl.ds(off, 64 * j), :] = _pack(p1[:128 * j])
        lo = [jnp.where(lo_swp if i % 2 == 0 else lo_nat,
                        p1[128 * j:, 128 * i:128 * (i + 1)], 0.0) for i in range(4)]
        hi = [jnp.where(hi_even if i % 2 == 0 else hi_odd,
                        p2[:, 128 * (i // 2):128 * (i // 2 + 1)], 0.0) for i in range(4)]
        p_ref[pl.ds(off + 64 * j, 32), :] = _pack(jnp.concatenate(lo, axis=1))
        p_ref[pl.ds(off + 64 * j + 32, 32), :] = _pack(jnp.concatenate(hi, axis=1))

    def stage_a_safe(k, par, j, p_ref):
        s = scores(k, par, j)
        bias = jnp.where(causal, 0.0, MASKB).astype(f32)
        sd = s[128 * j:] + jnp.concatenate([bias] * 4, axis=1)
        s = sd if j == 0 else jnp.concatenate([s[:128 * j], sd], axis=0)
        p = jnp.exp2(s - jnp.max(s, axis=0, keepdims=True))
        p_ref[pl.ds(64 * (j * (j + 1) // 2), 64 * (j + 1)), :] = _pack(p)

    def stage_b(use_mem, oslot, k, par, j, p_ref, swapped=True):
        c = 2 * k + par
        base = QW * par
        mwin = base - base % 16
        moff = base - mwin
        zrow = 72 if moff == 0 else 0
        srow = _iota((8, 128), 0)
        g4 = g_s[c, 0:4]
        off = 64 * (j * (j + 1) // 2)
        accs, dens = [], []
        for i in range(4):
            r0 = base + DH * i
            w = r0 - r0 % 16
            o = r0 - w
            vt = vt_u[pl.ds(_al(QW * k + w // 2, 8), 16), pl.ds(0, 128 * (j + 1))]
            orow = 15 if o < 14 else 0
            vt = jnp.where(_iota(vt.shape, 0) == orow, jnp.uint32(ONES2), vt)
            p = _tobf(p_ref[pl.ds(off, 64 * (j + 1)), pl.ds(128 * i, 128)])
            acc = _dot(_tobf(vt), p)
            if swapped and i % 2 == 0:
                acc = pltpu.roll(acc, 64, 1)
            dens.append(acc[2 * orow:2 * orow + 1])
            a0 = o - o % 8
            accs.append(acc[a0:a0 + 24])
        den4 = jnp.concatenate(dens, axis=0)
        den_s[0:4] = jnp.minimum(den_s[0:4], den4)
        den_s[4:8] = jnp.maximum(den_s[4:8], den4)
        rd4 = (1.0 - g4) / den4
        rds = [rd4[i:i + 1] for i in range(4)]
        if use_mem:
            mem = _dot_nt(_tobf(m_u[c]), _tobf(pqx[c, pl.ds(64 * j, 64), :]))
            rm4 = g4 / (mem[zrow:zrow + 4] + 1e-6)
            rms = [rm4[i:i + 1] for i in range(4)]
        for v in range(9):
            lo_h, hi_h = (8 * v) // DH, (8 * v + 7) // DH

            def piece(h):
                a = accs[h][8 * (v - (DH * h) // 8):8 * (v - (DH * h) // 8) + 8]
                if not use_mem:
                    return a * rds[h]
                return a * rds[h] + mem[moff + 8 * v:moff + 8 * v + 8] * rms[h]
            val = piece(lo_h)
            if hi_h != lo_h:
                val = jnp.where(srow < DH * hi_h - 8 * v, val, piece(hi_h))
            ot_s[oslot, pl.ds(_al(2 * QW * k + base + 8 * v, 8), 8), pl.ds(128 * j, 128)] = val

    def mem_update(k, par):
        c = 2 * k + par
        base = QW * par
        mwin = base - base % 16
        moff = base - mwin
        zrow = 72 if moff == 0 else 0
        vw = vt_u[pl.ds(_al(QW * k + mwin // 2, 8), 40), :]
        rr = _iota(vw.shape, 0)
        isz = (rr >= 36) if moff == 0 else (rr < 4)
        vw = jnp.where(isz, jnp.uint32(ONES2), vw)
        upd = _dot(_tobf(vw), _tobf(pkx[c]))
        r80 = _iota((80, 128), 0)
        l80 = (_iota((80, 128), 1) - (2 * QW * k + base)) & 127
        hrow = jnp.where((r80 >= zrow) & (r80 < zrow + 8), r80 - zrow, (r80 - moff) // DH)
        keep = (l80 >= DH * hrow) & (l80 < DH * hrow + DH) & (hrow < 4) & (hrow >= 0)
        mnew = m_f[c] + jnp.where(keep, upd, 0.0)
        m_f[c] = mnew
        m_u[c] = _pack(mnew)

    pb = (p0, p1)

    def step(use_mem, update, oslot, a, b):
        for j in range(4):
            if b is not None:
                stage_b(use_mem, oslot, b[0], b[1], j, pb[b[1]])
                if j == 3 and update:
                    mem_update(b[0], b[1])
            if a is not None:
                stage_a(a[0], a[1], j, pb[a[1]])

    def out_proj(s, t):
        c = 128 * t
        o = ot_s[s % 2, :, pl.ds(c, 128)].astype(bf)
        h = x_s[s, 0:D, pl.ds(c, 128)].astype(f32) + _dot(_tobf(wot_u[...]), o)
        h_s[4 * s + t] = h
        mean, rstd, sc = _ln_stats(lambda a, b: h[a:b], (wr_s[...], wrs_s[0:1]))
        st_s[4 * s + t, 0:1] = mean
        st_s[4 * s + t, 1:2] = rstd
        smax = jnp.max(sc, axis=1, keepdims=True)
        pos = (lane1 + (s * L + c)).astype(f32)
        sidx = jnp.min(jnp.where(sc == smax, pos, 1e9), axis=1, keepdims=True)
        new = jnp.concatenate([jnp.broadcast_to(smax, (1, 128)), jnp.broadcast_to(sidx, (1, 128)),
                               jnp.zeros((6, 128), f32)], axis=0)
        if t == 0:
            best_s[s] = new
        else:
            old = best_s[s]
            best_s[s] = jnp.where(smax > old[0:1, 0:1], new, old)

    def post(s, t):
        rstd = st_s[4 * s + t, 1:2]
        a = 1.0 + rstd
        b = st_s[4 * s + t, 0:1] * rstd
        out_s[s, :, pl.ds(128 * t, 128)] = (h_s[4 * s + t] * a - b).astype(bf)

    def finish(s):
        for t in range(4):
            out_proj(s, t)
            if t < 3:
                post(s, t)

    def attention(s):
        use_mem, update, o = s > 0, s < NSEG - 1, s % 2
        step(use_mem, update, o, (0, 0), None)
        if s > 0:
            for t in range(4):
                out_proj(s - 1, t)
                post(s - 1, t)
        for k in range(NQ // 2):
            step(use_mem, update, o, (k, 1), (k, 0))
            step(use_mem, update, o, (k + 1, 0) if k + 1 < NQ // 2 else None, (k, 1))
        if s > 0:
            out_copy(s - 1).start()

    half[0].wait()
    for t in range(2):
        prep(0, t)
    wq_lo.wait()
    w_copies[1].start()
    wq_hi.start()
    augment(wq_s, 0, 512)
    for t in range(2):
        proj_q(t)
    half[1].wait()
    w_copies[2].start()
    for t in range(2, 4):
        prep(0, t)
        proj_q(t)
    w_copies[1].wait()
    wq_hi.wait()
    augment(wq_s, 512, D)
    w_copies[3].start()
    for s in range(1, NSEG):
        x_copy(s).start()
    augment(wk_s)
    w4_u[...] = _tou(jnp.concatenate([wq_s[:, 512:D], wk_s[:, 512:D]], axis=1))
    for t in range(2):
        proj_k(t)
    w_copies[2].wait()
    augment(wv_s)
    wvt_u[...] = _tou(wv_s[...].T)
    wv_ok = jnp.max(jnp.abs(wv_s[0:D, :].astype(f32))) < WV_MAX
    for t in range(2, 4):
        proj_k(t)
    w_copies[3].wait()
    for c in small:
        c.wait()
    g32 = jax.nn.sigmoid(beta_ref[...].astype(f32)).reshape(1, H)
    sel = _iota((H, H), 1) == _iota((H, H), 0)
    gcol = jnp.sum(jnp.where(sel, g32, 0.0), axis=1, keepdims=True)
    for c in range(NQ):
        g_s[c, 0:4] = jnp.broadcast_to(gcol[4 * c:4 * c + 4], (4, 128))
    wr_s[...] = jnp.broadcast_to(wr_ref[...].astype(f32).reshape(1, D), (128, D)).T
    wrs_s[...] = jnp.broadcast_to(jnp.sum(wr_s[...], axis=0, keepdims=True), (8, 128))
    wot_u[...] = _tou(wo_s[...].T)
    for t in range(4):
        proj_v(0, t)
    attention(0)
    for s in range(1, NSEG):
        x_copy(s).wait()

    for s in range(1, NSEG):
        e_copies[s - 1].start()
        for t in range(4):
            prep(s, t)
        for t in range(4):
            proj_v(s, t)
        for t in range(4):
            proj_q(t)
            proj_k(t)
        attention(s)
    finish(NSEG - 1)
    post(NSEG - 1, 3)
    out_copy(NSEG - 1).start()

    dl = den_s[...]
    safe = jnp.logical_and(jnp.min(dl[0:4]) >= DEN_LO, jnp.max(dl[4:8]) <= DEN_HI)
    safe = jnp.logical_and(safe, wv_ok)

    @pl.when(jnp.logical_not(safe))
    def _():
        for s in range(NSEG):
            out_copy(s).wait()
        m_f[...] = jnp.zeros_like(m_f)
        m_u[...] = jnp.zeros_like(m_u)

        def seg_redo(s, carry):
            for t in range(4):
                prep(s, t)
                proj_v(s, t)
                proj_q(t)
                proj_k(t)

            def quads(k, carry):
                for par in range(2):
                    for j in range(4):
                        stage_a_safe(k, par, j, pb[par])
                        stage_b(True, s % 2, k, par, j, pb[par], swapped=False)
                    mem_update(k, par)
                return carry
            lax.fori_loop(0, NQ // 2, quads, 0)
            finish(s)
            post(s, 3)
            out_copy(s).start()
            return carry
        lax.fori_loop(0, NSEG, seg_redo, 0)

    for c in e_copies:
        c.wait()
    best = best_s[0]
    for s in range(1, NSEG):
        cand = best_s[s]
        best = jnp.where(cand[0:1, 0:1] > best[0:1, 0:1], cand, best)
    idx = jnp.clip(best[1, 0].astype(i32), 0, S - 1)
    blk = idx // 128
    col = idx - blk * 128
    onehot = ((_iota((16, 128), 1) == col) & (_iota((16, 128), 0) == 0)).astype(bf)
    ln = ((h_s[blk] - st_s[blk, 0:1]) * st_s[blk, 1:2]).astype(bf)
    xs = _dot_nt(onehot, ln).astype(bf)
    pick = (_iota((128, 128), 0) == col).astype(bf)
    xcol = _dot(ln, pick)
    fm = F - 128 * GU_VPU

    def first_layer(w_ref):
        acc = jnp.zeros((8, 128 * GU_VPU), f32)
        for i in range(D // 8):
            w = w_ref[8 * i:8 * i + 8, fm:F].astype(f32)
            acc = acc + w * jnp.concatenate([xcol[8 * i:8 * i + 8]] * GU_VPU, axis=1)
        return jnp.concatenate([_dot(xs, w_ref[:, 0:fm])[0:1],
                                jnp.sum(acc, axis=0, keepdims=True)], axis=1)
    gate = first_layer(wg_s)
    up = first_layer(wu_s)
    act = (gate * jax.nn.sigmoid(gate) * up).astype(bf)
    actf = act.astype(f32)
    fd = F - 128 * DN_VPU
    y = _dot_nt(jnp.broadcast_to(act[:, 0:fd], (16, fd)), wd_s[:, 0:fd])
    parts = []
    for i in range(D // 8):
        w = wd_s[8 * i:8 * i + 8, fd:F].astype(f32) * actf[:, fd:F]
        tot = w[:, 0:128]
        for c in range(1, DN_VPU):
            tot = tot + w[:, 128 * c:128 * (c + 1)]
        parts.append(tot)
    yv = jnp.sum(jnp.concatenate(parts, axis=0), axis=1, keepdims=True)
    yt = (jnp.broadcast_to(y[0:1], (128, D)).T + yv) * jax.nn.sigmoid(best[0:1, 0:1])
    for s in range(NSEG):
        out_copy(s).wait()
    seg = blk // 4
    c0 = pl.multiple_of((blk - seg * 4) * 128, 128)
    cur = out_s[seg, :, pl.ds(c0, 128)].astype(f32)
    hit = _iota((D, 128), 1) == col
    fin_s[...] = (cur + jnp.where(hit, yt, 0.0)).astype(bf)
    fin = cp(fin_s, out_hbm.at[:, pl.ds(pl.multiple_of(blk * 128, 128), 128)], sems.at[15])
    fin.start()
    fin.wait()


@jax.jit
def pallas_sequential_preLN__memory_aug_infini_attn__moe_arch_mod__prompt_kernel(
    A_x, A_wq, A_wk, A_wv, A_wo, A_beta, B_x, B_w_r, B_w_gate, B_w_up, B_w_down,
):
    hbm = pl.BlockSpec(memory_space=pltpu.HBM)
    vm = pltpu.VMEM
    x_t = A_x.reshape(S, D).T
    out_t = pl.pallas_call(
        _kernel,
        out_shape=jax.ShapeDtypeStruct((D, S), bf),
        in_specs=[hbm] * 10,
        out_specs=hbm,
        scratch_shapes=[
            vm((NSEG, DP, L), bf), vm((DP, D), bf), vm((DP, D), bf), vm((DP, D), bf), vm((D, D), bf),
            vm((D, F), bf), vm((D, F), bf), vm((D, F), bf),
            vm((DP // 2, 128), u32), vm((D // 2, DP), u32), vm((D // 2, D), u32),
            vm((L // 2, DP), u32), vm((4, 8, 128), f32), vm((4, 128, 128), f32),
            vm((NQ, L // 2, 128), u32), vm((NQ, L // 2, 128), u32),
            vm((NQ, L // 2, 128), u32), vm((NQ, L // 2, 128), u32),
            vm((D // 2, L), u32),
            vm((640, 512), u32), vm((640, 512), u32), vm((16, D, 128), f32),
            vm((2, D, L), f32), vm((NQ, 80, 128), f32), vm((NQ, 40, 128), u32),
            vm((NQ, 8, 128), f32), vm((D, 128), f32), vm((8, 128), f32), vm((NSEG, D, L), bf),
            vm((16, 8, 128), f32),
            vm((NSEG, 8, 128), f32), vm((8, 128), f32), vm((D, 128), bf),
            vm((H,), bf), vm((D,), bf),
            pltpu.SemaphoreType.DMA((20,)),
        ],
        compiler_params=pltpu.CompilerParams(vmem_limit_bytes=100 * 1024 * 1024),
        name="infini_moe",
    )(x_t, A_wq, A_wk, A_wv, A_wo, A_beta, B_w_r, B_w_gate, B_w_up, B_w_down.T)
    return out_t.T.reshape(1, S, D)
```

```python
import jax
import jax.numpy as jnp
from jax import lax
from jax.experimental import pallas as pl
from jax.experimental.pallas import tpu as pltpu

S, D, H, DH = 2048, 576, 32, 18
NSEG, L, F = 4, 512, 4608
DP = 640
NQ = 8
QW = 4 * DH
bf, u32, f32, i32 = jnp.bfloat16, jnp.uint32, jnp.float32, jnp.int32
LOG2E = 1.4426950408889634
QSCALE = DH ** -0.5 * LOG2E
MASKB = -1000000000.0 * LOG2E
EPS = 1e-5
NT = (((1,), (1,)), ((), ()))
ONES2 = 0x3F803F80
GU_VPU = 11
DN_VPU = 26
DEN_LO, DEN_HI, WV_MAX = 2.0 ** -60, 2.0 ** 60, 2.0 ** 40


def _tobf(x):
    return pltpu.bitcast(x, bf)


def _tou(x):
    return pltpu.bitcast(x, u32)


def _pack(x):
    return pltpu.bitcast(x.astype(bf), u32)


def _dot(a, b):
    return jnp.dot(a, b, preferred_element_type=f32)


def _dot_nt(a, b):
    return lax.dot_general(a, b, NT, preferred_element_type=f32)


def _phi(t):
    return jnp.where(t > 0, t + 1.0, jnp.exp(t))


def _rowsum(parts):
    acc = [jnp.sum(p.reshape(p.shape[0] // 8, 8, 128), axis=0) for p in parts]
    while len(acc) > 1:
        acc = [acc[i] + acc[i + 1] for i in range(0, len(acc), 2)]
    return jnp.sum(acc[0], axis=0, keepdims=True)


def _ln_stats(rows, w=None):
    d = [rows(144 * g, 144 * (g + 1)) for g in range(4)]
    m1 = _rowsum(d) * (1.0 / D)
    m2 = _rowsum([v * v for v in d]) * (1.0 / D)
    var = jnp.maximum(m2 - m1 * m1, 0.0)
    rstd = lax.rsqrt(var + EPS)
    if w is None:
        return m1, rstd
    dw = _rowsum([d[g] * w[0][144 * g:144 * (g + 1)] for g in range(4)])
    return m1, rstd, (dw - m1 * w[1]) * rstd


def _hi_lo(v):
    hi = v.astype(bf).astype(f32)
    return hi, (v - hi).astype(bf).astype(f32)


def _iota(shape, dim):
    return lax.broadcasted_iota(i32, shape, dim)


def _al(x, n):
    return x if isinstance(x, int) else pl.multiple_of(x, n)


def _kernel(x_hbm, wq_hbm, wk_hbm, wv_hbm, wo_hbm, beta_hbm, wr_hbm,
            wg_hbm, wu_hbm, wd_hbm, out_hbm,
            x_s, wq_s, wk_s, wv_s, wo_s, wg_s, wu_s, wd_s,
            w4_u, wvt_u, wot_u, xn_u, rs_s, rc_s, qx, kx, pqx, pkx, vt_u,
            p0, p1, h_s, ot_s, m_f, m_u, g_s, wr_s, wrs_s, out_s, st_s, best_s, den_s, fin_s,
            beta_ref, wr_ref, sems):
    cp = pltpu.make_async_copy

    def x_copy(s):
        return cp(x_hbm.at[:, pl.ds(_al(s * L, L), L)], x_s.at[s, pl.ds(0, D), :], sems.at[s])

    def out_copy(s):
        return cp(out_s.at[s], out_hbm.at[:, pl.ds(_al(s * L, L), L)], sems.at[11 + s])

    def prep(s, t):
        c = 128 * t
        mean, rstd = _ln_stats(lambda a, b: x_s[s, a:b, pl.ds(c, 128)].astype(f32))
        mh, ml = _hi_lo(mean)
        r16 = _iota((16, 128), 0)
        x_s[s, D:D + 16, pl.ds(c, 128)] = jnp.where(
            r16 < 2, mh, jnp.where(r16 == 2, ml, 0.0)).astype(bf)
        rs_s[t, 0:1] = rstd
        rc_s[t] = jnp.broadcast_to(rstd, (128, 128)).T
        xn_u[pl.ds(64 * t, 64), :] = _tou(x_s[s, :, pl.ds(c, 128)].T)

    def augment(w_ref, a=0, b=D):
        ones = jnp.ones((16, D), bf)
        hi, lo = _hi_lo(_dot(ones, w_ref[0:D, a:b])[0:1])
        r16 = _iota((16, b - a), 0)
        w_ref[D:D + 16, a:b] = jnp.where((r16 == 0) | (r16 == 2), -hi,
                                         jnp.where(r16 == 1, -lo, 0.0)).astype(bf)

    top = pl.ds(0, D)
    w_copies = [None, cp(wk_hbm, wk_s.at[top, :], sems.at[5]),
                cp(wv_hbm, wv_s.at[top, :], sems.at[6]), cp(wo_hbm, wo_s, sems.at[7])]
    e_copies = [cp(wg_hbm, wg_s, sems.at[8]), cp(wu_hbm, wu_s, sems.at[9]),
                cp(wd_hbm, wd_s, sems.at[10])]

    small = [cp(beta_hbm, beta_ref, sems.at[16]), cp(wr_hbm, wr_ref, sems.at[17])]
    half = [cp(x_hbm.at[:, pl.ds(256 * i, 256)], x_s.at[0, top, pl.ds(256 * i, 256)],
               sems.at[18 * i]) for i in range(2)]
    wq_lo = cp(wq_hbm.at[:, pl.ds(0, 512)], wq_s.at[top, pl.ds(0, 512)], sems.at[4])
    wq_hi = cp(wq_hbm.at[:, pl.ds(512, D - 512)], wq_s.at[top, pl.ds(512, D - 512)], sems.at[19])
    half[0].start()
    wq_lo.start()
    half[1].start()
    for c in small:
        c.start()

    m_f[...] = jnp.zeros_like(m_f)
    den_s[...] = jnp.ones_like(den_s)

    for w_ref in (wq_s, wk_s, wv_s):
        w_ref[D + 16:DP, :] = jnp.zeros((DP - D - 16, D), bf)
    for s in range(NSEG):
        x_s[s, D + 16:DP, :] = jnp.zeros((DP - D - 16, L), bf)

    lane1 = _iota((1, 128), 1)
    causal = _iota((128, 128), 0) <= _iota((128, 128), 1)

    def proj_q(t):
        rows = pl.ds(64 * t, 64)
        q = _dot(_tobf(xn_u[rows, :]), wq_s[:, 0:512]) * jnp.concatenate([rc_s[t]] * 4, axis=1)
        tiles = [q[:, 128 * i:128 * (i + 1)] for i in range(4)]
        raw = [_pack(v * QSCALE) for v in tiles]
        ph = [_pack(_phi(v)) for v in tiles]
        for c in range(NQ):
            i = c // 2
            if c % 2 == 0 or c == NQ - 1:
                qx[c, rows, :] = raw[i]
                pqx[c, rows, :] = ph[i]
            else:
                keep = lane1 >= (QW * c) % 128
                qx[c, rows, :] = jnp.where(keep, raw[i], raw[i + 1])
                pqx[c, rows, :] = jnp.where(keep, ph[i], ph[i + 1])

    def proj_k(t):
        rows = pl.ds(64 * t, 64)
        xn = _tobf(xn_u[rows, :])
        rc = rc_s[t]
        k = _dot(xn, wk_s[:, 0:512]) * jnp.concatenate([rc] * 4, axis=1)
        r4 = _dot(xn, _tobf(w4_u[...])) * rc
        tiles = [k[:, 128 * i:128 * (i + 1)] for i in range(4)] + [pltpu.roll(r4, 64, 1)]
        raw = [_pack(v) for v in tiles]
        ph = [_pack(_phi(v)) for v in tiles]
        for c in range(NQ):
            i = c // 2
            if c % 2 == 0:
                kx[c, rows, :] = raw[i]
                pkx[c, rows, :] = ph[i]
            else:
                keep = lane1 >= (QW * c) % 128
                kx[c, rows, :] = jnp.where(keep, raw[i], raw[i + 1])
                pkx[c, rows, :] = jnp.where(keep, ph[i], ph[i + 1])
        keep = lane1 >= (QW * (NQ - 1)) % 128
        qx[NQ - 1, rows, :] = jnp.where(keep, qx[NQ - 1, rows, :], _pack(r4 * QSCALE))
        pqx[NQ - 1, rows, :] = jnp.where(keep, pqx[NQ - 1, rows, :], _pack(_phi(r4)))

    def proj_v(s, t):
        vt = _dot(_tobf(wvt_u[...]), x_s[s, :, pl.ds(128 * t, 128)]) * rs_s[t, 0:1]
        vt_u[:, pl.ds(128 * t, 128)] = _pack(vt)

    def masked_q(k, par, j):
        q = qx[2 * k + par, pl.ds(64 * j, 64), :]
        out = []
        for i in range(4):
            st = (2 * QW * k + QW * par + DH * i) % 128
            out.append(q & jnp.where(((lane1 - st) & 127) < DH, jnp.uint32(0xFFFFFFFF),
                                     jnp.uint32(0)))
        return out

    def scores(k, par, j):
        qm = _tobf(jnp.concatenate(masked_q(k, par, j), axis=0))
        kk = _tobf(kx[2 * k + par, pl.ds(0, 64 * (j + 1)), :])
        return _dot_nt(kk, qm)

    r64, l64 = _iota((64, 128), 0), _iota((64, 128), 1)
    lo_nat = (l64 >= 64) | (r64 <= l64)
    lo_swp = (l64 < 64) | (r64 <= l64 - 64)
    hi_even = (l64 < 64) & (r64 <= l64)
    hi_odd = (l64 >= 64) & (r64 <= l64 - 64)

    def stage_a(k, par, j, p_ref):
        c = 2 * k + par
        qm = masked_q(k, par, j)
        w1 = [jnp.concatenate([qm[i][32:], qm[i][:32]], axis=0) if i % 2 == 0 else qm[i]
              for i in range(4)]
        w2 = [qm[i][32:] for i in range(4)]
        n1 = 128 * j + 64
        p1 = jnp.exp2(_dot_nt(_tobf(kx[c, pl.ds(0, n1 // 2), :]),
                              _tobf(jnp.concatenate(w1, axis=0))))
        p2 = jnp.exp2(_dot_nt(_tobf(kx[c, pl.ds(n1 // 2, 32), :]),
                              _tobf(jnp.concatenate(w2, axis=0))))
        off = 64 * (j * (j + 1) // 2)
        if j > 0:
            p_ref[pl.ds(off, 64 * j), :] = _pack(p1[:128 * j])
        lo = [jnp.where(lo_swp if i % 2 == 0 else lo_nat,
                        p1[128 * j:, 128 * i:128 * (i + 1)], 0.0) for i in range(4)]
        hi = [jnp.where(hi_even if i % 2 == 0 else hi_odd,
                        p2[:, 128 * (i // 2):128 * (i // 2 + 1)], 0.0) for i in range(4)]
        p_ref[pl.ds(off + 64 * j, 32), :] = _pack(jnp.concatenate(lo, axis=1))
        p_ref[pl.ds(off + 64 * j + 32, 32), :] = _pack(jnp.concatenate(hi, axis=1))

    def stage_a_safe(k, par, j, p_ref):
        s = scores(k, par, j)
        bias = jnp.where(causal, 0.0, MASKB).astype(f32)
        sd = s[128 * j:] + jnp.concatenate([bias] * 4, axis=1)
        s = sd if j == 0 else jnp.concatenate([s[:128 * j], sd], axis=0)
        p = jnp.exp2(s - jnp.max(s, axis=0, keepdims=True))
        p_ref[pl.ds(64 * (j * (j + 1) // 2), 64 * (j + 1)), :] = _pack(p)

    def stage_b(use_mem, oslot, k, par, j, p_ref, swapped=True):
        c = 2 * k + par
        base = QW * par
        mwin = base - base % 16
        moff = base - mwin
        zrow = 72 if moff == 0 else 0
        srow = _iota((8, 128), 0)
        g8 = g_s[c]
        off = 64 * (j * (j + 1) // 2)
        accs, dens = [], []
        for i in range(4):
            r0 = base + DH * i
            w = r0 - r0 % 16
            o = r0 - w
            vt = vt_u[pl.ds(_al(QW * k + w // 2, 8), 16), pl.ds(0, 128 * (j + 1))]
            orow = 15 if o < 14 else 0
            vt = jnp.where(_iota(vt.shape, 0) == orow, jnp.uint32(ONES2), vt)
            p = _tobf(p_ref[pl.ds(off, 64 * (j + 1)), pl.ds(128 * i, 128)])
            acc = _dot(_tobf(vt), p)
            if swapped and i % 2 == 0:
                acc = pltpu.roll(acc, 64, 1)
            dens.append(acc[2 * orow:2 * orow + 1])
            a0 = o - o % 8
            accs.append(acc[a0:a0 + 24])
        den4 = jnp.concatenate(dens, axis=0)
        den_s[0:4] = jnp.minimum(den_s[0:4], den4)
        den_s[4:8] = jnp.maximum(den_s[4:8], den4)
        if use_mem:
            mem = _dot_nt(_tobf(m_u[c]), _tobf(pqx[c, pl.ds(64 * j, 64), :]))
            r8 = g8 / jnp.concatenate([den4, mem[zrow:zrow + 4] + 1e-6], axis=0)
            rms = [r8[4 + i:5 + i] for i in range(4)]
        else:
            r8 = g8[0:4] / den4
        rds = [r8[i:i + 1] for i in range(4)]
        for v in range(9):
            lo_h, hi_h = (8 * v) // DH, (8 * v + 7) // DH

            def piece(h):
                a = accs[h][8 * (v - (DH * h) // 8):8 * (v - (DH * h) // 8) + 8]
                if not use_mem:
                    return a * rds[h]
                return a * rds[h] + mem[moff + 8 * v:moff + 8 * v + 8] * rms[h]
            val = piece(lo_h)
            if hi_h != lo_h:
                val = jnp.where(srow < DH * hi_h - 8 * v, val, piece(hi_h))
            ot_s[oslot, pl.ds(_al(2 * QW * k + base + 8 * v, 8), 8), pl.ds(128 * j, 128)] = val

    def mem_update(k, par):
        c = 2 * k + par
        base = QW * par
        mwin = base - base % 16
        moff = base - mwin
        zrow = 72 if moff == 0 else 0
        vw = vt_u[pl.ds(_al(QW * k + mwin // 2, 8), 40), :]
        rr = _iota(vw.shape, 0)
        isz = (rr >= 36) if moff == 0 else (rr < 4)
        vw = jnp.where(isz, jnp.uint32(ONES2), vw)
        upd = _dot(_tobf(vw), _tobf(pkx[c]))
        r80 = _iota((80, 128), 0)
        l80 = (_iota((80, 128), 1) - (2 * QW * k + base)) & 127
        hrow = jnp.where((r80 >= zrow) & (r80 < zrow + 8), r80 - zrow, (r80 - moff) // DH)
        keep = (l80 >= DH * hrow) & (l80 < DH * hrow + DH) & (hrow < 4) & (hrow >= 0)
        mnew = m_f[c] + jnp.where(keep, upd, 0.0)
        m_f[c] = mnew
        m_u[c] = _pack(mnew)

    pb = (p0, p1)

    def step(use_mem, update, oslot, a, b):
        for j in (3, 2, 1, 0):
            if a is not None:
                stage_a(a[0], a[1], j, pb[a[1]])
        for j in range(4):
            if b is not None:
                stage_b(use_mem, oslot, b[0], b[1], j, pb[b[1]])
        if b is not None and update:
            mem_update(b[0], b[1])

    def out_proj(s, t):
        c = 128 * t
        o = ot_s[s % 2, :, pl.ds(c, 128)].astype(bf)
        h = x_s[s, 0:D, pl.ds(c, 128)].astype(f32) + _dot(_tobf(wot_u[...]), o)
        h_s[4 * s + t] = h
        mean, rstd, sc = _ln_stats(lambda a, b: h[a:b], (wr_s[...], wrs_s[0:1]))
        st_s[4 * s + t, 0:1] = mean
        st_s[4 * s + t, 1:2] = rstd
        smax = jnp.max(sc, axis=1, keepdims=True)
        pos = (lane1 + (s * L + c)).astype(f32)
        sidx = jnp.min(jnp.where(sc == smax, pos, 1e9), axis=1, keepdims=True)
        new = jnp.concatenate([jnp.broadcast_to(smax, (1, 128)), jnp.broadcast_to(sidx, (1, 128)),
                               jnp.zeros((6, 128), f32)], axis=0)
        if t == 0:
            best_s[s] = new
        else:
            old = best_s[s]
            best_s[s] = jnp.where(smax > old[0:1, 0:1], new, old)

    def post(s, t):
        rstd = st_s[4 * s + t, 1:2]
        a = 1.0 + rstd
        b = st_s[4 * s + t, 0:1] * rstd
        out_s[s, :, pl.ds(128 * t, 128)] = (h_s[4 * s + t] * a - b).astype(bf)

    def finish(s):
        for t in range(4):
            out_proj(s, t)
            if t < 3:
                post(s, t)

    def attention(s):
        use_mem, update, o = s > 0, s < NSEG - 1, s % 2
        if s > 0:
            for t in range(4):
                out_proj(s - 1, t)
                post(s - 1, t)
        step(use_mem, update, o, (0, 0), None)
        for k in range(NQ // 2):
            step(use_mem, update, o, (k, 1), (k, 0))
            step(use_mem, update, o, (k + 1, 0) if k + 1 < NQ // 2 else None, (k, 1))
        if s > 0:
            out_copy(s - 1).start()

    half[0].wait()
    for t in range(2):
        prep(0, t)
    wq_lo.wait()
    w_copies[1].start()
    wq_hi.start()
    augment(wq_s, 0, 512)
    for t in range(2):
        proj_q(t)
    half[1].wait()
    w_copies[2].start()
    for t in range(2, 4):
        prep(0, t)
        proj_q(t)
    w_copies[1].wait()
    wq_hi.wait()
    augment(wq_s, 512, D)
    w_copies[3].start()
    for s in range(1, NSEG):
        x_copy(s).start()
    augment(wk_s)
    w4_u[...] = _tou(jnp.concatenate([wq_s[:, 512:D], wk_s[:, 512:D]], axis=1))
    for t in range(2):
        proj_k(t)
    w_copies[2].wait()
    augment(wv_s)
    wvt_u[...] = _tou(wv_s[...].T)
    wv_ok = jnp.max(jnp.abs(wv_s[0:D, :].astype(f32))) < WV_MAX
    for t in range(2, 4):
        proj_k(t)
    w_copies[3].wait()
    for c in small:
        c.wait()
    g32 = jax.nn.sigmoid(beta_ref[...].astype(f32)).reshape(1, H)
    sel = _iota((H, H), 1) == _iota((H, H), 0)
    gcol = jnp.sum(jnp.where(sel, g32, 0.0), axis=1, keepdims=True)
    for c in range(NQ):
        gq = jnp.broadcast_to(gcol[4 * c:4 * c + 4], (4, 128))
        g_s[c] = jnp.concatenate([1.0 - gq, gq], axis=0)
    wr_s[...] = jnp.broadcast_to(wr_ref[...].astype(f32).reshape(1, D), (128, D)).T
    wrs_s[...] = jnp.broadcast_to(jnp.sum(wr_s[...], axis=0, keepdims=True), (8, 128))
    wot_u[...] = _tou(wo_s[...].T)
    for t in range(4):
        proj_v(0, t)
    attention(0)
    for s in range(1, NSEG):
        x_copy(s).wait()

    for s in range(1, NSEG):
        e_copies[s - 1].start()
        for t in range(4):
            prep(s, t)
        for t in range(4):
            proj_v(s, t)
        for t in range(4):
            proj_q(t)
            proj_k(t)
        attention(s)
    finish(NSEG - 1)
    post(NSEG - 1, 3)
    out_copy(NSEG - 1).start()

    dl = den_s[...]
    safe = jnp.logical_and(jnp.min(dl[0:4]) >= DEN_LO, jnp.max(dl[4:8]) <= DEN_HI)
    safe = jnp.logical_and(safe, wv_ok)

    @pl.when(jnp.logical_not(safe))
    def _():
        for s in range(NSEG):
            out_copy(s).wait()
        m_f[...] = jnp.zeros_like(m_f)
        m_u[...] = jnp.zeros_like(m_u)

        def seg_redo(s, carry):
            for t in range(4):
                prep(s, t)
                proj_v(s, t)
                proj_q(t)
                proj_k(t)

            def quads(k, carry):
                for par in range(2):
                    for j in range(4):
                        stage_a_safe(k, par, j, pb[par])
                        stage_b(True, s % 2, k, par, j, pb[par], swapped=False)
                    mem_update(k, par)
                return carry
            lax.fori_loop(0, NQ // 2, quads, 0)
            finish(s)
            post(s, 3)
            out_copy(s).start()
            return carry
        lax.fori_loop(0, NSEG, seg_redo, 0)

    for c in e_copies:
        c.wait()
    best = best_s[0]
    for s in range(1, NSEG):
        cand = best_s[s]
        best = jnp.where(cand[0:1, 0:1] > best[0:1, 0:1], cand, best)
    idx = jnp.clip(best[1, 0].astype(i32), 0, S - 1)
    blk = idx // 128
    col = idx - blk * 128
    onehot = ((_iota((16, 128), 1) == col) & (_iota((16, 128), 0) == 0)).astype(bf)
    ln = ((h_s[blk] - st_s[blk, 0:1]) * st_s[blk, 1:2]).astype(bf)
    xs = _dot_nt(onehot, ln).astype(bf)
    pick = (_iota((128, 128), 0) == col).astype(bf)
    xcol = _dot(ln, pick)
    fm = F - 128 * GU_VPU

    def first_layer(w_ref):
        acc = jnp.zeros((8, 128 * GU_VPU), f32)
        for i in range(D // 8):
            w = w_ref[8 * i:8 * i + 8, fm:F].astype(f32)
            acc = acc + w * jnp.concatenate([xcol[8 * i:8 * i + 8]] * GU_VPU, axis=1)
        return jnp.concatenate([_dot(xs, w_ref[:, 0:fm])[0:1],
                                jnp.sum(acc, axis=0, keepdims=True)], axis=1)
    gate = first_layer(wg_s)
    up = first_layer(wu_s)
    act = (gate * jax.nn.sigmoid(gate) * up).astype(bf)
    actf = act.astype(f32)
    fd = F - 128 * DN_VPU
    y = _dot_nt(jnp.broadcast_to(act[:, 0:fd], (16, fd)), wd_s[:, 0:fd])
    parts = []
    for i in range(D // 8):
        w = wd_s[8 * i:8 * i + 8, fd:F].astype(f32) * actf[:, fd:F]
        tot = w[:, 0:128]
        for c in range(1, DN_VPU):
            tot = tot + w[:, 128 * c:128 * (c + 1)]
        parts.append(tot)
    yv = jnp.sum(jnp.concatenate(parts, axis=0), axis=1, keepdims=True)
    yt = (jnp.broadcast_to(y[0:1], (128, D)).T + yv) * jax.nn.sigmoid(best[0:1, 0:1])
    for s in range(NSEG):
        out_copy(s).wait()
    seg = blk // 4
    c0 = pl.multiple_of((blk - seg * 4) * 128, 128)
    cur = out_s[seg, :, pl.ds(c0, 128)].astype(f32)
    hit = _iota((D, 128), 1) == col
    fin_s[...] = (cur + jnp.where(hit, yt, 0.0)).astype(bf)
    fin = cp(fin_s, out_hbm.at[:, pl.ds(pl.multiple_of(blk * 128, 128), 128)], sems.at[15])
    fin.start()
    fin.wait()


@jax.jit
def pallas_sequential_preLN__memory_aug_infini_attn__moe_arch_mod__prompt_kernel(
    A_x, A_wq, A_wk, A_wv, A_wo, A_beta, B_x, B_w_r, B_w_gate, B_w_up, B_w_down,
):
    hbm = pl.BlockSpec(memory_space=pltpu.HBM)
    vm = pltpu.VMEM
    x_t = A_x.reshape(S, D).T
    out_t = pl.pallas_call(
        _kernel,
        out_shape=jax.ShapeDtypeStruct((D, S), bf),
        in_specs=[hbm] * 10,
        out_specs=hbm,
        scratch_shapes=[
            vm((NSEG, DP, L), bf), vm((DP, D), bf), vm((DP, D), bf), vm((DP, D), bf), vm((D, D), bf),
            vm((D, F), bf), vm((D, F), bf), vm((D, F), bf),
            vm((DP // 2, 128), u32), vm((D // 2, DP), u32), vm((D // 2, D), u32),
            vm((L // 2, DP), u32), vm((4, 8, 128), f32), vm((4, 128, 128), f32),
            vm((NQ, L // 2, 128), u32), vm((NQ, L // 2, 128), u32),
            vm((NQ, L // 2, 128), u32), vm((NQ, L // 2, 128), u32),
            vm((D // 2, L), u32),
            vm((640, 512), u32), vm((640, 512), u32), vm((16, D, 128), f32),
            vm((2, D, L), f32), vm((NQ, 80, 128), f32), vm((NQ, 40, 128), u32),
            vm((NQ, 8, 128), f32), vm((D, 128), f32), vm((8, 128), f32), vm((NSEG, D, L), bf),
            vm((16, 8, 128), f32),
            vm((NSEG, 8, 128), f32), vm((8, 128), f32), vm((D, 128), bf),
            vm((H,), bf), vm((D,), bf),
            pltpu.SemaphoreType.DMA((20,)),
        ],
        compiler_params=pltpu.CompilerParams(vmem_limit_bytes=100 * 1024 * 1024),
        name="infini_moe",
    )(x_t, A_wq, A_wk, A_wv, A_wo, A_beta, B_w_r, B_w_gate, B_w_up, B_w_down.T)
    return out_t.T.reshape(1, S, D)
```

```python
import jax
import jax.numpy as jnp
from jax import lax
from jax.experimental import pallas as pl
from jax.experimental.pallas import tpu as pltpu

S, D, H, DH = 2048, 576, 32, 18
NSEG, L, F = 4, 512, 4608
DP = 640
NQ = 8
QW = 4 * DH
bf, u32, f32, i32 = jnp.bfloat16, jnp.uint32, jnp.float32, jnp.int32
LOG2E = 1.4426950408889634
QSCALE = DH ** -0.5 * LOG2E
MASKB = -1000000000.0 * LOG2E
EPS = 1e-5
NT = (((1,), (1,)), ((), ()))
ONES2 = 0x3F803F80
E_GRP = 256
DEN_LO, DEN_HI, WV_MAX = 2.0 ** -60, 2.0 ** 60, 2.0 ** 40


def _tobf(x):
    return pltpu.bitcast(x, bf)


def _tou(x):
    return pltpu.bitcast(x, u32)


def _pack(x):
    return pltpu.bitcast(x.astype(bf), u32)


def _dot(a, b):
    return jnp.dot(a, b, preferred_element_type=f32)


def _dot_nt(a, b):
    return lax.dot_general(a, b, NT, preferred_element_type=f32)


def _phi(t):
    return jnp.where(t > 0, t + 1.0, jnp.exp(t))


def _rowsum(parts):
    acc = [jnp.sum(p.reshape(p.shape[0] // 8, 8, 128), axis=0) for p in parts]
    while len(acc) > 1:
        acc = [acc[i] + acc[i + 1] for i in range(0, len(acc), 2)]
    return jnp.sum(acc[0], axis=0, keepdims=True)


def _ln_stats(rows, w=None):
    d = [rows(144 * g, 144 * (g + 1)) for g in range(4)]
    m1 = _rowsum(d) * (1.0 / D)
    m2 = _rowsum([v * v for v in d]) * (1.0 / D)
    var = jnp.maximum(m2 - m1 * m1, 0.0)
    rstd = lax.rsqrt(var + EPS)
    if w is None:
        return m1, rstd
    dw = _rowsum([d[g] * w[0][144 * g:144 * (g + 1)] for g in range(4)])
    return m1, rstd, (dw - m1 * w[1]) * rstd


def _hi_lo(v):
    hi = v.astype(bf).astype(f32)
    return hi, (v - hi).astype(bf).astype(f32)


def _iota(shape, dim):
    return lax.broadcasted_iota(i32, shape, dim)


def _al(x, n):
    return x if isinstance(x, int) else pl.multiple_of(x, n)


def _kernel(x_hbm, wq_hbm, wk_hbm, wv_hbm, wo_hbm, beta_hbm, wr_hbm,
            wg_hbm, wu_hbm, wd_hbm, out_hbm,
            x_s, wq_s, wk_s, wv_s, wo_s, wg_s, wu_s, wd_s,
            w4_u, wvt_u, wot_u, xn_u, rs_s, rc_s, qx, kx, pqx, pkx, vt_u,
            p0, p1, h_s, ot_s, m_f, m_u, g_s, wr_s, wrs_s, out_s, st_s, best_s, den_s, fin_s,
            beta_ref, wr_ref, sems):
    cp = pltpu.make_async_copy

    def x_copy(s):
        return cp(x_hbm.at[:, pl.ds(_al(s * L, L), L)], x_s.at[s, pl.ds(0, D), :], sems.at[s])

    def out_copy(s):
        return cp(out_s.at[s], out_hbm.at[:, pl.ds(_al(s * L, L), L)], sems.at[11 + s])

    def prep(s, t):
        c = 128 * t
        mean, rstd = _ln_stats(lambda a, b: x_s[s, a:b, pl.ds(c, 128)].astype(f32))
        mh, ml = _hi_lo(mean)
        r16 = _iota((16, 128), 0)
        x_s[s, D:D + 16, pl.ds(c, 128)] = jnp.where(
            r16 < 2, mh, jnp.where(r16 == 2, ml, 0.0)).astype(bf)
        rs_s[t, 0:1] = rstd
        rc_s[t] = jnp.broadcast_to(rstd, (128, 128)).T
        xn_u[pl.ds(64 * t, 64), :] = _tou(x_s[s, :, pl.ds(c, 128)].T)

    def augment(w_ref, a=0, b=D):
        ones = jnp.ones((16, D), bf)
        hi, lo = _hi_lo(_dot(ones, w_ref[0:D, a:b])[0:1])
        r16 = _iota((16, b - a), 0)
        w_ref[D:D + 16, a:b] = jnp.where((r16 == 0) | (r16 == 2), -hi,
                                         jnp.where(r16 == 1, -lo, 0.0)).astype(bf)

    top = pl.ds(0, D)
    w_copies = [None, cp(wk_hbm, wk_s.at[top, :], sems.at[5]),
                cp(wv_hbm, wv_s.at[top, :], sems.at[6]), cp(wo_hbm, wo_s, sems.at[7])]
    e_copies = [cp(wg_hbm, wg_s, sems.at[8]), cp(wu_hbm, wu_s, sems.at[9]),
                cp(wd_hbm, wd_s, sems.at[10])]

    small = [cp(beta_hbm, beta_ref, sems.at[16]), cp(wr_hbm, wr_ref, sems.at[17])]
    half = [cp(x_hbm.at[:, pl.ds(256 * i, 256)], x_s.at[0, top, pl.ds(256 * i, 256)],
               sems.at[18 * i]) for i in range(2)]
    wq_lo = cp(wq_hbm.at[:, pl.ds(0, 512)], wq_s.at[top, pl.ds(0, 512)], sems.at[4])
    wq_hi = cp(wq_hbm.at[:, pl.ds(512, D - 512)], wq_s.at[top, pl.ds(512, D - 512)], sems.at[19])
    half[0].start()
    wq_lo.start()
    half[1].start()
    for c in small:
        c.start()

    m_f[...] = jnp.zeros_like(m_f)
    den_s[...] = jnp.ones_like(den_s)

    for w_ref in (wq_s, wk_s, wv_s):
        w_ref[D + 16:DP, :] = jnp.zeros((DP - D - 16, D), bf)
    for s in range(NSEG):
        x_s[s, D + 16:DP, :] = jnp.zeros((DP - D - 16, L), bf)

    lane1 = _iota((1, 128), 1)
    causal = _iota((128, 128), 0) <= _iota((128, 128), 1)

    def proj_q(t):
        rows = pl.ds(64 * t, 64)
        q = _dot(_tobf(xn_u[rows, :]), wq_s[:, 0:512]) * jnp.concatenate([rc_s[t]] * 4, axis=1)
        tiles = [q[:, 128 * i:128 * (i + 1)] for i in range(4)]
        raw = [_pack(v * QSCALE) for v in tiles]
        ph = [_pack(_phi(v)) for v in tiles]
        for c in range(NQ):
            i = c // 2
            if c % 2 == 0 or c == NQ - 1:
                qx[c, rows, :] = raw[i]
                pqx[c, rows, :] = ph[i]
            else:
                keep = lane1 >= (QW * c) % 128
                qx[c, rows, :] = jnp.where(keep, raw[i], raw[i + 1])
                pqx[c, rows, :] = jnp.where(keep, ph[i], ph[i + 1])

    def proj_k(t):
        rows = pl.ds(64 * t, 64)
        xn = _tobf(xn_u[rows, :])
        rc = rc_s[t]
        k = _dot(xn, wk_s[:, 0:512]) * jnp.concatenate([rc] * 4, axis=1)
        r4 = _dot(xn, _tobf(w4_u[...])) * rc
        tiles = [k[:, 128 * i:128 * (i + 1)] for i in range(4)] + [pltpu.roll(r4, 64, 1)]
        raw = [_pack(v) for v in tiles]
        ph = [_pack(_phi(v)) for v in tiles]
        for c in range(NQ):
            i = c // 2
            if c % 2 == 0:
                kx[c, rows, :] = raw[i]
                pkx[c, rows, :] = ph[i]
            else:
                keep = lane1 >= (QW * c) % 128
                kx[c, rows, :] = jnp.where(keep, raw[i], raw[i + 1])
                pkx[c, rows, :] = jnp.where(keep, ph[i], ph[i + 1])
        keep = lane1 >= (QW * (NQ - 1)) % 128
        qx[NQ - 1, rows, :] = jnp.where(keep, qx[NQ - 1, rows, :], _pack(r4 * QSCALE))
        pqx[NQ - 1, rows, :] = jnp.where(keep, pqx[NQ - 1, rows, :], _pack(_phi(r4)))

    def proj_v(s, t):
        vt = _dot(_tobf(wvt_u[...]), x_s[s, :, pl.ds(128 * t, 128)]) * rs_s[t, 0:1]
        vt_u[:, pl.ds(128 * t, 128)] = _pack(vt)

    def masked_q(k, par, j):
        q = qx[2 * k + par, pl.ds(64 * j, 64), :]
        out = []
        for i in range(4):
            st = (2 * QW * k + QW * par + DH * i) % 128
            out.append(q & jnp.where(((lane1 - st) & 127) < DH, jnp.uint32(0xFFFFFFFF),
                                     jnp.uint32(0)))
        return out

    def scores(k, par, j):
        qm = _tobf(jnp.concatenate(masked_q(k, par, j), axis=0))
        kk = _tobf(kx[2 * k + par, pl.ds(0, 64 * (j + 1)), :])
        return _dot_nt(kk, qm)

    r64, l64 = _iota((64, 128), 0), _iota((64, 128), 1)
    lo_nat = (l64 >= 64) | (r64 <= l64)
    lo_swp = (l64 < 64) | (r64 <= l64 - 64)
    hi_even = (l64 < 64) & (r64 <= l64)
    hi_odd = (l64 >= 64) & (r64 <= l64 - 64)

    def stage_a(k, par, j, p_ref):
        c = 2 * k + par
        qm = masked_q(k, par, j)
        w1 = [jnp.concatenate([qm[i][32:], qm[i][:32]], axis=0) if i % 2 == 0 else qm[i]
              for i in range(4)]
        w2 = [qm[i][32:] for i in range(4)]
        n1 = 128 * j + 64
        p1 = jnp.exp2(_dot_nt(_tobf(kx[c, pl.ds(0, n1 // 2), :]),
                              _tobf(jnp.concatenate(w1, axis=0))))
        p2 = jnp.exp2(_dot_nt(_tobf(kx[c, pl.ds(n1 // 2, 32), :]),
                              _tobf(jnp.concatenate(w2, axis=0))))
        off = 64 * (j * (j + 1) // 2)
        if j > 0:
            p_ref[pl.ds(off, 64 * j), :] = _pack(p1[:128 * j])
        lo = [jnp.where(lo_swp if i % 2 == 0 else lo_nat,
                        p1[128 * j:, 128 * i:128 * (i + 1)], 0.0) for i in range(4)]
        hi = [jnp.where(hi_even if i % 2 == 0 else hi_odd,
                        p2[:, 128 * (i // 2):128 * (i // 2 + 1)], 0.0) for i in range(4)]
        p_ref[pl.ds(off + 64 * j, 32), :] = _pack(jnp.concatenate(lo, axis=1))
        p_ref[pl.ds(off + 64 * j + 32, 32), :] = _pack(jnp.concatenate(hi, axis=1))

    def stage_a_safe(k, par, j, p_ref):
        s = scores(k, par, j)
        bias = jnp.where(causal, 0.0, MASKB).astype(f32)
        sd = s[128 * j:] + jnp.concatenate([bias] * 4, axis=1)
        s = sd if j == 0 else jnp.concatenate([s[:128 * j], sd], axis=0)
        p = jnp.exp2(s - jnp.max(s, axis=0, keepdims=True))
        p_ref[pl.ds(64 * (j * (j + 1) // 2), 64 * (j + 1)), :] = _pack(p)

    def stage_b(use_mem, oslot, k, par, j, p_ref, swapped=True):
        c = 2 * k + par
        base = QW * par
        mwin = base - base % 16
        moff = base - mwin
        zrow = 72 if moff == 0 else 0
        srow = _iota((8, 128), 0)
        g8 = g_s[c]
        off = 64 * (j * (j + 1) // 2)
        accs, dens = [], []
        for i in range(4):
            r0 = base + DH * i
            w = r0 - r0 % 16
            o = r0 - w
            vt = vt_u[pl.ds(_al(QW * k + w // 2, 8), 16), pl.ds(0, 128 * (j + 1))]
            orow = 15 if o < 14 else 0
            vt = jnp.where(_iota(vt.shape, 0) == orow, jnp.uint32(ONES2), vt)
            p = _tobf(p_ref[pl.ds(off, 64 * (j + 1)), pl.ds(128 * i, 128)])
            acc = _dot(_tobf(vt), p)
            if swapped and i % 2 == 0:
                acc = pltpu.roll(acc, 64, 1)
            dens.append(acc[2 * orow:2 * orow + 1])
            a0 = o - o % 8
            accs.append(acc[a0:a0 + 24])
        den4 = jnp.concatenate(dens, axis=0)
        den_s[0:4] = jnp.minimum(den_s[0:4], den4)
        den_s[4:8] = jnp.maximum(den_s[4:8], den4)
        if use_mem:
            mem = _dot_nt(_tobf(m_u[c]), _tobf(pqx[c, pl.ds(64 * j, 64), :]))
            r8 = g8 / jnp.concatenate([den4, mem[zrow:zrow + 4] + 1e-6], axis=0)
            rms = [r8[4 + i:5 + i] for i in range(4)]
        else:
            r8 = g8[0:4] / den4
        rds = [r8[i:i + 1] for i in range(4)]
        for v in range(9):
            lo_h, hi_h = (8 * v) // DH, (8 * v + 7) // DH

            def piece(h):
                a = accs[h][8 * (v - (DH * h) // 8):8 * (v - (DH * h) // 8) + 8]
                if not use_mem:
                    return a * rds[h]
                return a * rds[h] + mem[moff + 8 * v:moff + 8 * v + 8] * rms[h]
            val = piece(lo_h)
            if hi_h != lo_h:
                val = jnp.where(srow < DH * hi_h - 8 * v, val, piece(hi_h))
            ot_s[oslot, pl.ds(_al(2 * QW * k + base + 8 * v, 8), 8), pl.ds(128 * j, 128)] = val

    def mem_update(k, par):
        c = 2 * k + par
        base = QW * par
        mwin = base - base % 16
        moff = base - mwin
        zrow = 72 if moff == 0 else 0
        vw = vt_u[pl.ds(_al(QW * k + mwin // 2, 8), 40), :]
        rr = _iota(vw.shape, 0)
        isz = (rr >= 36) if moff == 0 else (rr < 4)
        vw = jnp.where(isz, jnp.uint32(ONES2), vw)
        upd = _dot(_tobf(vw), _tobf(pkx[c]))
        r80 = _iota((80, 128), 0)
        l80 = (_iota((80, 128), 1) - (2 * QW * k + base)) & 127
        hrow = jnp.where((r80 >= zrow) & (r80 < zrow + 8), r80 - zrow, (r80 - moff) // DH)
        keep = (l80 >= DH * hrow) & (l80 < DH * hrow + DH) & (hrow < 4) & (hrow >= 0)
        mnew = m_f[c] + jnp.where(keep, upd, 0.0)
        m_f[c] = mnew
        m_u[c] = _pack(mnew)

    pb = (p0, p1)

    def step(use_mem, update, oslot, a, b):
        for j in (3, 2, 1, 0):
            if a is not None:
                stage_a(a[0], a[1], j, pb[a[1]])
        for j in range(4):
            if b is not None:
                stage_b(use_mem, oslot, b[0], b[1], j, pb[b[1]])
        if b is not None and update:
            mem_update(b[0], b[1])

    def out_proj(s, t):
        c = 128 * t
        o = ot_s[s % 2, :, pl.ds(c, 128)].astype(bf)
        h = x_s[s, 0:D, pl.ds(c, 128)].astype(f32) + _dot(_tobf(wot_u[...]), o)
        h_s[4 * s + t] = h
        mean, rstd, sc = _ln_stats(lambda a, b: h[a:b], (wr_s[...], wrs_s[0:1]))
        st_s[4 * s + t, 0:1] = mean
        st_s[4 * s + t, 1:2] = rstd
        smax = jnp.max(sc, axis=1, keepdims=True)
        pos = (lane1 + (s * L + c)).astype(f32)
        sidx = jnp.min(jnp.where(sc == smax, pos, 1e9), axis=1, keepdims=True)
        new = jnp.concatenate([jnp.broadcast_to(smax, (1, 128)), jnp.broadcast_to(sidx, (1, 128)),
                               jnp.zeros((6, 128), f32)], axis=0)
        if t == 0:
            best_s[s] = new
        else:
            old = best_s[s]
            best_s[s] = jnp.where(smax > old[0:1, 0:1], new, old)

    def post(s, t):
        rstd = st_s[4 * s + t, 1:2]
        a = 1.0 + rstd
        b = st_s[4 * s + t, 0:1] * rstd
        out_s[s, :, pl.ds(128 * t, 128)] = (h_s[4 * s + t] * a - b).astype(bf)

    def finish(s):
        for t in range(4):
            out_proj(s, t)
            if t < 3:
                post(s, t)

    def attention(s):
        use_mem, update, o = s > 0, s < NSEG - 1, s % 2
        if s > 0:
            for t in range(4):
                out_proj(s - 1, t)
                post(s - 1, t)
        step(use_mem, update, o, (0, 0), None)
        for k in range(NQ // 2):
            step(use_mem, update, o, (k, 1), (k, 0))
            step(use_mem, update, o, (k + 1, 0) if k + 1 < NQ // 2 else None, (k, 1))
        if s > 0:
            out_copy(s - 1).start()

    half[0].wait()
    for t in range(2):
        prep(0, t)
    wq_lo.wait()
    w_copies[1].start()
    wq_hi.start()
    augment(wq_s, 0, 512)
    for t in range(2):
        proj_q(t)
    half[1].wait()
    w_copies[2].start()
    for t in range(2, 4):
        prep(0, t)
        proj_q(t)
    w_copies[1].wait()
    wq_hi.wait()
    augment(wq_s, 512, D)
    w_copies[3].start()
    for s in range(1, NSEG):
        x_copy(s).start()
    augment(wk_s)
    w4_u[...] = _tou(jnp.concatenate([wq_s[:, 512:D], wk_s[:, 512:D]], axis=1))
    for t in range(2):
        proj_k(t)
    w_copies[2].wait()
    augment(wv_s)
    wvt_u[...] = _tou(wv_s[...].T)
    wv_ok = jnp.max(jnp.abs(wv_s[0:D, :].astype(f32))) < WV_MAX
    for t in range(2, 4):
        proj_k(t)
    w_copies[3].wait()
    for c in small:
        c.wait()
    g32 = jax.nn.sigmoid(beta_ref[...].astype(f32)).reshape(1, H)
    sel = _iota((H, H), 1) == _iota((H, H), 0)
    gcol = jnp.sum(jnp.where(sel, g32, 0.0), axis=1, keepdims=True)
    for c in range(NQ):
        gq = jnp.broadcast_to(gcol[4 * c:4 * c + 4], (4, 128))
        g_s[c] = jnp.concatenate([1.0 - gq, gq], axis=0)
    wr_s[...] = jnp.broadcast_to(wr_ref[...].astype(f32).reshape(1, D), (128, D)).T
    wrs_s[...] = jnp.broadcast_to(jnp.sum(wr_s[...], axis=0, keepdims=True), (8, 128))
    wot_u[...] = _tou(wo_s[...].T)
    for t in range(4):
        proj_v(0, t)
    attention(0)
    for s in range(1, NSEG):
        x_copy(s).wait()

    for s in range(1, NSEG):
        e_copies[s - 1].start()
        for t in range(4):
            prep(s, t)
        for t in range(4):
            proj_v(s, t)
        for t in range(4):
            proj_q(t)
            proj_k(t)
        attention(s)
    finish(NSEG - 1)
    post(NSEG - 1, 3)
    out_copy(NSEG - 1).start()

    dl = den_s[...]
    safe = jnp.logical_and(jnp.min(dl[0:4]) >= DEN_LO, jnp.max(dl[4:8]) <= DEN_HI)
    safe = jnp.logical_and(safe, wv_ok)

    @pl.when(jnp.logical_not(safe))
    def _():
        for s in range(NSEG):
            out_copy(s).wait()
        m_f[...] = jnp.zeros_like(m_f)
        m_u[...] = jnp.zeros_like(m_u)

        def seg_redo(s, carry):
            for t in range(4):
                prep(s, t)
                proj_v(s, t)
                proj_q(t)
                proj_k(t)

            def quads(k, carry):
                for par in range(2):
                    for j in range(4):
                        stage_a_safe(k, par, j, pb[par])
                        stage_b(True, s % 2, k, par, j, pb[par], swapped=False)
                    mem_update(k, par)
                return carry
            lax.fori_loop(0, NQ // 2, quads, 0)
            finish(s)
            post(s, 3)
            out_copy(s).start()
            return carry
        lax.fori_loop(0, NSEG, seg_redo, 0)

    for c in e_copies:
        c.wait()
    best = best_s[0]
    for s in range(1, NSEG):
        cand = best_s[s]
        best = jnp.where(cand[0:1, 0:1] > best[0:1, 0:1], cand, best)
    idx = jnp.clip(best[1, 0].astype(i32), 0, S - 1)
    blk = idx // 128
    col = idx - blk * 128
    onehot = ((_iota((16, 128), 1) == col) & (_iota((16, 128), 0) == 0)).astype(bf)
    ln = ((h_s[blk] - st_s[blk, 0:1]) * st_s[blk, 1:2]).astype(bf)
    xs = _dot_nt(onehot, ln).astype(bf)
    accs = [None] * (D // 8)
    for g in range(F // E_GRP):
        c0, c1 = E_GRP * g, E_GRP * (g + 1)
        gate = _dot(xs, wg_s[:, c0:c1])[0:1]
        up = _dot(xs, wu_s[:, c0:c1])[0:1]
        act = (gate * jax.nn.sigmoid(gate) * up).astype(bf).astype(f32)
        for i in range(D // 8):
            w = wd_s[8 * i:8 * i + 8, c0:c1].astype(f32) * act
            tot = w[:, 0:128]
            for c in range(1, E_GRP // 128):
                tot = tot + w[:, 128 * c:128 * (c + 1)]
            accs[i] = tot if g == 0 else accs[i] + tot
    yv = jnp.sum(jnp.concatenate(accs, axis=0), axis=1, keepdims=True)
    yt = yv * jax.nn.sigmoid(best[0:1, 0:1])
    for s in range(NSEG):
        out_copy(s).wait()
    seg = blk // 4
    c0 = pl.multiple_of((blk - seg * 4) * 128, 128)
    cur = out_s[seg, :, pl.ds(c0, 128)].astype(f32)
    hit = _iota((D, 128), 1) == col
    fin_s[...] = (cur + jnp.where(hit, yt, 0.0)).astype(bf)
    fin = cp(fin_s, out_hbm.at[:, pl.ds(pl.multiple_of(blk * 128, 128), 128)], sems.at[15])
    fin.start()
    fin.wait()


@jax.jit
def pallas_sequential_preLN__memory_aug_infini_attn__moe_arch_mod__prompt_kernel(
    A_x, A_wq, A_wk, A_wv, A_wo, A_beta, B_x, B_w_r, B_w_gate, B_w_up, B_w_down,
):
    hbm = pl.BlockSpec(memory_space=pltpu.HBM)
    vm = pltpu.VMEM
    x_t = A_x.reshape(S, D).T
    out_t = pl.pallas_call(
        _kernel,
        out_shape=jax.ShapeDtypeStruct((D, S), bf),
        in_specs=[hbm] * 10,
        out_specs=hbm,
        scratch_shapes=[
            vm((NSEG, DP, L), bf), vm((DP, D), bf), vm((DP, D), bf), vm((DP, D), bf), vm((D, D), bf),
            vm((D, F), bf), vm((D, F), bf), vm((D, F), bf),
            vm((DP // 2, 128), u32), vm((D // 2, DP), u32), vm((D // 2, D), u32),
            vm((L // 2, DP), u32), vm((4, 8, 128), f32), vm((4, 128, 128), f32),
            vm((NQ, L // 2, 128), u32), vm((NQ, L // 2, 128), u32),
            vm((NQ, L // 2, 128), u32), vm((NQ, L // 2, 128), u32),
            vm((D // 2, L), u32),
            vm((640, 512), u32), vm((640, 512), u32), vm((16, D, 128), f32),
            vm((2, D, L), f32), vm((NQ, 80, 128), f32), vm((NQ, 40, 128), u32),
            vm((NQ, 8, 128), f32), vm((D, 128), f32), vm((8, 128), f32), vm((NSEG, D, L), bf),
            vm((16, 8, 128), f32),
            vm((NSEG, 8, 128), f32), vm((8, 128), f32), vm((D, 128), bf),
            vm((H,), bf), vm((D,), bf),
            pltpu.SemaphoreType.DMA((20,)),
        ],
        compiler_params=pltpu.CompilerParams(vmem_limit_bytes=100 * 1024 * 1024),
        name="infini_moe",
    )(x_t, A_wq, A_wk, A_wv, A_wo, A_beta, B_w_r, B_w_gate, B_w_up, B_w_down.T)
    return out_t.T.reshape(1, S, D)
```

```python
import jax
import jax.numpy as jnp
from jax import lax
from jax.experimental import pallas as pl
from jax.experimental.pallas import tpu as pltpu

S, D, H, DH = 2048, 576, 32, 18
NSEG, L, F = 4, 512, 4608
DP = 640
NQ = 8
QW = 4 * DH
bf, u32, f32, i32 = jnp.bfloat16, jnp.uint32, jnp.float32, jnp.int32
LOG2E = 1.4426950408889634
QSCALE = DH ** -0.5 * LOG2E
MASKB = -1000000000.0 * LOG2E
EPS = 1e-5
NT = (((1,), (1,)), ((), ()))
ONES2 = 0x3F803F80
E_GRP = 256
DEN_LO, DEN_HI, WV_MAX = 2.0 ** -60, 2.0 ** 60, 2.0 ** 40


def _tobf(x):
    return pltpu.bitcast(x, bf)


def _tou(x):
    return pltpu.bitcast(x, u32)


def _pack(x):
    return pltpu.bitcast(x.astype(bf), u32)


def _dot(a, b):
    return jnp.dot(a, b, preferred_element_type=f32)


def _dot_nt(a, b):
    return lax.dot_general(a, b, NT, preferred_element_type=f32)


def _phi(t):
    return jnp.where(t > 0, t + 1.0, jnp.exp(t))


def _sigmoid(t):
    return 0.5 * jnp.tanh(0.5 * t) + 0.5


def _rowsum(parts):
    acc = [jnp.sum(p.reshape(p.shape[0] // 8, 8, 128), axis=0) for p in parts]
    while len(acc) > 1:
        acc = [acc[i] + acc[i + 1] for i in range(0, len(acc), 2)]
    return jnp.sum(acc[0], axis=0, keepdims=True)


def _ln_stats(rows, w=None):
    d = [rows(144 * g, 144 * (g + 1)) for g in range(4)]
    m1 = _rowsum(d) * (1.0 / D)
    m2 = _rowsum([v * v for v in d]) * (1.0 / D)
    var = jnp.maximum(m2 - m1 * m1, 0.0)
    rstd = lax.rsqrt(var + EPS)
    if w is None:
        return m1, rstd
    dw = _rowsum([d[g] * w[0][144 * g:144 * (g + 1)] for g in range(4)])
    return m1, rstd, (dw - m1 * w[1]) * rstd


def _hi_lo(v):
    hi = v.astype(bf).astype(f32)
    return hi, (v - hi).astype(bf).astype(f32)


def _iota(shape, dim):
    return lax.broadcasted_iota(i32, shape, dim)


def _al(x, n):
    return x if isinstance(x, int) else pl.multiple_of(x, n)


def _kernel(x_hbm, wq_hbm, wk_hbm, wv_hbm, wo_hbm, beta_hbm, wr_hbm,
            wg_hbm, wu_hbm, wd_hbm, out_hbm,
            x_s, wq_s, wk_s, wv_s, wo_s, wg_s, wu_s, wd_s,
            w4_u, wvt_u, wot_u, xn_u, rs_s, rc_s, qx, kx, pqx, pkx, vt_u,
            p0, p1, h_s, ot_s, m_f, m_u, g_s, wr_s, wrs_s, out_s, st_s, best_s, den_s, fin_s,
            beta_ref, wr_ref, sems):
    cp = pltpu.make_async_copy

    def x_copy(s):
        return cp(x_hbm.at[:, pl.ds(_al(s * L, L), L)], x_s.at[s, pl.ds(0, D), :], sems.at[s])

    def out_copy(s):
        return cp(out_s.at[s], out_hbm.at[:, pl.ds(_al(s * L, L), L)], sems.at[11 + s])

    def prep(s, t):
        c = _al(128 * t, 128)
        mean, rstd = _ln_stats(lambda a, b: x_s[s, a:b, pl.ds(c, 128)].astype(f32))
        mh, ml = _hi_lo(mean)
        r16 = _iota((16, 128), 0)
        x_s[s, D:D + 16, pl.ds(c, 128)] = jnp.where(
            r16 < 2, mh, jnp.where(r16 == 2, ml, 0.0)).astype(bf)
        rs_s[t, 0:1] = rstd
        rc_s[t] = jnp.broadcast_to(rstd, (128, 128)).T
        xn_u[pl.ds(_al(64 * t, 64), 64), :] = _tou(x_s[s, :, pl.ds(c, 128)].T)

    def augment(w_ref, a=0, b=D):
        ones = jnp.ones((16, D), bf)
        hi, lo = _hi_lo(_dot(ones, w_ref[0:D, a:b])[0:1])
        r16 = _iota((16, b - a), 0)
        w_ref[D:D + 16, a:b] = jnp.where((r16 == 0) | (r16 == 2), -hi,
                                         jnp.where(r16 == 1, -lo, 0.0)).astype(bf)

    top = pl.ds(0, D)
    w_copies = [None, cp(wk_hbm, wk_s.at[top, :], sems.at[5]),
                cp(wv_hbm, wv_s.at[top, :], sems.at[6]), cp(wo_hbm, wo_s, sems.at[7])]
    e_copies = [cp(wg_hbm, wg_s, sems.at[8]), cp(wu_hbm, wu_s, sems.at[9]),
                cp(wd_hbm, wd_s, sems.at[10])]

    small = [cp(beta_hbm, beta_ref, sems.at[16]), cp(wr_hbm, wr_ref, sems.at[17])]
    half = [cp(x_hbm.at[:, pl.ds(256 * i, 256)], x_s.at[0, top, pl.ds(256 * i, 256)],
               sems.at[18 * i]) for i in range(2)]
    wq_lo = cp(wq_hbm.at[:, pl.ds(0, 512)], wq_s.at[top, pl.ds(0, 512)], sems.at[4])
    wq_hi = cp(wq_hbm.at[:, pl.ds(512, D - 512)], wq_s.at[top, pl.ds(512, D - 512)], sems.at[19])
    half[0].start()
    wq_lo.start()
    half[1].start()
    for c in small:
        c.start()

    m_f[...] = jnp.zeros_like(m_f)
    den_s[...] = jnp.ones_like(den_s)

    for w_ref in (wq_s, wk_s, wv_s):
        w_ref[D + 16:DP, :] = jnp.zeros((DP - D - 16, D), bf)
    for s in range(NSEG):
        x_s[s, D + 16:DP, :] = jnp.zeros((DP - D - 16, L), bf)

    lane1 = _iota((1, 128), 1)
    causal = _iota((128, 128), 0) <= _iota((128, 128), 1)

    def proj_q(t):
        rows = pl.ds(_al(64 * t, 64), 64)
        q = _dot(_tobf(xn_u[rows, :]), wq_s[:, 0:512]) * jnp.concatenate([rc_s[t]] * 4, axis=1)
        tiles = [q[:, 128 * i:128 * (i + 1)] for i in range(4)]
        raw = [_pack(v * QSCALE) for v in tiles]
        ph = [_pack(_phi(v)) for v in tiles]
        for c in range(NQ):
            i = c // 2
            if c % 2 == 0 or c == NQ - 1:
                qx[c, rows, :] = raw[i]
                pqx[c, rows, :] = ph[i]
            else:
                keep = lane1 >= (QW * c) % 128
                qx[c, rows, :] = jnp.where(keep, raw[i], raw[i + 1])
                pqx[c, rows, :] = jnp.where(keep, ph[i], ph[i + 1])

    def proj_k(t):
        rows = pl.ds(_al(64 * t, 64), 64)
        xn = _tobf(xn_u[rows, :])
        rc = rc_s[t]
        k = _dot(xn, wk_s[:, 0:512]) * jnp.concatenate([rc] * 4, axis=1)
        r4 = _dot(xn, _tobf(w4_u[...])) * rc
        tiles = [k[:, 128 * i:128 * (i + 1)] for i in range(4)] + [pltpu.roll(r4, 64, 1)]
        raw = [_pack(v) for v in tiles]
        ph = [_pack(_phi(v)) for v in tiles]
        for c in range(NQ):
            i = c // 2
            if c % 2 == 0:
                kx[c, rows, :] = raw[i]
                pkx[c, rows, :] = ph[i]
            else:
                keep = lane1 >= (QW * c) % 128
                kx[c, rows, :] = jnp.where(keep, raw[i], raw[i + 1])
                pkx[c, rows, :] = jnp.where(keep, ph[i], ph[i + 1])
        keep = lane1 >= (QW * (NQ - 1)) % 128
        qx[NQ - 1, rows, :] = jnp.where(keep, qx[NQ - 1, rows, :], _pack(r4 * QSCALE))
        pqx[NQ - 1, rows, :] = jnp.where(keep, pqx[NQ - 1, rows, :], _pack(_phi(r4)))

    def proj_v(s, t):
        c = pl.ds(_al(128 * t, 128), 128)
        vt_u[:, c] = _pack(_dot(_tobf(wvt_u[...]), x_s[s, :, c]) * rs_s[t, 0:1])

    def masked_q(k, par, j):
        q = qx[2 * k + par, pl.ds(64 * j, 64), :]
        out = []
        for i in range(4):
            st = (2 * QW * k + QW * par + DH * i) % 128
            out.append(q & jnp.where(((lane1 - st) & 127) < DH, jnp.uint32(0xFFFFFFFF),
                                     jnp.uint32(0)))
        return out

    def scores(k, par, j):
        qm = _tobf(jnp.concatenate(masked_q(k, par, j), axis=0))
        kk = _tobf(kx[2 * k + par, pl.ds(0, 64 * (j + 1)), :])
        return _dot_nt(kk, qm)

    r64, l64 = _iota((64, 128), 0), _iota((64, 128), 1)
    lo_nat = (l64 >= 64) | (r64 <= l64)
    lo_swp = (l64 < 64) | (r64 <= l64 - 64)
    hi_even = (l64 < 64) & (r64 <= l64)
    hi_odd = (l64 >= 64) & (r64 <= l64 - 64)

    def stage_a(k, par, j, p_ref):
        c = 2 * k + par
        qm = masked_q(k, par, j)
        w1 = [jnp.concatenate([qm[i][32:], qm[i][:32]], axis=0) if i % 2 == 0 else qm[i]
              for i in range(4)]
        w2 = [qm[i][32:] for i in range(4)]
        n1 = 128 * j + 64
        p1 = jnp.exp2(_dot_nt(_tobf(kx[c, pl.ds(0, n1 // 2), :]),
                              _tobf(jnp.concatenate(w1, axis=0))))
        p2 = jnp.exp2(_dot_nt(_tobf(kx[c, pl.ds(n1 // 2, 32), :]),
                              _tobf(jnp.concatenate(w2, axis=0))))
        off = 64 * (j * (j + 1) // 2)
        if j > 0:
            p_ref[pl.ds(off, 64 * j), :] = _pack(p1[:128 * j])
        lo = [jnp.where(lo_swp if i % 2 == 0 else lo_nat,
                        p1[128 * j:, 128 * i:128 * (i + 1)], 0.0) for i in range(4)]
        hi = [jnp.where(hi_even if i % 2 == 0 else hi_odd,
                        p2[:, 128 * (i // 2):128 * (i // 2 + 1)], 0.0) for i in range(4)]
        p_ref[pl.ds(off + 64 * j, 32), :] = _pack(jnp.concatenate(lo, axis=1))
        p_ref[pl.ds(off + 64 * j + 32, 32), :] = _pack(jnp.concatenate(hi, axis=1))

    def stage_a_safe(k, par, j, p_ref):
        s = scores(k, par, j)
        bias = jnp.where(causal, 0.0, MASKB).astype(f32)
        sd = s[128 * j:] + jnp.concatenate([bias] * 4, axis=1)
        s = sd if j == 0 else jnp.concatenate([s[:128 * j], sd], axis=0)
        p = jnp.exp2(s - jnp.max(s, axis=0, keepdims=True))
        p_ref[pl.ds(64 * (j * (j + 1) // 2), 64 * (j + 1)), :] = _pack(p)

    def stage_b(use_mem, oslot, k, par, j, p_ref, swapped=True):
        c = 2 * k + par
        base = QW * par
        mwin = base - base % 16
        moff = base - mwin
        zrow = 72 if moff == 0 else 0
        srow = _iota((8, 128), 0)
        g8 = g_s[c]
        off = 64 * (j * (j + 1) // 2)
        accs, dens = [], []
        for i in range(4):
            r0 = base + DH * i
            w = r0 - r0 % 16
            o = r0 - w
            vt = vt_u[pl.ds(_al(QW * k + w // 2, 8), 16), pl.ds(0, 128 * (j + 1))]
            orow = 15 if o < 14 else 0
            vt = jnp.where(_iota(vt.shape, 0) == orow, jnp.uint32(ONES2), vt)
            p = _tobf(p_ref[pl.ds(off, 64 * (j + 1)), pl.ds(128 * i, 128)])
            acc = _dot(_tobf(vt), p)
            if swapped and i % 2 == 0:
                acc = pltpu.roll(acc, 64, 1)
            dens.append(acc[2 * orow:2 * orow + 1])
            a0 = o - o % 8
            accs.append(acc[a0:a0 + 24])
        den4 = jnp.concatenate(dens, axis=0)
        den_s[0:4] = jnp.minimum(den_s[0:4], den4)
        den_s[4:8] = jnp.maximum(den_s[4:8], den4)
        if use_mem:
            mem = _dot_nt(_tobf(m_u[c]), _tobf(pqx[c, pl.ds(64 * j, 64), :]))
            r8 = g8 / jnp.concatenate([den4, mem[zrow:zrow + 4] + 1e-6], axis=0)
            rms = [r8[4 + i:5 + i] for i in range(4)]
        else:
            r8 = g8[0:4] / den4
        rds = [r8[i:i + 1] for i in range(4)]
        for v in range(9):
            lo_h, hi_h = (8 * v) // DH, (8 * v + 7) // DH

            def piece(h):
                a = accs[h][8 * (v - (DH * h) // 8):8 * (v - (DH * h) // 8) + 8]
                if not use_mem:
                    return a * rds[h]
                return a * rds[h] + mem[moff + 8 * v:moff + 8 * v + 8] * rms[h]
            val = piece(lo_h)
            if hi_h != lo_h:
                val = jnp.where(srow < DH * hi_h - 8 * v, val, piece(hi_h))
            ot_s[oslot, pl.ds(_al(2 * QW * k + base + 8 * v, 8), 8), pl.ds(128 * j, 128)] = val

    def mem_update(k, par):
        c = 2 * k + par
        base = QW * par
        mwin = base - base % 16
        moff = base - mwin
        zrow = 72 if moff == 0 else 0
        vw = vt_u[pl.ds(_al(QW * k + mwin // 2, 8), 40), :]
        rr = _iota(vw.shape, 0)
        isz = (rr >= 36) if moff == 0 else (rr < 4)
        vw = jnp.where(isz, jnp.uint32(ONES2), vw)
        upd = _dot(_tobf(vw), _tobf(pkx[c]))
        r80 = _iota((80, 128), 0)
        l80 = (_iota((80, 128), 1) - (2 * QW * k + base)) & 127
        hrow = jnp.where((r80 >= zrow) & (r80 < zrow + 8), r80 - zrow, (r80 - moff) // DH)
        keep = (l80 >= DH * hrow) & (l80 < DH * hrow + DH) & (hrow < 4) & (hrow >= 0)
        mnew = m_f[c] + jnp.where(keep, upd, 0.0)
        m_f[c] = mnew
        m_u[c] = _pack(mnew)

    pb = (p0, p1)

    def step(use_mem, update, oslot, a, b):
        for j in (3, 2, 1, 0):
            if a is not None:
                stage_a(a[0], a[1], j, pb[a[1]])
        for j in range(4):
            if b is not None:
                stage_b(use_mem, oslot, b[0], b[1], j, pb[b[1]])
        if b is not None and update:
            mem_update(b[0], b[1])

    def out_proj(s, t):
        c = _al(128 * t, 128)
        o = ot_s[s % 2, :, pl.ds(c, 128)].astype(bf)
        h = x_s[s, 0:D, pl.ds(c, 128)].astype(f32) + _dot(_tobf(wot_u[...]), o)
        h_s[4 * s + t] = h
        mean, rstd, sc = _ln_stats(lambda a, b: h[a:b], (wr_s[...], wrs_s[0:1]))
        st_s[4 * s + t, 0:1] = mean
        st_s[4 * s + t, 1:2] = rstd
        smax = jnp.max(sc, axis=1, keepdims=True)
        pos = (lane1 + (s * L + c)).astype(f32)
        sidx = jnp.min(jnp.where(sc == smax, pos, 1e9), axis=1, keepdims=True)
        new = jnp.concatenate([jnp.broadcast_to(smax, (1, 128)), jnp.broadcast_to(sidx, (1, 128)),
                               jnp.zeros((6, 128), f32)], axis=0)
        if isinstance(t, int) and t == 0:
            best_s[s] = new
        else:
            old = best_s[s]
            better = smax > old[0:1, 0:1]
            if not isinstance(t, int):
                better = jnp.logical_or(better, t == 0)
            best_s[s] = jnp.where(better, new, old)

    def post(s, t):
        rstd = st_s[4 * s + t, 1:2]
        a = 1.0 + rstd
        b = st_s[4 * s + t, 0:1] * rstd
        out_s[s, :, pl.ds(_al(128 * t, 128), 128)] = (h_s[4 * s + t] * a - b).astype(bf)

    def finish(s):
        for t in range(4):
            out_proj(s, t)
            if t < 3:
                post(s, t)

    def attention(s):
        use_mem, update, o = s > 0, s < NSEG - 1, s % 2
        if s > 0:
            for t in range(4):
                out_proj(s - 1, t)
                post(s - 1, t)
        step(use_mem, update, o, (0, 0), None)
        for k in range(NQ // 2):
            step(use_mem, update, o, (k, 1), (k, 0))
            step(use_mem, update, o, (k + 1, 0) if k + 1 < NQ // 2 else None, (k, 1))
        if s > 0:
            out_copy(s - 1).start()

    half[0].wait()
    for t in range(2):
        prep(0, t)
    wq_lo.wait()
    w_copies[1].start()
    wq_hi.start()
    augment(wq_s, 0, 512)
    for t in range(2):
        proj_q(t)
    half[1].wait()
    w_copies[2].start()
    for t in range(2, 4):
        prep(0, t)
        proj_q(t)
    w_copies[1].wait()
    wq_hi.wait()
    augment(wq_s, 512, D)
    w_copies[3].start()
    for s in range(1, NSEG):
        x_copy(s).start()
    augment(wk_s)
    w4_u[...] = _tou(jnp.concatenate([wq_s[:, 512:D], wk_s[:, 512:D]], axis=1))
    for t in range(2):
        proj_k(t)
    w_copies[2].wait()
    augment(wv_s)
    wvt_u[...] = _tou(wv_s[...].T)
    wv_ok = jnp.max(jnp.abs(wv_s[0:D, :].astype(f32))) < WV_MAX
    for t in range(2, 4):
        proj_k(t)
    w_copies[3].wait()
    for c in small:
        c.wait()
    g32 = jax.nn.sigmoid(beta_ref[...].astype(f32)).reshape(1, H)
    sel = _iota((H, H), 1) == _iota((H, H), 0)
    gcol = jnp.sum(jnp.where(sel, g32, 0.0), axis=1, keepdims=True)
    for c in range(NQ):
        gq = jnp.broadcast_to(gcol[4 * c:4 * c + 4], (4, 128))
        g_s[c] = jnp.concatenate([1.0 - gq, gq], axis=0)
    wr_s[...] = jnp.broadcast_to(wr_ref[...].astype(f32).reshape(1, D), (128, D)).T
    wrs_s[...] = jnp.broadcast_to(jnp.sum(wr_s[...], axis=0, keepdims=True), (8, 128))
    wot_u[...] = _tou(wo_s[...].T)
    for t in range(4):
        proj_v(0, t)
    attention(0)
    for s in range(1, NSEG):
        x_copy(s).wait()

    for s in range(1, NSEG):
        e_copies[s - 1].start()
        for t in range(4):
            prep(s, t)
        for t in range(4):
            proj_v(s, t)
        for t in range(4):
            proj_q(t)
            proj_k(t)
        attention(s)
    finish(NSEG - 1)
    post(NSEG - 1, 3)
    out_copy(NSEG - 1).start()

    dl = den_s[...]
    safe = jnp.logical_and(jnp.min(dl[0:4]) >= DEN_LO, jnp.max(dl[4:8]) <= DEN_HI)
    safe = jnp.logical_and(safe, wv_ok)

    @pl.when(jnp.logical_not(safe))
    def _():
        for s in range(NSEG):
            out_copy(s).wait()
        m_f[...] = jnp.zeros_like(m_f)
        m_u[...] = jnp.zeros_like(m_u)

        def seg_redo(s, carry):
            def inputs(t, carry):
                prep(s, t)
                proj_v(s, t)
                proj_q(t)
                proj_k(t)
                return carry
            lax.fori_loop(0, 4, inputs, 0)

            def quads(k, carry):
                for par in range(2):
                    for j in range(4):
                        stage_a_safe(k, par, j, pb[par])
                        stage_b(True, s % 2, k, par, j, pb[par], swapped=False)
                    mem_update(k, par)
                return carry
            lax.fori_loop(0, NQ // 2, quads, 0)

            def outputs(t, carry):
                out_proj(s, t)
                post(s, t)
                return carry
            lax.fori_loop(0, 4, outputs, 0)
            out_copy(s).start()
            return carry
        lax.fori_loop(0, NSEG, seg_redo, 0)

    for c in e_copies:
        c.wait()
    best = best_s[0]
    for q in range(1, NSEG):
        cand = best_s[q]
        best = jnp.where(cand[0:1, 0:1] > best[0:1, 0:1], cand, best)
    idx = jnp.clip(best[1, 0].astype(i32), 0, S - 1)
    blk = idx // 128
    col = idx - blk * 128
    onehot = ((_iota((16, 128), 1) == col) & (_iota((16, 128), 0) == 0)).astype(bf)
    ln = ((h_s[blk] - st_s[blk, 0:1]) * st_s[blk, 1:2]).astype(bf)
    xs = _dot_nt(onehot, ln).astype(bf)
    accs = [None] * (D // 8)
    for g in range(F // E_GRP):
        c0, c1 = E_GRP * g, E_GRP * (g + 1)
        gate = _dot(xs, wg_s[:, c0:c1])[0:1]
        up = _dot(xs, wu_s[:, c0:c1])[0:1]
        act = (gate * _sigmoid(gate) * up).astype(bf).astype(f32)
        for i in range(D // 8):
            w = wd_s[8 * i:8 * i + 8, c0:c1].astype(f32) * act
            tot = w[:, 0:128]
            for c in range(1, E_GRP // 128):
                tot = tot + w[:, 128 * c:128 * (c + 1)]
            accs[i] = tot if g == 0 else accs[i] + tot
    yv = jnp.sum(jnp.concatenate(accs, axis=0), axis=1, keepdims=True)
    yt = yv * jax.nn.sigmoid(best[0:1, 0:1])
    seg = blk // 4
    c0 = pl.multiple_of((blk - seg * 4) * 128, 128)
    cur = out_s[seg, :, pl.ds(c0, 128)].astype(f32)
    hit = _iota((D, 128), 1) == col
    fin_s[...] = (cur + jnp.where(hit, yt, 0.0)).astype(bf)
    for s in range(NSEG):
        out_copy(s).wait()
    fin = cp(fin_s, out_hbm.at[:, pl.ds(pl.multiple_of(blk * 128, 128), 128)], sems.at[15])
    fin.start()
    fin.wait()


@jax.jit
def pallas_sequential_preLN__memory_aug_infini_attn__moe_arch_mod__prompt_kernel(
    A_x, A_wq, A_wk, A_wv, A_wo, A_beta, B_x, B_w_r, B_w_gate, B_w_up, B_w_down,
):
    hbm = pl.BlockSpec(memory_space=pltpu.HBM)
    vm = pltpu.VMEM
    x_t = A_x.reshape(S, D).T
    out_t = pl.pallas_call(
        _kernel,
        out_shape=jax.ShapeDtypeStruct((D, S), bf),
        in_specs=[hbm] * 10,
        out_specs=hbm,
        scratch_shapes=[
            vm((NSEG, DP, L), bf), vm((DP, D), bf), vm((DP, D), bf), vm((DP, D), bf), vm((D, D), bf),
            vm((D, F), bf), vm((D, F), bf), vm((D, F), bf),
            vm((DP // 2, 128), u32), vm((D // 2, DP), u32), vm((D // 2, D), u32),
            vm((L // 2, DP), u32), vm((4, 8, 128), f32), vm((4, 128, 128), f32),
            vm((NQ, L // 2, 128), u32), vm((NQ, L // 2, 128), u32),
            vm((NQ, L // 2, 128), u32), vm((NQ, L // 2, 128), u32),
            vm((D // 2, L), u32),
            vm((640, 512), u32), vm((640, 512), u32), vm((16, D, 128), f32),
            vm((2, D, L), f32), vm((NQ, 80, 128), f32), vm((NQ, 40, 128), u32),
            vm((NQ, 8, 128), f32), vm((D, 128), f32), vm((8, 128), f32), vm((NSEG, D, L), bf),
            vm((16, 8, 128), f32),
            vm((NSEG, 8, 128), f32), vm((8, 128), f32), vm((D, 128), bf),
            vm((H,), bf), vm((D,), bf),
            pltpu.SemaphoreType.DMA((20,)),
        ],
        compiler_params=pltpu.CompilerParams(vmem_limit_bytes=100 * 1024 * 1024),
        name="infini_moe",
    )(x_t, A_wq, A_wk, A_wv, A_wo, A_beta, B_w_r, B_w_gate, B_w_up, B_w_down.T)
    return out_t.T.reshape(1, S, D)
```
